```python
import jax
import jax.numpy as jnp

def _softmax(x, axis=-1):
    return jax.nn.softmax(x, axis=axis)
def _gelu(x):
    return jax.nn.gelu(x, approximate=True)
def _silu(x):
    return jax.nn.silu(x)
def _sigmoid(x):
    return jax.nn.sigmoid(x)
def _layernorm(x, axis=-1, eps=1e-5):
    m = jnp.mean(x, axis=axis, keepdims=True)
    v = jnp.var(x, axis=axis, keepdims=True)
    return (x - m) / jnp.sqrt(v + eps)
def _scatter_add(tgt, idx, src, axis=0):
    return tgt.at[idx].add(src)
def _segment_sum(src, seg, n):
    return jax.ops.segment_sum(src, seg, n)
class _Rng:
    def __init__(self, key):
        self._k = key
    def _next(self):
        self._k, sub = jax.random.split(self._k)
        return sub
    def normal(self, shape):
        return jax.random.normal(self._next(), shape, dtype=jnp.bfloat16)
    def randint(self, lo, hi, shape):
        return jax.random.randint(self._next(), shape, lo, hi, dtype=jnp.int32)
    def uniform(self, shape, lo=0.0, hi=1.0):
        return jax.random.uniform(self._next(), shape, jnp.bfloat16, lo, hi)
    def permutation(self, n):
        return jax.random.permutation(self._next(), n)


kernel_name = 'interleave_layers__sliding_block__moe_arch_mod__prompt'

def setup_inputs():
    _rng = _Rng(jax.random.key(int.from_bytes(__import__("os").urandom(4), "little")))
    _w = (lambda a: (lambda t: t.astype(jnp.bfloat16) if jnp.issubdtype(t.dtype, jnp.floating) else t)(jnp.asarray(a)))
    def _A_setup():
        B, S, D = 1, 2048, 1024
        return {
            "x": _w((lambda *s: _rng.normal(s) * 0.05)(B, S, D)),
            "wqkv": _w((lambda *s: _rng.normal(s) * 0.05)(D, 3 * D)),
            "wo": _w((lambda *s: _rng.normal(s) * 0.05)(D, D)),
        }
    _A_in = _A_setup()

    def _B_setup():
        B, S, D, F, C = 1, 2048, 1024, 3584, 1
        return {
            "x": _w((lambda *s: _rng.normal(s) * 0.05)(B, S, D)),
            "w_r": _w((lambda *s: _rng.normal(s) * 0.05)(D)),
            "w_gate": _w((lambda *s: _rng.normal(s) * 0.05)(D, F)),
            "w_up": _w((lambda *s: _rng.normal(s) * 0.05)(D, F)),
            "w_down": _w((lambda *s: _rng.normal(s) * 0.05)(F, D)),
        }
    _B_in = _B_setup()

    return {
        "A_x": _A_in["x"],
        "A_wqkv": _A_in["wqkv"],
        "A_wo": _A_in["wo"],
        "B_x": _B_in["x"],
        "B_w_r": _B_in["w_r"],
        "B_w_gate": _B_in["w_gate"],
        "B_w_up": _B_in["w_up"],
        "B_w_down": _B_in["w_down"],
    }

def reference(A_x, A_wqkv, A_wo, B_x, B_w_r, B_w_gate, B_w_up, B_w_down):
    def _A_ref(x, wqkv, wo):
        B, S, D = x.shape
        H = 32; Dh = D // H; W = 256
        qkv = (lambda x, *d: x.transpose(*d))((x @ wqkv).reshape(B, S, 3, H, Dh), 2, 0, 3, 1, 4)
        q, k, v = qkv[0], qkv[1], qkv[2]
        scores = jnp.einsum("bhqd,bhkd->bhqk", q, k) * (Dh ** -0.5)
        idx = jnp.arange(S)
        mask = (idx[:, None] - idx[None, :] >= 0) & (idx[:, None] - idx[None, :] < W)
        scores = jnp.where(mask[None, None], scores, -1e9)
        p = _softmax(scores, axis=-1)
        o = jnp.einsum("bhqk,bhkd->bhqd", p, v)
        return (lambda x, *d: x.transpose(*d))(o, 0, 2, 1, 3).reshape(B, S, D) @ wo

    def _B_ref(x, w_r, w_gate, w_up, w_down):
        B, S, D = x.shape
        C = 1
        r = x @ w_r
        idx = jnp.argsort(-r, axis=-1)[:, :C]
        idx_e = jnp.repeat(idx.reshape(B, C, 1), D, axis=2)
        x_sel = jnp.take_along_axis(x, idx_e, axis=1)
        g = _silu(x_sel @ w_gate)
        u = x_sel @ w_up
        y = (g * u) @ w_down
        r_sel = _sigmoid(jnp.take_along_axis(r, idx, axis=1))
        y = y * r_sel.reshape(B, C, 1)
        b_off = (jnp.arange(B) * S).reshape(B, 1)
        flat_idx = (idx + b_off).reshape(B * C)
        zero = (x * 0.0).reshape(B * S, D)
        upd = _scatter_add(zero, flat_idx, y.reshape(B * C, D), axis=0)
        return x + upd.reshape(B, S, D)

    x = A_x
    x = x + _A_ref(_layernorm(x, axis=-1), A_wqkv, A_wo)
    x = x + _B_ref(_layernorm(x, axis=-1), B_w_r, B_w_gate, B_w_up, B_w_down)
    x = x + _A_ref(_layernorm(x, axis=-1), A_wqkv, A_wo)
    x = x + _B_ref(_layernorm(x, axis=-1), B_w_r, B_w_gate, B_w_up, B_w_down)
    return x
```

```python
import math

import jax
import jax.numpy as jnp
import jax.experimental.pallas as pl
import jax.experimental.pallas.tpu as pltpu

F32 = jnp.float32
BF16 = jnp.bfloat16
U32 = jnp.uint32
I32 = jnp.int32

S = 2048
D = 1024
DH = 32
WIN = 256
FF = 3584
NG = 8
SB = 128
NSB = S // SB
QA = 32
XR = WIN + QA
TB = 256
NTB = S // TB
EPS = 1e-5
NEG = -1e30
QSCALE = (DH ** -0.5) * math.log2(math.e)
NT_DIMS = (((1,), (1,)), ((), ()))
N_LAYERS = 2


def _layernorm(x):
    mean = jnp.sum(x, axis=1, keepdims=True) * (1.0 / D)
    xc = x - mean
    var = jnp.sum(xc * xc, axis=1, keepdims=True) * (1.0 / D)
    return xc * jax.lax.rsqrt(var + EPS)


def _packed(ref):
    return ref.bitcast(U32)


def _as_bf16(v):
    return pltpu.bitcast(v, BF16)


def _ln_stage(xres, xn, r0):
    y = _layernorm(xres[pl.ds(r0, TB), :].astype(F32))
    for c in range(NG):
        xn[c, pl.ds(r0, TB), :] = y[:, c * 128:(c + 1) * 128].astype(BF16)


def _qkv_stage(xn, wqkv, qs, ks, vts, r0, kt0):
    xp = _packed(xn)
    wp = _packed(wqkv)
    h0 = pl.multiple_of(r0 // 2, TB // 2)
    lhs = _as_bf16(jnp.concatenate(
        [xp[c, pl.ds(h0, TB // 2), :] for c in range(NG)], axis=1))
    for j in range(3 * NG):
        y = jnp.dot(lhs, _as_bf16(wp[j]), preferred_element_type=F32)
        if j < NG:
            qs[j, pl.ds(r0, TB), :] = (y * QSCALE).astype(BF16)
        elif j < 2 * NG:
            ks[j - NG, pl.ds(r0, TB), :] = y.astype(BF16)
        else:
            c = j - 2 * NG
            for t in range(TB // 128):
                vts[kt0 + t, c * 128:(c + 1) * 128, :] = (
                    y[t * 128:(t + 1) * 128, :].T.astype(BF16))


def _score_stage(qs, ks, xs, ms, sb, g, static_sb=None):
    lane = jax.lax.broadcasted_iota(I32, (QA, 128), 1)
    li = lane % QA
    row = jax.lax.broadcasted_iota(I32, (QA, 128), 0)
    m_lo = row > li
    m_hi = row <= li
    lg = jax.lax.broadcasted_iota(I32, (QA // 2, 128), 1) // QA
    qp = _packed(qs)
    kp = _packed(ks)
    for a in range(4):
        if static_sb is None:
            qa2 = pl.multiple_of(sb * (SB // 2) + (QA // 2) * a, QA // 2)
            q = qp[g, pl.ds(qa2, QA // 2), :]
            first = 0
            k = kp[g, pl.ds(qa2 - WIN // 2, XR // 2), :]
        else:
            qa = static_sb * SB + QA * a
            q = qp[g, qa // 2:(qa + QA) // 2, :]
            first = WIN - qa
            k = kp[g, 0:(XR - first) // 2, :]
        qbd = jnp.concatenate(
            [jnp.where(lg == ((a - p) % 4), q, jnp.zeros_like(q)) for p in range(4)],
            axis=0)
        x = jax.lax.dot_general(_as_bf16(k), _as_bf16(qbd), NT_DIMS,
                                preferred_element_type=F32)
        n = XR - first
        hi = jnp.where(m_hi, x[n - QA:n], NEG)
        if first == 0:
            lo = jnp.where(m_lo, x[0:QA], NEG)
            x = jnp.concatenate([lo, x[QA:n - QA], hi], axis=0)
        elif n > QA:
            x = jnp.concatenate(
                [jnp.full((first, 128), NEG, F32), x[0:n - QA], hi], axis=0)
        else:
            x = jnp.concatenate([jnp.full((first, 128), NEG, F32), hi], axis=0)
        xs[g, a] = x
        j0 = first // 16
        m0 = x[16 * j0:16 * j0 + 8]
        m1 = x[16 * j0 + 8:16 * j0 + 16]
        for j in range(j0 + 1, XR // 16):
            m0 = jnp.maximum(m0, x[16 * j:16 * j + 8])
            m1 = jnp.maximum(m1, x[16 * j + 8:16 * j + 16])
        mm = jnp.max(jnp.maximum(m0, m1), axis=0, keepdims=True)
        ms[g, a] = jnp.broadcast_to(mm, (8, 128))


def _exp_stage(xs, ms, ps, ls, g, never):
    for a in range(4):
        m = ms[g, a]
        s0 = s1 = None
        for j in range(XR // 16):
            e0 = jnp.exp2(xs[g, a, 16 * j:16 * j + 8, :] - m)
            e1 = jnp.exp2(xs[g, a, 16 * j + 8:16 * j + 16, :] - m)
            s0 = e0 if s0 is None else s0 + e0
            s1 = e1 if s1 is None else s1 + e1
            if j == XR // 16 - 1:
                s = s0 + s1
                e1 = jnp.where(never, s, e1)
            ps[g, a, 16 * j:16 * j + 16, :] = (
                jnp.concatenate([e0, e1], axis=0).astype(BF16))
        ls[g, a] = s


def _pv_stage(ps, ls, vts, os_, sb, g):
    lg8 = jax.lax.broadcasted_iota(I32, (8, 128), 1) // QA
    odd = (lg8 % 2) == 1
    hi2 = lg8 >= 2
    zero = jnp.zeros((8, 128), U32)
    pp = _packed(ps)
    vp = _packed(vts)

    def sel(c, x, y):
        if x is None and y is None:
            return None
        return jnp.where(c, zero if x is None else x, zero if y is None else y)

    acc = [None] * 4
    for kt in range(3):
        yrows = [[] for _ in range(4)]
        for r in range(8 * kt, 8 * kt + 8):
            pr = []
            for a in range(4):
                j = r - 2 * a
                pr.append(pp[g, a, 8 * j:8 * j + 8, :] if 0 <= j < XR // 16 else None)
            z = [sel(odd, pr[(a + 1) % 4], pr[a]) for a in range(4)]
            for h in range(4):
                y = sel(hi2, z[(h + 2) % 4], z[h])
                yrows[h].append(zero if y is None else y)
        for h in range(4):
            y = _as_bf16(jnp.concatenate(yrows[h], axis=0))
            r0 = (g * 128 + DH * h) // 2
            vt = _as_bf16(vp[sb + kt, r0:r0 + DH // 2, :])
            ot = jnp.dot(vt, y, preferred_element_type=F32)
            acc[h] = ot if acc[h] is None else acc[h] + ot
    l = [jnp.sum(ls[g, a], axis=0, keepdims=True) for a in range(4)]
    lg1 = jax.lax.broadcasted_iota(I32, (1, 128), 1) // QA
    lz = [jnp.where((lg1 % 2) == 1, l[(a + 1) % 4], l[a]) for a in range(4)]
    ly = [jnp.where(lg1 >= 2, lz[(h + 2) % 4], lz[h]) for h in range(4)]
    t = jnp.concatenate([acc[h] * (1.0 / ly[h]) for h in range(4)], axis=0).T
    lgrp = jax.lax.broadcasted_iota(I32, (QA, 128), 1) // QA
    outs = []
    for a in range(4):
        r = t[QA * ((a - 3) % 4):QA * ((a - 3) % 4) + QA]
        for h in (2, 1, 0):
            p = (a - h) % 4
            r = jnp.where(lgrp == h, t[QA * p:QA * p + QA], r)
        outs.append(r)
    os_[g] = jnp.concatenate(outs, axis=0).astype(BF16)


def _proj_stage(os_, wo, wr, xres, xn, best_v, best_i, sb):
    op = _packed(os_)
    wp = _packed(wo)
    r0 = pl.multiple_of(sb * SB, SB)
    lhs = _as_bf16(jnp.concatenate([op[g] for g in range(NG)], axis=1))
    acc = jnp.concatenate(
        [jnp.dot(lhs, _as_bf16(wp[j]), preferred_element_type=F32) for j in range(NG)],
        axis=1)
    x = xres[pl.ds(r0, SB), :].astype(F32) + acc
    y = _layernorm(x)
    r = jnp.sum(y * wr[...], axis=1, keepdims=True)
    xres[pl.ds(r0, SB), :] = (x + y).astype(BF16)
    for c in range(NG):
        xn[c, pl.ds(r0, SB), :] = y[:, c * 128:(c + 1) * 128].astype(BF16)
    bv = best_v[...]
    bi = best_i[...]
    sub = jax.lax.broadcasted_iota(I32, (8, 1), 0)
    for rg in range(SB // 8):
        rr = r[8 * rg:8 * rg + 8]
        take = rr > bv
        bv = jnp.where(take, rr, bv)
        bi = jnp.where(take, sub + (r0 + 8 * rg), bi)
    best_v[...] = bv
    best_i[...] = bi


def _router_ffn(xn, wg, wu, wd, best_v, best_i):
    bv = best_v[...]
    bi = best_i[...]
    rmax = jnp.max(bv)
    idx = jnp.min(jnp.where(bv == rmax, bi, S))
    grp = idx >> 4
    xp = _packed(xn)
    h0 = pl.multiple_of(grp * 8, 8)
    lhs = _as_bf16(jnp.concatenate(
        [xp[c, pl.ds(h0, 8), :] for c in range(NG)], axis=1))
    hg = jnp.dot(lhs, wg[...], preferred_element_type=F32)
    hu = jnp.dot(lhs, wu[...], preferred_element_type=F32)
    act = (hg * jax.nn.sigmoid(hg) * hu).astype(BF16)
    y = jnp.dot(act, wd[...], preferred_element_type=F32)
    gate = jax.nn.sigmoid(jnp.full((1, 1), rmax, F32))
    row = jax.lax.broadcasted_iota(I32, (16, D), 0)
    upd = jnp.where(row == (idx & 15), y * gate, 0.0)
    return pl.multiple_of(grp * 16, 16), upd


def _kernel(flag, x_hbm, wqkv_hbm, wo_hbm, wr_ref, wg_hbm, wu_hbm, wd_hbm, out_hbm,
            xres, xn, qs, ks, vts, xs, ms, ps, ls, os_, wqkv, wo, wr, wg, wu, wd,
            best_v, best_i, sem_x, sem_w, sem_o):
    x_cp = [pltpu.make_async_copy(x_hbm.at[0, pl.ds(t * TB, TB), :],
                                  xres.at[pl.ds(t * TB, TB), :], sem_x.at[t])
            for t in range(NTB)]
    wqkv_cp = [pltpu.make_async_copy(wqkv_hbm.at[:, pl.ds(j * 128, 128)],
                                     wqkv.at[j], sem_w.at[0])
               for j in range(3 * NG)]
    wo_cp = [pltpu.make_async_copy(wo_hbm.at[:, pl.ds(j * 128, 128)],
                                   wo.at[j], sem_w.at[1])
             for j in range(NG)]
    ffn_cp = [pltpu.make_async_copy(src, dst, sem_w.at[2])
              for src, dst in ((wg_hbm, wg), (wu_hbm, wu), (wd_hbm, wd))]
    for cp in x_cp[:2] + wqkv_cp + x_cp[2:] + wo_cp + ffn_cp:
        cp.start()

    vts[0:2] = jnp.zeros((2,) + vts.shape[1:], BF16)
    xres[S:S + TB, :] = jnp.zeros((TB, D), BF16)
    wr[...] = wr_ref[...].astype(F32).reshape(1, D)
    for cp in x_cp:
        cp.wait()
    for cp in wqkv_cp:
        cp.wait()
    for cp in wo_cp:
        cp.wait()
    for cp in ffn_cp:
        cp.wait()

    def out_copy(r0, n, slot):
        return pltpu.make_async_copy(xres.at[pl.ds(r0, n), :],
                                     out_hbm.at[0, pl.ds(r0, n), :], sem_o.at[slot])

    def layer(l, carry):
        never = jnp.full((8, 128), flag[0], I32) != 0

        _ln_stage(xres, xn, 0)

        def p1_step(t, c):
            r0 = pl.multiple_of(t * TB, TB)
            _ln_stage(xres, xn, r0 + TB)
            _qkv_stage(xn, wqkv, qs, ks, vts, r0, 2 + t * (TB // 128))
            return c

        jax.lax.fori_loop(0, NTB, p1_step, 0)

        best_v[...] = jnp.full((8, 1), -jnp.inf, F32)
        best_i[...] = jnp.zeros((8, 1), I32)

        def pv_all(sb):
            for g in range(NG):
                _pv_stage(ps, ls, vts, os_, sb, g)

        def exp_all():
            for g in range(NG):
                _exp_stage(xs, ms, ps, ls, g, never)

        def proj(sb):
            _proj_stage(os_, wo, wr, xres, xn, best_v, best_i, sb)

        def emit_out(sb):
            @pl.when(l == N_LAYERS - 1)
            def _():
                out_copy(pl.multiple_of(sb * SB, SB), SB, sb).start()

        one = flag[0] + 1

        def pre0(_, c):
            for g in range(NG):
                _score_stage(qs, ks, xs, ms, None, g, static_sb=0)
            return c

        def pre1(_, c):
            exp_all()
            for g in range(NG):
                _score_stage(qs, ks, xs, ms, None, g, static_sb=1)
            return c

        def steady(s, c):
            pv_all(s - 1)
            exp_all()
            for g in range(2):
                _score_stage(qs, ks, xs, ms, s + 1, g)
            proj(s - 1)
            for g in range(2, NG):
                _score_stage(qs, ks, xs, ms, s + 1, g)
            emit_out(s - 1)
            return c

        def post0(_, c):
            pv_all(NSB - 2)
            exp_all()
            proj(NSB - 2)
            emit_out(NSB - 2)
            return c

        def post1(_, c):
            pv_all(NSB - 1)
            proj(NSB - 1)
            emit_out(NSB - 1)
            return c

        jax.lax.fori_loop(0, one, pre0, 0)
        jax.lax.fori_loop(0, one, pre1, 0)
        jax.lax.fori_loop(1, NSB - 1, steady, 0)
        jax.lax.fori_loop(0, one, post0, 0)
        jax.lax.fori_loop(0, one, post1, 0)

        g0, upd = _router_ffn(xn, wg, wu, wd, best_v, best_i)

        @pl.when(l == N_LAYERS - 1)
        def _():
            for sb in range(NSB):
                out_copy(sb * SB, SB, sb).wait()

        xres[pl.ds(g0, 16), :] = (
            xres[pl.ds(g0, 16), :].astype(F32) + upd).astype(BF16)

        @pl.when(l == N_LAYERS - 1)
        def _():
            cp = out_copy(g0, 16, NSB)
            cp.start()
            cp.wait()

        return carry

    jax.lax.fori_loop(0, N_LAYERS, layer, 0)


@jax.jit
def pallas_interleave_layers__sliding_block__moe_arch_mod__prompt_kernel(
    A_x: jax.Array,
    A_wqkv: jax.Array,
    A_wo: jax.Array,
    B_x: jax.Array,
    B_w_r: jax.Array,
    B_w_gate: jax.Array,
    B_w_up: jax.Array,
    B_w_down: jax.Array,
):
    del B_x
    any_spec = pl.BlockSpec(memory_space=pl.ANY)
    scratch = [
        pltpu.VMEM((S + TB, D), BF16),
        pltpu.VMEM((NG, S + TB, 128), BF16),
        pltpu.VMEM((NG, S, 128), BF16),
        pltpu.VMEM((NG, S, 128), BF16),
        pltpu.VMEM((NSB + 2, D, 128), BF16),
        pltpu.VMEM((NG, 4, XR, 128), F32),
        pltpu.VMEM((NG, 4, 8, 128), F32),
        pltpu.VMEM((NG, 4, XR, 128), BF16),
        pltpu.VMEM((NG, 4, 8, 128), F32),
        pltpu.VMEM((NG, SB, 128), BF16),
        pltpu.VMEM((3 * NG, D, 128), BF16),
        pltpu.VMEM((NG, D, 128), BF16),
        pltpu.VMEM((1, D), F32),
        pltpu.VMEM((D, FF), BF16),
        pltpu.VMEM((D, FF), BF16),
        pltpu.VMEM((FF, D), BF16),
        pltpu.VMEM((8, 1), F32),
        pltpu.VMEM((8, 1), I32),
        pltpu.SemaphoreType.DMA((NTB,)),
        pltpu.SemaphoreType.DMA((3,)),
        pltpu.SemaphoreType.DMA((NSB + 1,)),
    ]
    flag = jnp.zeros((1,), I32)
    return pl.pallas_call(
        _kernel,
        out_shape=jax.ShapeDtypeStruct((1, S, D), BF16),
        in_specs=[pl.BlockSpec(memory_space=pltpu.SMEM),
                  any_spec, any_spec, any_spec,
                  pl.BlockSpec(memory_space=pltpu.VMEM),
                  any_spec, any_spec, any_spec],
        out_specs=any_spec,
        scratch_shapes=scratch,
        compiler_params=pltpu.CompilerParams(vmem_limit_bytes=112 * 1024 * 1024),
        name="swa_moe",
    )(flag, A_x, A_wqkv, A_wo, B_w_r, B_w_gate, B_w_up, B_w_down)
```

```python
import math

import jax
import jax.numpy as jnp
import jax.experimental.pallas as pl
import jax.experimental.pallas.tpu as pltpu

F32 = jnp.float32
BF16 = jnp.bfloat16
U32 = jnp.uint32
I32 = jnp.int32

S = 2048
D = 1024
DH = 32
WIN = 256
FF = 3584
NG = 8
SB = 128
NSB = S // SB
QA = 32
XR = WIN + QA
TB = 256
NTB = S // TB
EPS = 1e-5
NEG = -1e30
QSCALE = (DH ** -0.5) * math.log2(math.e)
NT_DIMS = (((1,), (1,)), ((), ()))
N_LAYERS = 2
W_GROUP = 4


def _scope(name):
    return jax.named_scope(name)


def _layernorm(x):
    mean = jnp.sum(x, axis=1, keepdims=True) * (1.0 / D)
    xc = x - mean
    var = jnp.sum(xc * xc, axis=1, keepdims=True) * (1.0 / D)
    return xc * jax.lax.rsqrt(var + EPS)


def _packed(ref):
    return ref.bitcast(U32)


def _as_bf16(v):
    return pltpu.bitcast(v, BF16)


def _ln_stage(xres, xn, t):
    r0 = t * TB if isinstance(t, int) else pl.multiple_of(t * TB, TB)
    y = _layernorm(xres[pl.ds(r0, TB), :].astype(F32))
    for c in range(NG):
        xn[c, pl.ds(r0, TB), :] = y[:, c * 128:(c + 1) * 128].astype(BF16)


QKV_ORDER = list(range(2 * NG, 3 * NG)) + list(range(2 * NG))


def _qkv_stage(xn, wqkv, qs, ks, vts, t, before_chunk=None):
    xp = _packed(xn)
    wp = _packed(wqkv)
    if isinstance(t, int):
        r0, h0 = t * TB, t * (TB // 2)
    else:
        r0 = pl.multiple_of(t * TB, TB)
        h0 = pl.multiple_of(t * (TB // 2), TB // 2)
    kt0 = 2 + t * (TB // 128)
    lhs = _as_bf16(jnp.concatenate(
        [xp[c, pl.ds(h0, TB // 2), :] for c in range(NG)], axis=1))
    for n, j in enumerate(QKV_ORDER):
        if before_chunk is not None:
            before_chunk(n)
        y = jnp.dot(lhs, _as_bf16(wp[j]), preferred_element_type=F32)
        if j < NG:
            qs[j, pl.ds(r0, TB), :] = (y * QSCALE).astype(BF16)
        elif j < 2 * NG:
            ks[j - NG, pl.ds(r0, TB), :] = y.astype(BF16)
        else:
            c = j - 2 * NG
            for t in range(TB // 128):
                vts[kt0 + t, c * 128:(c + 1) * 128, :] = (
                    y[t * 128:(t + 1) * 128, :].T.astype(BF16))


def _score_stage(qs, ks, xs, ms, sb, g, static_sb=None):
    lane = jax.lax.broadcasted_iota(I32, (QA, 128), 1)
    li = lane % QA
    row = jax.lax.broadcasted_iota(I32, (QA, 128), 0)
    m_lo = row > li
    m_hi = row <= li
    lg = jax.lax.broadcasted_iota(I32, (QA // 2, 128), 1) // QA
    qp = _packed(qs)
    kp = _packed(ks)
    for a in range(4):
        if static_sb is None:
            qa2 = pl.multiple_of(sb * (SB // 2) + (QA // 2) * a, QA // 2)
            q = qp[g, pl.ds(qa2, QA // 2), :]
            first = 0
            k = kp[g, pl.ds(qa2 - WIN // 2, XR // 2), :]
        else:
            qa = static_sb * SB + QA * a
            q = qp[g, qa // 2:(qa + QA) // 2, :]
            first = WIN - qa
            k = kp[g, 0:(XR - first) // 2, :]
        qbd = jnp.concatenate(
            [jnp.where(lg == ((a - p) % 4), q, jnp.zeros_like(q)) for p in range(4)],
            axis=0)
        x = jax.lax.dot_general(_as_bf16(k), _as_bf16(qbd), NT_DIMS,
                                preferred_element_type=F32)
        n = XR - first
        hi = jnp.where(m_hi, x[n - QA:n], NEG)
        if first == 0:
            lo = jnp.where(m_lo, x[0:QA], NEG)
            x = jnp.concatenate([lo, x[QA:n - QA], hi], axis=0)
        elif n > QA:
            x = jnp.concatenate(
                [jnp.full((first, 128), NEG, F32), x[0:n - QA], hi], axis=0)
        else:
            x = jnp.concatenate([jnp.full((first, 128), NEG, F32), hi], axis=0)
        xs[g, a] = x
        j0 = first // 16
        m0 = x[16 * j0:16 * j0 + 8]
        m1 = x[16 * j0 + 8:16 * j0 + 16]
        for j in range(j0 + 1, XR // 16):
            m0 = jnp.maximum(m0, x[16 * j:16 * j + 8])
            m1 = jnp.maximum(m1, x[16 * j + 8:16 * j + 16])
        mm = jnp.max(jnp.maximum(m0, m1), axis=0, keepdims=True)
        ms[g, a] = jnp.broadcast_to(mm, (8, 128))


def _exp_stage(xs, ms, ps, ls, g, never):
    for a in range(4):
        m = ms[g, a]
        s0 = s1 = None
        for j in range(XR // 16):
            e0 = jnp.exp2(xs[g, a, pl.ds(16 * j, 8, stride=2), :] - m)
            e1 = jnp.exp2(xs[g, a, pl.ds(16 * j + 1, 8, stride=2), :] - m)
            s0 = e0 if s0 is None else s0 + e0
            s1 = e1 if s1 is None else s1 + e1
            if j == XR // 16 - 1:
                s = s0 + s1
                e1 = jnp.where(never, s, e1)
            ps[g, a, 8 * j:8 * j + 8, :] = pltpu.pack_elementwise(
                [e0, e1], packed_dtype=BF16).astype(U32)
        ls[g, a] = s


def _pv_stage(ps, ls, vts, os_, sb, g):
    lg8 = jax.lax.broadcasted_iota(I32, (8, 128), 1) // QA
    odd = (lg8 % 2) == 1
    hi2 = lg8 >= 2
    zero = jnp.zeros((8, 128), U32)
    pp = ps
    vp = _packed(vts)

    def sel(c, x, y):
        if x is None and y is None:
            return None
        return jnp.where(c, zero if x is None else x, zero if y is None else y)

    acc = [None] * 4
    for kt in range(3):
        yrows = [[] for _ in range(4)]
        for r in range(8 * kt, 8 * kt + 8):
            pr = []
            for a in range(4):
                j = r - 2 * a
                pr.append(pp[g, a, 8 * j:8 * j + 8, :] if 0 <= j < XR // 16 else None)
            z = [sel(odd, pr[(a + 1) % 4], pr[a]) for a in range(4)]
            for h in range(4):
                y = sel(hi2, z[(h + 2) % 4], z[h])
                yrows[h].append(zero if y is None else y)
        for h in range(4):
            y = _as_bf16(jnp.concatenate(yrows[h], axis=0))
            r0 = (g * 128 + DH * h) // 2
            vt = _as_bf16(vp[sb + kt, r0:r0 + DH // 2, :])
            ot = jnp.dot(vt, y, preferred_element_type=F32)
            acc[h] = ot if acc[h] is None else acc[h] + ot
    l = [jnp.sum(ls[g, a], axis=0, keepdims=True) for a in range(4)]
    lg1 = jax.lax.broadcasted_iota(I32, (1, 128), 1) // QA
    lz = [jnp.where((lg1 % 2) == 1, l[(a + 1) % 4], l[a]) for a in range(4)]
    ly = [jnp.where(lg1 >= 2, lz[(h + 2) % 4], lz[h]) for h in range(4)]
    t = jnp.concatenate([acc[h] * (1.0 / ly[h]) for h in range(4)], axis=0).T
    lgrp = jax.lax.broadcasted_iota(I32, (QA, 128), 1) // QA
    outs = []
    for a in range(4):
        r = t[QA * ((a - 3) % 4):QA * ((a - 3) % 4) + QA]
        for h in (2, 1, 0):
            p = (a - h) % 4
            r = jnp.where(lgrp == h, t[QA * p:QA * p + QA], r)
        outs.append(r)
    os_[g] = jnp.concatenate(outs, axis=0).astype(BF16)


def _proj_stage(os_, wo, wr, xres, xn, best_v, best_i, sb, pins=None, never=None):
    op = _packed(os_)
    wp = _packed(wo)
    r0 = pl.multiple_of(sb * SB, SB)
    lhs = jnp.concatenate([op[g] for g in range(NG)], axis=1)
    cols = []
    for j in range(NG):
        lj = lhs
        if pins is not None and pins[j]:
            v = pins[j][0]
            for w in pins[j][1:]:
                v = v | w
            head = jnp.where(never, v, lhs[0:8, 0:128])
            top = jnp.concatenate([head, lhs[0:8, 128:]], axis=1)
            lj = jnp.concatenate([top, lhs[8:]], axis=0)
        cols.append(jnp.dot(_as_bf16(lj), _as_bf16(wp[j]), preferred_element_type=F32))
    acc = jnp.concatenate(cols, axis=1)
    x = xres[pl.ds(r0, SB), :].astype(F32) + acc
    y = _layernorm(x)
    r = jnp.sum(y * wr[...], axis=1, keepdims=True)
    xres[pl.ds(r0, SB), :] = (x + y).astype(BF16)
    for c in range(NG):
        xn[c, pl.ds(r0, SB), :] = y[:, c * 128:(c + 1) * 128].astype(BF16)
    bv = best_v[...]
    bi = best_i[...]
    sub = jax.lax.broadcasted_iota(I32, (8, 1), 0)
    for rg in range(SB // 8):
        rr = r[8 * rg:8 * rg + 8]
        take = rr > bv
        bv = jnp.where(take, rr, bv)
        bi = jnp.where(take, sub + (r0 + 8 * rg), bi)
    best_v[...] = bv
    best_i[...] = bi


def _router_ffn(xn, wg, wu, wd, best_v, best_i):
    bv = best_v[...]
    bi = best_i[...]
    rmax = jnp.max(bv)
    idx = jnp.min(jnp.where(bv == rmax, bi, S))
    grp = idx >> 4
    xp = _packed(xn)
    h0 = pl.multiple_of(grp * 8, 8)
    lhs = _as_bf16(jnp.concatenate(
        [xp[c, pl.ds(h0, 8), :] for c in range(NG)], axis=1))
    hg = jnp.dot(lhs, wg[...], preferred_element_type=F32)
    hu = jnp.dot(lhs, wu[...], preferred_element_type=F32)
    act = (hg * jax.nn.sigmoid(hg) * hu).astype(BF16)
    y = jnp.dot(act, wd[...], preferred_element_type=F32)
    gate = jax.nn.sigmoid(jnp.full((1, 1), rmax, F32))
    row = jax.lax.broadcasted_iota(I32, (16, D), 0)
    upd = jnp.where(row == (idx & 15), y * gate, 0.0)
    return pl.multiple_of(grp * 16, 16), upd


def _kernel(flag, x_hbm, wqkv_hbm, wo_hbm, wr_ref, wg_hbm, wu_hbm, wd_hbm, out_hbm,
            xres, xn, qs, ks, vts, xs, ms, ps, ls, os_, wqkv, wo, wr, wg, wu, wd,
            best_v, best_i, sem_x, sem_q, sem_w, sem_o):
    x_cp = [pltpu.make_async_copy(x_hbm.at[0, pl.ds(t * TB, TB), :],
                                  xres.at[pl.ds(t * TB, TB), :], sem_x.at[t])
            for t in range(NTB)]
    wqkv_cp = [pltpu.make_async_copy(wqkv_hbm.at[:, pl.ds(j * 128, 128)],
                                     wqkv.at[j], sem_q.at[n // W_GROUP])
               for n, j in enumerate(QKV_ORDER)]
    wo_cp = [pltpu.make_async_copy(wo_hbm.at[:, pl.ds(j * 128, 128)],
                                   wo.at[j], sem_w.at[0])
             for j in range(NG)]
    ffn_cp = [pltpu.make_async_copy(src, dst, sem_w.at[1])
              for src, dst in ((wg_hbm, wg), (wu_hbm, wu), (wd_hbm, wd))]
    for cp in x_cp[:2] + wqkv_cp:
        cp.start()

    vts[0:2] = jnp.zeros((2,) + vts.shape[1:], BF16)
    xres[S:S + TB, :] = jnp.zeros((TB, D), BF16)
    wr[...] = wr_ref[...].astype(F32).reshape(1, D)
    x_cp[0].wait()

    def out_copy(r0, n, slot):
        return pltpu.make_async_copy(xres.at[pl.ds(r0, n), :],
                                     out_hbm.at[0, pl.ds(r0, n), :], sem_o.at[slot])

    def layer(l, carry):
        never = jnp.full((8, 128), flag[0], I32) != 0

        with _scope('ln0'):
            _ln_stage(xres, xn, 0)

        @pl.when(l == 0)
        def _():
            def wait_group(n):
                if n % W_GROUP == 0:
                    for cp in wqkv_cp[n:n + W_GROUP]:
                        cp.wait()
                if n == 3 * NG - 2 * W_GROUP:
                    for cp in x_cp[2:]:
                        cp.start()

            with _scope('p1_first'):
                x_cp[1].wait()
                _qkv_stage(xn, wqkv, qs, ks, vts, 0, wait_group)
                _ln_stage(xres, xn, 1)
            for cp in wo_cp + ffn_cp:
                cp.start()

        def p1_step(t, c):
            @pl.when(jnp.logical_and(l == 0, t + 1 < NTB))
            def _():
                tn = jnp.minimum(t + 1, NTB - 1)
                pltpu.make_async_copy(
                    x_hbm.at[0, pl.ds(tn * TB, TB), :],
                    xres.at[pl.ds(tn * TB, TB), :], sem_x.at[tn]).wait()

            _qkv_stage(xn, wqkv, qs, ks, vts, t)
            _ln_stage(xres, xn, t + 1)
            return c

        with _scope('p1_loop'):
            jax.lax.fori_loop(jnp.where(l == 0, 1, 0), NTB, p1_step, 0)

        @pl.when(l == 0)
        def _():
            for cp in wo_cp:
                cp.wait()

        best_v[...] = jnp.full((8, 1), -jnp.inf, F32)
        best_i[...] = jnp.zeros((8, 1), I32)

        def pv_all(sb):
            for g in range(NG):
                _pv_stage(ps, ls, vts, os_, sb, g)

        def exp_all():
            for g in range(NG):
                _exp_stage(xs, ms, ps, ls, g, never)

        def proj(sb, pinned=()):
            pp = ps
            pins = [[pp[g, a, XR // 2 - 8:XR // 2, :] for a in range(4)]
                    if g in pinned else [] for g in range(NG)]
            _proj_stage(os_, wo, wr, xres, xn, best_v, best_i, sb, pins, never)

        def emit_out(sb):
            @pl.when(l == N_LAYERS - 1)
            def _():
                out_copy(pl.multiple_of(sb * SB, SB), SB, sb).start()

        one = flag[0] + 1

        def pre0(_, c):
            for g in range(NG):
                _score_stage(qs, ks, xs, ms, None, g, static_sb=0)
            return c

        def pre1(_, c):
            exp_all()
            for g in range(NG):
                _score_stage(qs, ks, xs, ms, None, g, static_sb=1)
            return c

        def steady(s, c):
            pv_all(s - 1)
            exp_all()
            for g in range(2):
                _score_stage(qs, ks, xs, ms, s + 1, g)
            proj(s - 1)
            for g in range(2, NG):
                _score_stage(qs, ks, xs, ms, s + 1, g)
            emit_out(s - 1)
            return c

        def post0(_, c):
            pv_all(NSB - 2)
            exp_all()
            proj(NSB - 2)
            emit_out(NSB - 2)
            return c

        def post1(_, c):
            pv_all(NSB - 1)
            proj(NSB - 1)
            emit_out(NSB - 1)
            return c

        with _scope('pre'):
            jax.lax.fori_loop(0, one, pre0, 0)
            jax.lax.fori_loop(0, one, pre1, 0)
        with _scope('steady'):
            jax.lax.fori_loop(1, NSB - 1, steady, 0)
        with _scope('post'):
            jax.lax.fori_loop(0, one, post0, 0)
            jax.lax.fori_loop(0, one, post1, 0)

        @pl.when(l == 0)
        def _():
            for cp in ffn_cp:
                cp.wait()

        with _scope('ffn'):
            g0, upd = _router_ffn(xn, wg, wu, wd, best_v, best_i)

        @pl.when(l == N_LAYERS - 1)
        def _():
            for sb in range(NSB):
                out_copy(sb * SB, SB, sb).wait()

        xres[pl.ds(g0, 16), :] = (
            xres[pl.ds(g0, 16), :].astype(F32) + upd).astype(BF16)

        @pl.when(l == N_LAYERS - 1)
        def _():
            cp = out_copy(g0, 16, NSB)
            cp.start()
            cp.wait()

        return carry

    jax.lax.fori_loop(0, N_LAYERS, layer, 0)


@jax.jit
def pallas_interleave_layers__sliding_block__moe_arch_mod__prompt_kernel(
    A_x: jax.Array,
    A_wqkv: jax.Array,
    A_wo: jax.Array,
    B_x: jax.Array,
    B_w_r: jax.Array,
    B_w_gate: jax.Array,
    B_w_up: jax.Array,
    B_w_down: jax.Array,
):
    del B_x
    any_spec = pl.BlockSpec(memory_space=pl.ANY)
    scratch = [
        pltpu.VMEM((S + TB, D), BF16),
        pltpu.VMEM((NG, S + TB, 128), BF16),
        pltpu.VMEM((NG, S, 128), BF16),
        pltpu.VMEM((NG, S, 128), BF16),
        pltpu.VMEM((NSB + 2, D, 128), BF16),
        pltpu.VMEM((NG, 4, XR, 128), F32),
        pltpu.VMEM((NG, 4, 8, 128), F32),
        pltpu.VMEM((NG, 4, XR // 2, 128), U32),
        pltpu.VMEM((NG, 4, 8, 128), F32),
        pltpu.VMEM((NG, SB, 128), BF16),
        pltpu.VMEM((3 * NG, D, 128), BF16),
        pltpu.VMEM((NG, D, 128), BF16),
        pltpu.VMEM((1, D), F32),
        pltpu.VMEM((D, FF), BF16),
        pltpu.VMEM((D, FF), BF16),
        pltpu.VMEM((FF, D), BF16),
        pltpu.VMEM((8, 1), F32),
        pltpu.VMEM((8, 1), I32),
        pltpu.SemaphoreType.DMA((NTB,)),
        pltpu.SemaphoreType.DMA((3 * NG // W_GROUP,)),
        pltpu.SemaphoreType.DMA((2,)),
        pltpu.SemaphoreType.DMA((NSB + 1,)),
    ]
    flag = jnp.zeros((1,), I32)
    return pl.pallas_call(
        _kernel,
        out_shape=jax.ShapeDtypeStruct((1, S, D), BF16),
        in_specs=[pl.BlockSpec(memory_space=pltpu.SMEM),
                  any_spec, any_spec, any_spec,
                  pl.BlockSpec(memory_space=pltpu.VMEM),
                  any_spec, any_spec, any_spec],
        out_specs=any_spec,
        scratch_shapes=scratch,
        compiler_params=pltpu.CompilerParams(vmem_limit_bytes=112 * 1024 * 1024),
        name="swa_moe",
    )(flag, A_x, A_wqkv, A_wo, B_w_r, B_w_gate, B_w_up, B_w_down)
```

```python
import math

import jax
import jax.numpy as jnp
import jax.experimental.pallas as pl
import jax.experimental.pallas.tpu as pltpu

F32 = jnp.float32
BF16 = jnp.bfloat16
U32 = jnp.uint32
I32 = jnp.int32

S = 2048
D = 1024
DH = 32
WIN = 256
FF = 3584
NG = 8
SB = 128
NSB = S // SB
QA = 32
XR = WIN + QA
TB = 256
NTB = S // TB
EPS = 1e-5
NEG = -1e30
QSCALE = (DH ** -0.5) * math.log2(math.e)
NT_DIMS = (((1,), (1,)), ((), ()))
N_LAYERS = 2
W_GROUP = 4


def _scope(name):
    return jax.named_scope(name)


def _layernorm(x):
    mean = jnp.sum(x, axis=1, keepdims=True) * (1.0 / D)
    xc = x - mean
    var = jnp.sum(xc * xc, axis=1, keepdims=True) * (1.0 / D)
    return xc * jax.lax.rsqrt(var + EPS)


def _packed(ref):
    return ref.bitcast(U32)


def _as_bf16(v):
    return pltpu.bitcast(v, BF16)


def _ln_stage(xres, xn, t):
    r0 = t * TB if isinstance(t, int) else pl.multiple_of(t * TB, TB)
    y = _layernorm(xres[pl.ds(r0, TB), :].astype(F32))
    for c in range(NG):
        xn[c, pl.ds(r0, TB), :] = y[:, c * 128:(c + 1) * 128].astype(BF16)


QKV_ORDER = list(range(2 * NG, 3 * NG)) + list(range(2 * NG))


def _qkv_stage(xn, wqkv, qs, ks, vts, t, before_chunk=None):
    xp = _packed(xn)
    wp = _packed(wqkv)
    if isinstance(t, int):
        r0, h0 = t * TB, t * (TB // 2)
    else:
        r0 = pl.multiple_of(t * TB, TB)
        h0 = pl.multiple_of(t * (TB // 2), TB // 2)
    kt0 = 2 + t * (TB // 128)
    lhs = _as_bf16(jnp.concatenate(
        [xp[c, pl.ds(h0, TB // 2), :] for c in range(NG)], axis=1))
    for n, j in enumerate(QKV_ORDER):
        if before_chunk is not None:
            before_chunk(n)
        y = jnp.dot(lhs, _as_bf16(wp[j]), preferred_element_type=F32)
        if j < NG:
            qs[j, pl.ds(r0, TB), :] = (y * QSCALE).astype(BF16)
        elif j < 2 * NG:
            ks[j - NG, pl.ds(r0, TB), :] = y.astype(BF16)
        else:
            c = j - 2 * NG
            for t in range(TB // 128):
                vts[kt0 + t, c * 128:(c + 1) * 128, :] = (
                    y[t * 128:(t + 1) * 128, :].T.astype(BF16))


def _score_stage(qs, ks, xs, ms, sb, g, static_sb=None):
    lane = jax.lax.broadcasted_iota(I32, (QA, 128), 1)
    li = lane % QA
    row = jax.lax.broadcasted_iota(I32, (QA, 128), 0)
    m_lo = row > li
    m_hi = row <= li
    lg = jax.lax.broadcasted_iota(I32, (QA // 2, 128), 1) // QA
    qp = _packed(qs)
    kp = _packed(ks)
    for a in range(4):
        if static_sb is None:
            qa2 = pl.multiple_of(sb * (SB // 2) + (QA // 2) * a, QA // 2)
            q = qp[g, pl.ds(qa2, QA // 2), :]
            first = 0
            k = kp[g, pl.ds(qa2 - WIN // 2, XR // 2), :]
        else:
            qa = static_sb * SB + QA * a
            q = qp[g, qa // 2:(qa + QA) // 2, :]
            first = WIN - qa
            k = kp[g, 0:(XR - first) // 2, :]
        qbd = jnp.concatenate(
            [jnp.where(lg == ((a - p) % 4), q, jnp.zeros_like(q)) for p in range(4)],
            axis=0)
        x = jax.lax.dot_general(_as_bf16(k), _as_bf16(qbd), NT_DIMS,
                                preferred_element_type=F32)
        n = XR - first
        hi = jnp.where(m_hi, x[n - QA:n], NEG)
        if first == 0:
            lo = jnp.where(m_lo, x[0:QA], NEG)
            x = jnp.concatenate([lo, x[QA:n - QA], hi], axis=0)
        elif n > QA:
            x = jnp.concatenate(
                [jnp.full((first, 128), NEG, F32), x[0:n - QA], hi], axis=0)
        else:
            x = jnp.concatenate([jnp.full((first, 128), NEG, F32), hi], axis=0)
        xs[g, a] = x
        j0 = first // 16
        m0 = x[16 * j0:16 * j0 + 8]
        m1 = x[16 * j0 + 8:16 * j0 + 16]
        for j in range(j0 + 1, XR // 16):
            m0 = jnp.maximum(m0, x[16 * j:16 * j + 8])
            m1 = jnp.maximum(m1, x[16 * j + 8:16 * j + 16])
        mm = jnp.max(jnp.maximum(m0, m1), axis=0, keepdims=True)
        ms[g, a] = jnp.broadcast_to(mm, (8, 128))


def _exp_stage(xs, ms, ps, ls, g, never, after=None):
    for a in range(4):
        m = ms[g, a]
        if after is not None:
            m = jnp.where(never, after, m)
        s0 = s1 = None
        for j in range(XR // 16):
            e0 = jnp.exp2(xs[g, a, pl.ds(16 * j, 8, stride=2), :] - m)
            e1 = jnp.exp2(xs[g, a, pl.ds(16 * j + 1, 8, stride=2), :] - m)
            s0 = e0 if s0 is None else s0 + e0
            s1 = e1 if s1 is None else s1 + e1
            if j == XR // 16 - 1:
                s = s0 + s1
                e1 = jnp.where(never, s, e1)
            ps[g, a, 8 * j:8 * j + 8, :] = pltpu.pack_elementwise(
                [e0, e1], packed_dtype=BF16).astype(U32)
        ls[g, a] = s


def _pv_stage(ps, ls, vts, os_, sb, g):
    lg8 = jax.lax.broadcasted_iota(I32, (8, 128), 1) // QA
    odd = (lg8 % 2) == 1
    hi2 = lg8 >= 2
    zero = jnp.zeros((8, 128), U32)
    pp = ps
    vp = _packed(vts)

    def sel(c, x, y):
        if x is None and y is None:
            return None
        return jnp.where(c, zero if x is None else x, zero if y is None else y)

    acc = [None] * 4
    for kt in range(3):
        yrows = [[] for _ in range(4)]
        for r in range(8 * kt, 8 * kt + 8):
            pr = []
            for a in range(4):
                j = r - 2 * a
                pr.append(pp[g, a, 8 * j:8 * j + 8, :] if 0 <= j < XR // 16 else None)
            z = [sel(odd, pr[(a + 1) % 4], pr[a]) for a in range(4)]
            for h in range(4):
                y = sel(hi2, z[(h + 2) % 4], z[h])
                yrows[h].append(zero if y is None else y)
        for h in range(4):
            y = _as_bf16(jnp.concatenate(yrows[h], axis=0))
            r0 = (g * 128 + DH * h) // 2
            vt = _as_bf16(vp[sb + kt, r0:r0 + DH // 2, :])
            ot = jnp.dot(vt, y, preferred_element_type=F32)
            acc[h] = ot if acc[h] is None else acc[h] + ot
    l = [jnp.sum(ls[g, a], axis=0, keepdims=True) for a in range(4)]
    lg1 = jax.lax.broadcasted_iota(I32, (1, 128), 1) // QA
    lz = [jnp.where((lg1 % 2) == 1, l[(a + 1) % 4], l[a]) for a in range(4)]
    ly = [jnp.where(lg1 >= 2, lz[(h + 2) % 4], lz[h]) for h in range(4)]
    t = jnp.concatenate([acc[h] * (1.0 / ly[h]) for h in range(4)], axis=0).T
    lgrp = jax.lax.broadcasted_iota(I32, (QA, 128), 1) // QA
    outs = []
    for a in range(4):
        r = t[QA * ((a - 3) % 4):QA * ((a - 3) % 4) + QA]
        for h in (2, 1, 0):
            p = (a - h) % 4
            r = jnp.where(lgrp == h, t[QA * p:QA * p + QA], r)
        outs.append(r)
    os_[g] = jnp.concatenate(outs, axis=0).astype(BF16)


def _proj_stage(os_, wo, wr, xres, xn, best_v, best_i, sb, never,
                overlap=None, fence=None):
    op = _packed(os_)
    wp = _packed(wo)
    r0 = sb * SB if isinstance(sb, int) else pl.multiple_of(sb * SB, SB)
    lhs = jnp.concatenate([op[g] for g in range(NG)], axis=1)
    cols = []
    for j in range(NG):
        lj = lhs
        if overlap is not None and j == NG - 1:
            head = jnp.where(never, fence(), lhs[0:8, 0:128])
            top = jnp.concatenate([head, lhs[0:8, 128:]], axis=1)
            lj = jnp.concatenate([top, lhs[8:]], axis=0)
        y = jnp.dot(_as_bf16(lj), _as_bf16(wp[j]), preferred_element_type=F32)
        cols.append(y)
        if overlap is not None and j == 0:
            overlap(y[0:8])
    x = xres[pl.ds(r0, SB), :].astype(F32) + jnp.concatenate(cols, axis=1)
    mean = jnp.sum(x, axis=1, keepdims=True) * (1.0 / D)
    xc = x - mean
    var = jnp.sum(xc * xc, axis=1, keepdims=True) * (1.0 / D)
    rstd = jax.lax.rsqrt(var + EPS)
    y = x * rstd - mean * rstd
    r = jnp.sum(y * wr[...], axis=1, keepdims=True)
    xres[pl.ds(r0, SB), :] = (x + y).astype(BF16)
    for c in range(NG):
        xn[c, pl.ds(r0, SB), :] = y[:, c * 128:(c + 1) * 128].astype(BF16)
    bv = best_v[...]
    bi = best_i[...]
    sub = jax.lax.broadcasted_iota(I32, (8, 1), 0)
    for rg in range(SB // 8):
        rr = r[8 * rg:8 * rg + 8]
        take = rr > bv
        bv = jnp.where(take, rr, bv)
        bi = jnp.where(take, sub + (r0 + 8 * rg), bi)
    best_v[...] = bv
    best_i[...] = bi


def _router_ffn(xn, wg, wu, wd, best_v, best_i):
    bv = best_v[...]
    bi = best_i[...]
    rmax = jnp.max(bv, axis=0, keepdims=True)
    idx = jnp.min(jnp.where(bv == rmax, bi, S))
    grp = idx >> 4
    xp = _packed(xn)
    h0 = pl.multiple_of(grp * 8, 8)
    lhs = _as_bf16(jnp.concatenate(
        [xp[c, pl.ds(h0, 8), :] for c in range(NG)], axis=1))
    wgp, wup, wdp = _packed(wg), _packed(wu), _packed(wd)
    act = []
    for j in range(FF // 128):
        hg = jnp.dot(lhs, _as_bf16(wgp[j]), preferred_element_type=F32)
        hu = jnp.dot(lhs, _as_bf16(wup[j]), preferred_element_type=F32)
        act.append(hg * jax.nn.sigmoid(hg) * hu)
    act = jnp.concatenate(act, axis=1).astype(BF16)
    y = jnp.concatenate(
        [jnp.dot(act, _as_bf16(wdp[j]), preferred_element_type=F32) for j in range(NG)],
        axis=1)
    row = jax.lax.broadcasted_iota(I32, (16, D), 0)
    upd = jnp.where(row == (idx & 15), y * jax.nn.sigmoid(rmax), 0.0)
    return pl.multiple_of(grp * 16, 16), upd


def _kernel(flag, x_hbm, wqkv_hbm, wo_hbm, wr_ref, wg_hbm, wu_hbm, wd_hbm, out_hbm,
            xres, xn, qs, ks, vts, xs, ms, ps, ls, os_, wqkv, wo, wr, wg, wu, wd,
            best_v, best_i, sem_x, sem_q, sem_w, sem_o):
    x_cp = [pltpu.make_async_copy(x_hbm.at[0, pl.ds(t * TB, TB), :],
                                  xres.at[pl.ds(t * TB, TB), :], sem_x.at[t])
            for t in range(NTB)]
    wqkv_cp = [pltpu.make_async_copy(wqkv_hbm.at[:, pl.ds(j * 128, 128)],
                                     wqkv.at[j], sem_q.at[n // W_GROUP])
               for n, j in enumerate(QKV_ORDER)]
    wo_cp = [pltpu.make_async_copy(wo_hbm.at[:, pl.ds(j * 128, 128)],
                                   wo.at[j], sem_w.at[0])
             for j in range(NG)]
    ffn_cp = [pltpu.make_async_copy(src.at[:, pl.ds(j * 128, 128)], dst.at[j],
                                    sem_w.at[1])
              for src, dst in ((wg_hbm, wg), (wu_hbm, wu), (wd_hbm, wd))
              for j in range(dst.shape[0])]
    for cp in x_cp[:1] + wqkv_cp[:W_GROUP]:
        cp.start()

    with _scope('init'):
        vts[0:2] = jnp.zeros((2,) + vts.shape[1:], BF16)
        xres[S:S + TB, :] = jnp.zeros((TB, D), BF16)
        wr[...] = wr_ref[...].astype(F32).reshape(1, D)
    with _scope('xwait'):
        x_cp[0].wait()
    for cp in wqkv_cp[W_GROUP:2 * W_GROUP] + x_cp[1:2]:
        cp.start()

    def out_copy(r0, n, slot):
        return pltpu.make_async_copy(xres.at[pl.ds(r0, n), :],
                                     out_hbm.at[0, pl.ds(r0, n), :], sem_o.at[slot])

    def layer(l, carry):
        never = jnp.full((8, 128), flag[0], I32) != 0

        with _scope('ln0'):
            _ln_stage(xres, xn, 0)

        @pl.when(l == 0)
        def _():
            def wait_group(n):
                if n % W_GROUP == 0:
                    for cp in wqkv_cp[n:n + W_GROUP]:
                        cp.wait()
                    for cp in wqkv_cp[n + 2 * W_GROUP:n + 3 * W_GROUP]:
                        cp.start()
                if n == 2 * W_GROUP:
                    x_cp[1].wait()
                if n == 3 * NG - 2 * W_GROUP:
                    for cp in x_cp[2:]:
                        cp.start()

            with _scope('p1_first'):
                _qkv_stage(xn, wqkv, qs, ks, vts, 0, wait_group)
                _ln_stage(xres, xn, 1)
            for cp in wo_cp + ffn_cp:
                cp.start()

        def p1_step(t, c):
            @pl.when(jnp.logical_and(l == 0, t + 1 < NTB))
            def _():
                tn = jnp.minimum(t + 1, NTB - 1)
                pltpu.make_async_copy(
                    x_hbm.at[0, pl.ds(tn * TB, TB), :],
                    xres.at[pl.ds(tn * TB, TB), :], sem_x.at[tn]).wait()

            _qkv_stage(xn, wqkv, qs, ks, vts, t)
            _ln_stage(xres, xn, t + 1)
            return c

        with _scope('p1_loop'):
            jax.lax.fori_loop(jnp.where(l == 0, 1, 0), NTB, p1_step, 0)

        @pl.when(l == 0)
        def _():
            with _scope('wowait'):
                for cp in wo_cp:
                    cp.wait()

        best_v[...] = jnp.full((8, 1), -jnp.inf, F32)
        best_i[...] = jnp.zeros((8, 1), I32)

        def pv_all(sb):
            for g in range(NG):
                _pv_stage(ps, ls, vts, os_, sb, g)

        def exp_groups(gs, after=None):
            for g in gs:
                _exp_stage(xs, ms, ps, ls, g, never, after)

        def proj(sb, exp_gs=None):
            if exp_gs is None:
                _proj_stage(os_, wo, wr, xres, xn, best_v, best_i, sb, never)
            else:
                _proj_stage(os_, wo, wr, xres, xn, best_v, best_i, sb, never,
                            overlap=lambda v: exp_groups(exp_gs, v),
                            fence=lambda: ps[flag[0], 0, 0:8, :])

        def emit_out(sb):
            @pl.when(l == N_LAYERS - 1)
            def _():
                out_copy(pl.multiple_of(sb * SB, SB), SB, sb).start()

        one = flag[0] + 1

        def pre0(_, c):
            for g in range(NG):
                _score_stage(qs, ks, xs, ms, None, g, static_sb=0)
            return c

        def pre1(_, c):
            exp_groups(range(NG))
            for g in range(NG):
                _score_stage(qs, ks, xs, ms, None, g, static_sb=1)
            return c

        def steady(s, c):
            pv_all(s - 1)
            exp_groups([0])
            _score_stage(qs, ks, xs, ms, s + 1, 0)
            proj(s - 1, range(1, NG))
            for g in range(1, NG):
                _score_stage(qs, ks, xs, ms, s + 1, g)
            emit_out(s - 1)
            return c

        def post0(_, c):
            pv_all(NSB - 2)
            proj(NSB - 2, range(NG))
            emit_out(NSB - 2)
            return c

        def post1(_, c):
            pv_all(NSB - 1)
            proj(NSB - 1)
            emit_out(NSB - 1)
            return c

        with _scope('pre'):
            jax.lax.fori_loop(0, one, pre0, 0)
            jax.lax.fori_loop(0, one, pre1, 0)
        with _scope('steady'):
            jax.lax.fori_loop(1, NSB - 1, steady, 0)
        with _scope('post'):
            jax.lax.fori_loop(0, one, post0, 0)
            jax.lax.fori_loop(0, one, post1, 0)

        @pl.when(l == 0)
        def _():
            with _scope('ffnwait'):
                for cp in ffn_cp:
                    cp.wait()

        with _scope('ffn'):
            g0, upd = _router_ffn(xn, wg, wu, wd, best_v, best_i)

        @pl.when(l == N_LAYERS - 1)
        def _():
            with _scope('owait'):
                for sb in range(NSB):
                    out_copy(sb * SB, SB, sb).wait()

        xres[pl.ds(g0, 16), :] = (
            xres[pl.ds(g0, 16), :].astype(F32) + upd).astype(BF16)

        @pl.when(l == N_LAYERS - 1)
        def _():
            with _scope('ofinal'):
                cp = out_copy(g0, 16, NSB)
                cp.start()
                cp.wait()

        return carry

    jax.lax.fori_loop(0, N_LAYERS, layer, 0)


@jax.jit
def pallas_interleave_layers__sliding_block__moe_arch_mod__prompt_kernel(
    A_x: jax.Array,
    A_wqkv: jax.Array,
    A_wo: jax.Array,
    B_x: jax.Array,
    B_w_r: jax.Array,
    B_w_gate: jax.Array,
    B_w_up: jax.Array,
    B_w_down: jax.Array,
):
    del B_x
    any_spec = pl.BlockSpec(memory_space=pl.ANY)
    scratch = [
        pltpu.VMEM((S + TB, D), BF16),
        pltpu.VMEM((NG, S + TB, 128), BF16),
        pltpu.VMEM((NG, S, 128), BF16),
        pltpu.VMEM((NG, S, 128), BF16),
        pltpu.VMEM((NSB + 2, D, 128), BF16),
        pltpu.VMEM((NG, 4, XR, 128), F32),
        pltpu.VMEM((NG, 4, 8, 128), F32),
        pltpu.VMEM((NG, 4, XR // 2, 128), U32),
        pltpu.VMEM((NG, 4, 8, 128), F32),
        pltpu.VMEM((NG, SB, 128), BF16),
        pltpu.VMEM((3 * NG, D, 128), BF16),
        pltpu.VMEM((NG, D, 128), BF16),
        pltpu.VMEM((1, D), F32),
        pltpu.VMEM((FF // 128, D, 128), BF16),
        pltpu.VMEM((FF // 128, D, 128), BF16),
        pltpu.VMEM((NG, FF, 128), BF16),
        pltpu.VMEM((8, 1), F32),
        pltpu.VMEM((8, 1), I32),
        pltpu.SemaphoreType.DMA((NTB,)),
        pltpu.SemaphoreType.DMA((3 * NG // W_GROUP,)),
        pltpu.SemaphoreType.DMA((2,)),
        pltpu.SemaphoreType.DMA((NSB + 1,)),
    ]
    flag = jnp.zeros((1,), I32)
    return pl.pallas_call(
        _kernel,
        out_shape=jax.ShapeDtypeStruct((1, S, D), BF16),
        in_specs=[pl.BlockSpec(memory_space=pltpu.SMEM),
                  any_spec, any_spec, any_spec,
                  pl.BlockSpec(memory_space=pltpu.VMEM),
                  any_spec, any_spec, any_spec],
        out_specs=any_spec,
        scratch_shapes=scratch,
        compiler_params=pltpu.CompilerParams(vmem_limit_bytes=112 * 1024 * 1024),
        name="swa_moe",
    )(flag, A_x, A_wqkv, A_wo, B_w_r, B_w_gate, B_w_up, B_w_down)
```

```python
import math

import jax
import jax.numpy as jnp
import jax.experimental.pallas as pl
import jax.experimental.pallas.tpu as pltpu

F32 = jnp.float32
BF16 = jnp.bfloat16
U32 = jnp.uint32
I32 = jnp.int32

S = 2048
D = 1024
DH = 32
WIN = 256
FF = 3584
NG = 8
SB = 128
NSB = S // SB
QA = 32
XR = WIN + QA
TB = 256
NTB = S // TB
EPS = 1e-5
NEG = -1e30
QSCALE = (DH ** -0.5) * math.log2(math.e)
NT_DIMS = (((1,), (1,)), ((), ()))
N_LAYERS = 2
W_GROUP = 4


def _scope(name):
    return jax.named_scope(name)


def _layernorm(x):
    mean = jnp.sum(x, axis=1, keepdims=True) * (1.0 / D)
    xc = x - mean
    var = jnp.sum(xc * xc, axis=1, keepdims=True) * (1.0 / D)
    return xc * jax.lax.rsqrt(var + EPS)


def _packed(ref):
    return ref.bitcast(U32)


def _as_bf16(v):
    return pltpu.bitcast(v, BF16)


def _ln_stage(xres, xn, t):
    r0 = t * TB if isinstance(t, int) else pl.multiple_of(t * TB, TB)
    y = _layernorm(xres[pl.ds(r0, TB), :].astype(F32))
    for c in range(NG):
        xn[c, pl.ds(r0, TB), :] = y[:, c * 128:(c + 1) * 128].astype(BF16)


QKV_ORDER = list(range(2 * NG, 3 * NG)) + list(range(2 * NG))


def _qkv_stage(xn, wqkv, qs, ks, vts, t, before_chunk=None):
    xp = _packed(xn)
    wp = _packed(wqkv)
    if isinstance(t, int):
        r0, h0 = t * TB, t * (TB // 2)
    else:
        r0 = pl.multiple_of(t * TB, TB)
        h0 = pl.multiple_of(t * (TB // 2), TB // 2)
    kt0 = 2 + t * (TB // 128)
    lhs = _as_bf16(jnp.concatenate(
        [xp[c, pl.ds(h0, TB // 2), :] for c in range(NG)], axis=1))
    for n, j in enumerate(QKV_ORDER):
        if before_chunk is not None:
            before_chunk(n)
        y = jnp.dot(lhs, _as_bf16(wp[j]), preferred_element_type=F32)
        if j < NG:
            qs[j, pl.ds(r0, TB), :] = (y * QSCALE).astype(BF16)
        elif j < 2 * NG:
            ks[j - NG, pl.ds(r0, TB), :] = y.astype(BF16)
        else:
            c = j - 2 * NG
            for t in range(TB // 128):
                vts[kt0 + t, c * 128:(c + 1) * 128, :] = (
                    y[t * 128:(t + 1) * 128, :].T.astype(BF16))


def _score_stage(qs, ks, xs, ms, sb, g, static_sb=None):
    lane = jax.lax.broadcasted_iota(I32, (QA, 128), 1)
    li = lane % QA
    row = jax.lax.broadcasted_iota(I32, (QA, 128), 0)
    m_lo = row > li
    m_hi = row <= li
    lg = jax.lax.broadcasted_iota(I32, (QA // 2, 128), 1) // QA
    qp = _packed(qs)
    kp = _packed(ks)
    for a in range(4):
        if static_sb is None:
            qa2 = pl.multiple_of(sb * (SB // 2) + (QA // 2) * a, QA // 2)
            q = qp[g, pl.ds(qa2, QA // 2), :]
            first = 0
            k = kp[g, pl.ds(qa2 - WIN // 2, XR // 2), :]
        else:
            qa = static_sb * SB + QA * a
            q = qp[g, qa // 2:(qa + QA) // 2, :]
            first = WIN - qa
            k = kp[g, 0:(XR - first) // 2, :]
        qbd = jnp.concatenate(
            [jnp.where(lg == ((a - p) % 4), q, jnp.zeros_like(q)) for p in range(4)],
            axis=0)
        x = jax.lax.dot_general(_as_bf16(k), _as_bf16(qbd), NT_DIMS,
                                preferred_element_type=F32)
        n = XR - first
        hi = jnp.where(m_hi, x[n - QA:n], NEG)
        if first == 0:
            lo = jnp.where(m_lo, x[0:QA], NEG)
            x = jnp.concatenate([lo, x[QA:n - QA], hi], axis=0)
        elif n > QA:
            x = jnp.concatenate(
                [jnp.full((first, 128), NEG, F32), x[0:n - QA], hi], axis=0)
        else:
            x = jnp.concatenate([jnp.full((first, 128), NEG, F32), hi], axis=0)
        xs[g, a] = x
        j0 = first // 16
        m0 = x[16 * j0:16 * j0 + 8]
        m1 = x[16 * j0 + 8:16 * j0 + 16]
        for j in range(j0 + 1, XR // 16):
            m0 = jnp.maximum(m0, x[16 * j:16 * j + 8])
            m1 = jnp.maximum(m1, x[16 * j + 8:16 * j + 16])
        mm = jnp.max(jnp.maximum(m0, m1), axis=0, keepdims=True)
        ms[g, a] = jnp.broadcast_to(mm, (8, 128))
    return m0


def _exp_stage(xs, ms, ps, ls, g, never, after=None):
    for a in range(4):
        m = ms[g, a]
        if after is not None:
            m = jnp.where(never, after, m)
        s0 = s1 = None
        for j in range(XR // 16):
            e0 = jnp.exp2(xs[g, a, pl.ds(16 * j, 8, stride=2), :] - m)
            e1 = jnp.exp2(xs[g, a, pl.ds(16 * j + 1, 8, stride=2), :] - m)
            s0 = e0 if s0 is None else s0 + e0
            s1 = e1 if s1 is None else s1 + e1
            if j == XR // 16 - 1:
                s = s0 + s1
                e1 = jnp.where(never, s, e1)
            ps[g, a, 8 * j:8 * j + 8, :] = pltpu.pack_elementwise(
                [e0, e1], packed_dtype=BF16).astype(U32)
        ls[g, a] = s


def _pv_stage(ps, ls, vts, sb, g):
    lg8 = jax.lax.broadcasted_iota(I32, (8, 128), 1) // QA
    odd = (lg8 % 2) == 1
    hi2 = lg8 >= 2
    zero = jnp.zeros((8, 128), U32)
    pp = ps
    vp = _packed(vts)

    def sel(c, x, y):
        if x is None and y is None:
            return None
        return jnp.where(c, zero if x is None else x, zero if y is None else y)

    acc = [None] * 4
    for kt in range(3):
        yrows = [[] for _ in range(4)]
        for r in range(8 * kt, 8 * kt + 8):
            pr = []
            for a in range(4):
                j = r - 2 * a
                pr.append(pp[g, a, 8 * j:8 * j + 8, :] if 0 <= j < XR // 16 else None)
            z = [sel(odd, pr[(a + 1) % 4], pr[a]) for a in range(4)]
            for h in range(4):
                y = sel(hi2, z[(h + 2) % 4], z[h])
                yrows[h].append(zero if y is None else y)
        for h in range(4):
            y = _as_bf16(jnp.concatenate(yrows[h], axis=0))
            r0 = (g * 128 + DH * h) // 2
            vt = _as_bf16(vp[sb + kt, r0:r0 + DH // 2, :])
            ot = jnp.dot(vt, y, preferred_element_type=F32)
            acc[h] = ot if acc[h] is None else acc[h] + ot
    l = [jnp.sum(ls[g, a], axis=0, keepdims=True) for a in range(4)]
    lg1 = jax.lax.broadcasted_iota(I32, (1, 128), 1) // QA
    lz = [jnp.where((lg1 % 2) == 1, l[(a + 1) % 4], l[a]) for a in range(4)]
    ly = [jnp.where(lg1 >= 2, lz[(h + 2) % 4], lz[h]) for h in range(4)]
    return jnp.concatenate([acc[h] * (1.0 / ly[h]) for h in range(4)], axis=0)


def _unrotate_stage(ot, os_, g):
    t = ot.T
    lgrp = jax.lax.broadcasted_iota(I32, (QA, 128), 1) // QA
    odd = (lgrp % 2) == 1
    hi2 = lgrp >= 2
    tp = [t[QA * p:QA * p + QA] for p in range(4)]
    z = [jnp.where(odd, tp[(a - 1) % 4], tp[a]) for a in range(4)]
    outs = [jnp.where(hi2, z[(a - 2) % 4], z[a]) for a in range(4)]
    os_[g] = jnp.concatenate(outs, axis=0).astype(BF16)


def _proj_stage(os_, wo, wr, xres, xn, best_v, best_i, sb, never,
                overlap=None, fence=None):
    op = _packed(os_)
    wp = _packed(wo)
    r0 = sb * SB if isinstance(sb, int) else pl.multiple_of(sb * SB, SB)
    lhs = jnp.concatenate([op[g] for g in range(NG)], axis=1)
    cols = []
    for j in range(NG):
        lj = lhs
        if overlap is not None and j == NG - 1:
            head = jnp.where(never, fence(), lhs[0:8, 0:128])
            top = jnp.concatenate([head, lhs[0:8, 128:]], axis=1)
            lj = jnp.concatenate([top, lhs[8:]], axis=0)
        y = jnp.dot(_as_bf16(lj), _as_bf16(wp[j]), preferred_element_type=F32)
        cols.append(y)
        if overlap is not None and j == 0:
            overlap(y[0:8])
    x = xres[pl.ds(r0, SB), :].astype(F32) + jnp.concatenate(cols, axis=1)
    mean = jnp.sum(x, axis=1, keepdims=True) * (1.0 / D)
    xc = x - mean
    var = jnp.sum(xc * xc, axis=1, keepdims=True) * (1.0 / D)
    rstd = jax.lax.rsqrt(var + EPS)
    y = x * rstd - mean * rstd
    r = jnp.sum(y * wr[...], axis=1, keepdims=True)
    xres[pl.ds(r0, SB), :] = (x + y).astype(BF16)
    for c in range(NG):
        xn[c, pl.ds(r0, SB), :] = y[:, c * 128:(c + 1) * 128].astype(BF16)
    bv = best_v[...]
    bi = best_i[...]
    sub = jax.lax.broadcasted_iota(I32, (8, 1), 0)
    for rg in range(SB // 8):
        rr = r[8 * rg:8 * rg + 8]
        take = rr > bv
        bv = jnp.where(take, rr, bv)
        bi = jnp.where(take, sub + (r0 + 8 * rg), bi)
    best_v[...] = bv
    best_i[...] = bi


def _router_ffn(xn, wg, wu, wd, best_v, best_i):
    bv = best_v[...]
    bi = best_i[...]
    rmax = jnp.max(bv, axis=0, keepdims=True)
    idx = jnp.min(jnp.where(bv == rmax, bi, S))
    grp = idx >> 4
    xp = _packed(xn)
    h0 = pl.multiple_of(grp * 8, 8)
    lhs = _as_bf16(jnp.concatenate(
        [xp[c, pl.ds(h0, 8), :] for c in range(NG)], axis=1))
    wgp, wup, wdp = _packed(wg), _packed(wu), _packed(wd)
    act = []
    for j in range(FF // 128):
        hg = jnp.dot(lhs, _as_bf16(wgp[j]), preferred_element_type=F32)
        hu = jnp.dot(lhs, _as_bf16(wup[j]), preferred_element_type=F32)
        act.append(hg * jax.nn.sigmoid(hg) * hu)
    act = jnp.concatenate(act, axis=1).astype(BF16)
    y = jnp.concatenate(
        [jnp.dot(act, _as_bf16(wdp[j]), preferred_element_type=F32) for j in range(NG)],
        axis=1)
    row = jax.lax.broadcasted_iota(I32, (16, D), 0)
    upd = jnp.where(row == (idx & 15), y * jax.nn.sigmoid(rmax), 0.0)
    return pl.multiple_of(grp * 16, 16), upd


def _kernel(flag, x_hbm, wqkv_hbm, wo_hbm, wr_ref, wg_hbm, wu_hbm, wd_hbm, out_hbm,
            xres, xn, qs, ks, vts, xs, ms, ps, ls, os_, wqkv, wo, wr, wg, wu, wd,
            best_v, best_i, sem_x, sem_q, sem_w, sem_o):
    x_cp = [pltpu.make_async_copy(x_hbm.at[0, pl.ds(t * TB, TB), :],
                                  xres.at[pl.ds(t * TB, TB), :], sem_x.at[t])
            for t in range(NTB)]
    wqkv_cp = [pltpu.make_async_copy(wqkv_hbm.at[:, pl.ds(j * 128, 128)],
                                     wqkv.at[j], sem_q.at[n // W_GROUP])
               for n, j in enumerate(QKV_ORDER)]
    wo_cp = [pltpu.make_async_copy(wo_hbm.at[:, pl.ds(j * 128, 128)],
                                   wo.at[j], sem_w.at[0])
             for j in range(NG)]
    ffn_cp = [pltpu.make_async_copy(src.at[:, pl.ds(j * 128, 128)], dst.at[j],
                                    sem_w.at[1])
              for src, dst in ((wg_hbm, wg), (wu_hbm, wu), (wd_hbm, wd))
              for j in range(dst.shape[0])]
    for cp in x_cp[:1] + wqkv_cp[:W_GROUP]:
        cp.start()

    with _scope('init'):
        vts[0:2] = jnp.zeros((2,) + vts.shape[1:], BF16)
        xres[S:S + TB, :] = jnp.zeros((TB, D), BF16)
        wr[...] = wr_ref[...].astype(F32).reshape(1, D)
    with _scope('xwait'):
        x_cp[0].wait()
    for cp in wqkv_cp[W_GROUP:2 * W_GROUP] + x_cp[1:2]:
        cp.start()

    def out_copy(r0, n, slot):
        return pltpu.make_async_copy(xres.at[pl.ds(r0, n), :],
                                     out_hbm.at[0, pl.ds(r0, n), :], sem_o.at[slot])

    def layer(l, carry):
        never = jnp.full((8, 128), flag[0], I32) != 0

        with _scope('ln0'):
            _ln_stage(xres, xn, 0)

        @pl.when(l == 0)
        def _():
            def wait_group(n):
                if n % W_GROUP == 0:
                    for cp in wqkv_cp[n:n + W_GROUP]:
                        cp.wait()
                    for cp in wqkv_cp[n + 2 * W_GROUP:n + 3 * W_GROUP]:
                        cp.start()
                if n == 2 * W_GROUP:
                    x_cp[1].wait()
                if n == 3 * NG - 2 * W_GROUP:
                    for cp in x_cp[2:]:
                        cp.start()

            with _scope('p1_first'):
                _qkv_stage(xn, wqkv, qs, ks, vts, 0, wait_group)
                _ln_stage(xres, xn, 1)
            for cp in wo_cp + ffn_cp:
                cp.start()

        def p1_step(t, c):
            @pl.when(jnp.logical_and(l == 0, t + 1 < NTB))
            def _():
                tn = jnp.minimum(t + 1, NTB - 1)
                pltpu.make_async_copy(
                    x_hbm.at[0, pl.ds(tn * TB, TB), :],
                    xres.at[pl.ds(tn * TB, TB), :], sem_x.at[tn]).wait()

            _qkv_stage(xn, wqkv, qs, ks, vts, t)
            _ln_stage(xres, xn, t + 1)
            return c

        with _scope('p1_loop'):
            jax.lax.fori_loop(jnp.where(l == 0, 1, 0), NTB, p1_step, 0)

        @pl.when(l == 0)
        def _():
            with _scope('wowait'):
                for cp in wo_cp:
                    cp.wait()

        best_v[...] = jnp.full((8, 1), -jnp.inf, F32)
        best_i[...] = jnp.zeros((8, 1), I32)

        def pv_all(sb):
            for g in range(NG):
                _unrotate_stage(_pv_stage(ps, ls, vts, sb, g), os_, g)

        def exp_groups(gs, after=None):
            for g in gs:
                _exp_stage(xs, ms, ps, ls, g, never, after)

        def proj(sb, exp_gs=None):
            if exp_gs is None:
                _proj_stage(os_, wo, wr, xres, xn, best_v, best_i, sb, never)
            else:
                _proj_stage(os_, wo, wr, xres, xn, best_v, best_i, sb, never,
                            overlap=lambda v: exp_groups(exp_gs, v),
                            fence=lambda: ps[flag[0], 0, 0:8, :])

        def emit_out(sb):
            @pl.when(l == N_LAYERS - 1)
            def _():
                out_copy(pl.multiple_of(sb * SB, SB), SB, sb).start()

        one = flag[0] + 1

        def pre0(_, c):
            for g in range(NG):
                _score_stage(qs, ks, xs, ms, None, g, static_sb=0)
            return c

        def pre1(_, c):
            exp_groups(range(NG))
            for g in range(NG):
                _score_stage(qs, ks, xs, ms, None, g, static_sb=1)
            return c

        def steady(s, c):
            pv_all(s - 1)
            exp_groups([0])
            _score_stage(qs, ks, xs, ms, s + 1, 0)
            proj(s - 1, range(1, NG))
            for g in range(1, NG):
                _score_stage(qs, ks, xs, ms, s + 1, g)
            emit_out(s - 1)
            return c

        def post0(_, c):
            pv_all(NSB - 2)
            proj(NSB - 2, range(NG))
            emit_out(NSB - 2)
            return c

        def post1(_, c):
            pv_all(NSB - 1)
            proj(NSB - 1)
            emit_out(NSB - 1)
            return c

        with _scope('pre'):
            jax.lax.fori_loop(0, one, pre0, 0)
            jax.lax.fori_loop(0, one, pre1, 0)
        with _scope('steady'):
            jax.lax.fori_loop(1, NSB - 1, steady, 0)
        with _scope('post'):
            jax.lax.fori_loop(0, one, post0, 0)
            jax.lax.fori_loop(0, one, post1, 0)

        @pl.when(l == 0)
        def _():
            with _scope('ffnwait'):
                for cp in ffn_cp:
                    cp.wait()

        with _scope('ffn'):
            g0, upd = _router_ffn(xn, wg, wu, wd, best_v, best_i)

        @pl.when(l == N_LAYERS - 1)
        def _():
            with _scope('owait'):
                for sb in range(NSB):
                    out_copy(sb * SB, SB, sb).wait()

        xres[pl.ds(g0, 16), :] = (
            xres[pl.ds(g0, 16), :].astype(F32) + upd).astype(BF16)

        @pl.when(l == N_LAYERS - 1)
        def _():
            with _scope('ofinal'):
                cp = out_copy(g0, 16, NSB)
                cp.start()
                cp.wait()

        return carry

    jax.lax.fori_loop(0, N_LAYERS, layer, 0)


@jax.jit
def pallas_interleave_layers__sliding_block__moe_arch_mod__prompt_kernel(
    A_x: jax.Array,
    A_wqkv: jax.Array,
    A_wo: jax.Array,
    B_x: jax.Array,
    B_w_r: jax.Array,
    B_w_gate: jax.Array,
    B_w_up: jax.Array,
    B_w_down: jax.Array,
):
    del B_x
    any_spec = pl.BlockSpec(memory_space=pl.ANY)
    scratch = [
        pltpu.VMEM((S + TB, D), BF16),
        pltpu.VMEM((NG, S + TB, 128), BF16),
        pltpu.VMEM((NG, S, 128), BF16),
        pltpu.VMEM((NG, S, 128), BF16),
        pltpu.VMEM((NSB + 2, D, 128), BF16),
        pltpu.VMEM((NG, 4, XR, 128), F32),
        pltpu.VMEM((NG, 4, 8, 128), F32),
        pltpu.VMEM((NG, 4, XR // 2, 128), U32),
        pltpu.VMEM((NG, 4, 8, 128), F32),
        pltpu.VMEM((NG, SB, 128), BF16),
        pltpu.VMEM((3 * NG, D, 128), BF16),
        pltpu.VMEM((NG, D, 128), BF16),
        pltpu.VMEM((1, D), F32),
        pltpu.VMEM((FF // 128, D, 128), BF16),
        pltpu.VMEM((FF // 128, D, 128), BF16),
        pltpu.VMEM((NG, FF, 128), BF16),
        pltpu.VMEM((8, 1), F32),
        pltpu.VMEM((8, 1), I32),
        pltpu.SemaphoreType.DMA((NTB,)),
        pltpu.SemaphoreType.DMA((3 * NG // W_GROUP,)),
        pltpu.SemaphoreType.DMA((2,)),
        pltpu.SemaphoreType.DMA((NSB + 1,)),
    ]
    flag = jnp.zeros((1,), I32)
    return pl.pallas_call(
        _kernel,
        out_shape=jax.ShapeDtypeStruct((1, S, D), BF16),
        in_specs=[pl.BlockSpec(memory_space=pltpu.SMEM),
                  any_spec, any_spec, any_spec,
                  pl.BlockSpec(memory_space=pltpu.VMEM),
                  any_spec, any_spec, any_spec],
        out_specs=any_spec,
        scratch_shapes=scratch,
        compiler_params=pltpu.CompilerParams(vmem_limit_bytes=112 * 1024 * 1024),
        name="swa_moe",
    )(flag, A_x, A_wqkv, A_wo, B_w_r, B_w_gate, B_w_up, B_w_down)
```

```python
import math

import jax
import jax.numpy as jnp
import jax.experimental.pallas as pl
import jax.experimental.pallas.tpu as pltpu

F32 = jnp.float32
BF16 = jnp.bfloat16
U32 = jnp.uint32
I32 = jnp.int32

S = 2048
D = 1024
DH = 32
WIN = 256
FF = 3584
NG = 8
SB = 128
NSB = S // SB
QA = 32
XR = WIN + QA
TB = 256
NTB = S // TB
EPS = 1e-5
NEG = -1e30
QSCALE = (DH ** -0.5) * math.log2(math.e)
NT_DIMS = (((1,), (1,)), ((), ()))
N_LAYERS = 2
P1_LAST_SCORES_AT = 16
POST_PV_AT = 6
W_GROUP = 4


def _scope(name):
    return jax.named_scope(name)


def _layernorm(x):
    mean = jnp.sum(x, axis=1, keepdims=True) * (1.0 / D)
    xc = x - mean
    var = jnp.sum(xc * xc, axis=1, keepdims=True) * (1.0 / D)
    return xc * jax.lax.rsqrt(var + EPS)


def _packed(ref):
    return ref.bitcast(U32)


def _as_bf16(v):
    return pltpu.bitcast(v, BF16)


def _ln_stage(xres, xn, t):
    r0 = t * TB if isinstance(t, int) else pl.multiple_of(t * TB, TB)
    y = _layernorm(xres[pl.ds(r0, TB), :].astype(F32))
    for c in range(NG):
        xn[c, pl.ds(r0, TB), :] = y[:, c * 128:(c + 1) * 128].astype(BF16)


QKV_ORDER = list(range(2 * NG, 3 * NG)) + list(range(2 * NG))


def _qkv_stage(xn, wqkv, qs, ks, vts, t, before_chunk=None):
    xp = _packed(xn)
    wp = _packed(wqkv)
    if isinstance(t, int):
        r0, h0 = t * TB, t * (TB // 2)
    else:
        r0 = pl.multiple_of(t * TB, TB)
        h0 = pl.multiple_of(t * (TB // 2), TB // 2)
    kt0 = 2 + t * (TB // 128)
    lhs = _as_bf16(jnp.concatenate(
        [xp[c, pl.ds(h0, TB // 2), :] for c in range(NG)], axis=1))
    for n, j in enumerate(QKV_ORDER):
        if before_chunk is not None:
            before_chunk(n)
        y = jnp.dot(lhs, _as_bf16(wp[j]), preferred_element_type=F32)
        if j < NG:
            qs[j, pl.ds(r0, TB), :] = (y * QSCALE).astype(BF16)
        elif j < 2 * NG:
            ks[j - NG, pl.ds(r0, TB), :] = y.astype(BF16)
        else:
            c = j - 2 * NG
            for t in range(TB // 128):
                vts[kt0 + t, c * 128:(c + 1) * 128, :] = (
                    y[t * 128:(t + 1) * 128, :].T.astype(BF16))


def _score_stage(qs, ks, xs, ms, sb, g, static_sb=None):
    lane = jax.lax.broadcasted_iota(I32, (QA, 128), 1)
    li = lane % QA
    row = jax.lax.broadcasted_iota(I32, (QA, 128), 0)
    m_lo = row > li
    m_hi = row <= li
    lg = jax.lax.broadcasted_iota(I32, (QA // 2, 128), 1) // QA
    qp = _packed(qs)
    kp = _packed(ks)
    for a in range(4):
        if static_sb is None:
            qa2 = pl.multiple_of(sb * (SB // 2) + (QA // 2) * a, QA // 2)
            q = qp[g, pl.ds(qa2, QA // 2), :]
            first = 0
            k = kp[g, pl.ds(qa2 - WIN // 2, XR // 2), :]
        else:
            qa = static_sb * SB + QA * a
            q = qp[g, qa // 2:(qa + QA) // 2, :]
            first = WIN - qa
            k = kp[g, 0:(XR - first) // 2, :]
        qbd = jnp.concatenate(
            [jnp.where(lg == ((a - p) % 4), q, jnp.zeros_like(q)) for p in range(4)],
            axis=0)
        x = jax.lax.dot_general(_as_bf16(k), _as_bf16(qbd), NT_DIMS,
                                preferred_element_type=F32)
        n = XR - first
        hi = jnp.where(m_hi, x[n - QA:n], NEG)
        if first == 0:
            lo = jnp.where(m_lo, x[0:QA], NEG)
            x = jnp.concatenate([lo, x[QA:n - QA], hi], axis=0)
        elif n > QA:
            x = jnp.concatenate(
                [jnp.full((first, 128), NEG, F32), x[0:n - QA], hi], axis=0)
        else:
            x = jnp.concatenate([jnp.full((first, 128), NEG, F32), hi], axis=0)
        xs[g, a] = x
        j0 = first // 16
        m0 = x[16 * j0:16 * j0 + 8]
        m1 = x[16 * j0 + 8:16 * j0 + 16]
        for j in range(j0 + 1, XR // 16):
            m0 = jnp.maximum(m0, x[16 * j:16 * j + 8])
            m1 = jnp.maximum(m1, x[16 * j + 8:16 * j + 16])
        mm = jnp.max(jnp.maximum(m0, m1), axis=0, keepdims=True)
        ms[g, a] = jnp.broadcast_to(mm, (8, 128))
    return m0


def _exp_stage(xs, ms, ps, ls, g, never, after=None):
    for a in range(4):
        m = ms[g, a]
        if after is not None:
            m = jnp.where(never, after, m)
        s0 = s1 = None
        for j in range(XR // 16):
            e0 = jnp.exp2(xs[g, a, pl.ds(16 * j, 8, stride=2), :] - m)
            e1 = jnp.exp2(xs[g, a, pl.ds(16 * j + 1, 8, stride=2), :] - m)
            s0 = e0 if s0 is None else s0 + e0
            s1 = e1 if s1 is None else s1 + e1
            if j == XR // 16 - 1:
                s = s0 + s1
                e1 = jnp.where(never, s, e1)
            ps[g, a, 8 * j:8 * j + 8, :] = pltpu.pack_elementwise(
                [e0, e1], packed_dtype=BF16).astype(U32)
        ls[g, a] = s


def _pv_stage(ps, ls, vts, sb, g):
    lg8 = jax.lax.broadcasted_iota(I32, (8, 128), 1) // QA
    odd = (lg8 % 2) == 1
    hi2 = lg8 >= 2
    zero = jnp.zeros((8, 128), U32)
    pp = ps
    vp = _packed(vts)

    def sel(c, x, y):
        if x is None and y is None:
            return None
        return jnp.where(c, zero if x is None else x, zero if y is None else y)

    acc = [None] * 4
    for kt in range(3):
        yrows = [[] for _ in range(4)]
        for r in range(8 * kt, 8 * kt + 8):
            pr = []
            for a in range(4):
                j = r - 2 * a
                pr.append(pp[g, a, 8 * j:8 * j + 8, :] if 0 <= j < XR // 16 else None)
            z = [sel(odd, pr[(a + 1) % 4], pr[a]) for a in range(4)]
            for h in range(4):
                y = sel(hi2, z[(h + 2) % 4], z[h])
                yrows[h].append(zero if y is None else y)
        for h in range(4):
            y = _as_bf16(jnp.concatenate(yrows[h], axis=0))
            r0 = (g * 128 + DH * h) // 2
            vt = _as_bf16(vp[sb + kt, r0:r0 + DH // 2, :])
            ot = jnp.dot(vt, y, preferred_element_type=F32)
            acc[h] = ot if acc[h] is None else acc[h] + ot
    l = [jnp.sum(ls[g, a], axis=0, keepdims=True) for a in range(4)]
    lg1 = jax.lax.broadcasted_iota(I32, (1, 128), 1) // QA
    lz = [jnp.where((lg1 % 2) == 1, l[(a + 1) % 4], l[a]) for a in range(4)]
    ly = [jnp.where(lg1 >= 2, lz[(h + 2) % 4], lz[h]) for h in range(4)]
    return jnp.concatenate([acc[h] * (1.0 / ly[h]) for h in range(4)], axis=0)


def _unrotate_stage(ot, os_, g):
    t = ot.T
    lgrp = jax.lax.broadcasted_iota(I32, (QA, 128), 1) // QA
    odd = (lgrp % 2) == 1
    hi2 = lgrp >= 2
    tp = [t[QA * p:QA * p + QA] for p in range(4)]
    z = [jnp.where(odd, tp[(a - 1) % 4], tp[a]) for a in range(4)]
    outs = [jnp.where(hi2, z[(a - 2) % 4], z[a]) for a in range(4)]
    os_[g] = jnp.concatenate(outs, axis=0).astype(BF16)


def _proj_stage(os_, wo, wr, xres, xn, best_v, best_i, sb, never,
                overlap=None, fence=None, fence_at=NG - 1, before_chunk=None):
    op = _packed(os_)
    wp = _packed(wo)
    r0 = sb * SB if isinstance(sb, int) else pl.multiple_of(sb * SB, SB)
    lhs = jnp.concatenate([op[g] for g in range(NG)], axis=1)
    cols = []
    for j in range(NG):
        if before_chunk is not None:
            before_chunk(j)
        lj = lhs
        if overlap is not None and j == fence_at:
            head = jnp.where(never, fence(), lhs[0:8, 0:128])
            top = jnp.concatenate([head, lhs[0:8, 128:]], axis=1)
            lj = jnp.concatenate([top, lhs[8:]], axis=0)
        y = jnp.dot(_as_bf16(lj), _as_bf16(wp[j]), preferred_element_type=F32)
        cols.append(y)
        if overlap is not None and j == 0:
            overlap(y[0:8])
    x = xres[pl.ds(r0, SB), :].astype(F32) + jnp.concatenate(cols, axis=1)
    mean = jnp.sum(x, axis=1, keepdims=True) * (1.0 / D)
    xc = x - mean
    var = jnp.sum(xc * xc, axis=1, keepdims=True) * (1.0 / D)
    rstd = jax.lax.rsqrt(var + EPS)
    y = x * rstd - mean * rstd
    r = jnp.sum(y * wr[...], axis=1, keepdims=True)
    xres[pl.ds(r0, SB), :] = (x + y).astype(BF16)
    for c in range(NG):
        xn[c, pl.ds(r0, SB), :] = y[:, c * 128:(c + 1) * 128].astype(BF16)
    bv = best_v[...]
    bi = best_i[...]
    sub = jax.lax.broadcasted_iota(I32, (8, 1), 0)
    for rg in range(SB // 8):
        rr = r[8 * rg:8 * rg + 8]
        take = rr > bv
        bv = jnp.where(take, rr, bv)
        bi = jnp.where(take, sub + (r0 + 8 * rg), bi)
    best_v[...] = bv
    best_i[...] = bi


def _router_ffn(xn, wg, wu, wd, best_v, best_i):
    bv = best_v[...]
    bi = best_i[...]
    rmax = jnp.max(bv, axis=0, keepdims=True)
    idx = jnp.min(jnp.where(bv == rmax, bi, S))
    grp = idx >> 4
    xp = _packed(xn)
    h0 = pl.multiple_of(grp * 8, 8)
    lhs = _as_bf16(jnp.concatenate(
        [xp[c, pl.ds(h0, 8), :] for c in range(NG)], axis=1))
    wgp, wup, wdp = _packed(wg), _packed(wu), _packed(wd)
    act = []
    for j in range(FF // 128):
        hg = jnp.dot(lhs, _as_bf16(wgp[j]), preferred_element_type=F32)
        hu = jnp.dot(lhs, _as_bf16(wup[j]), preferred_element_type=F32)
        act.append(hg * jax.nn.sigmoid(hg) * hu)
    act = jnp.concatenate(act, axis=1).astype(BF16)
    y = jnp.concatenate(
        [jnp.dot(act, _as_bf16(wdp[j]), preferred_element_type=F32) for j in range(NG)],
        axis=1)
    row = jax.lax.broadcasted_iota(I32, (16, D), 0)
    upd = jnp.where(row == (idx & 15), y * jax.nn.sigmoid(rmax), 0.0)
    return pl.multiple_of(grp * 16, 16), upd


def _kernel(x_hbm, wqkv_hbm, wo_hbm, wr_ref, wg_hbm, wu_hbm, wd_hbm, out_hbm,
            xres, xn, qs, ks, vts, xs, ms, ps, ls, os_, wqkv, wo, wr, wg, wu, wd,
            best_v, best_i, zero, sem_x, sem_q, sem_w, sem_o):
    zero[0] = 0

    x_cp = [pltpu.make_async_copy(x_hbm.at[0, pl.ds(t * TB, TB), :],
                                  xres.at[pl.ds(t * TB, TB), :], sem_x.at[t])
            for t in range(NTB)]
    wqkv_cp = [pltpu.make_async_copy(wqkv_hbm.at[:, pl.ds(j * 128, 128)],
                                     wqkv.at[j], sem_q.at[n // W_GROUP])
               for n, j in enumerate(QKV_ORDER)]
    wo_cp = [pltpu.make_async_copy(wo_hbm.at[:, pl.ds(j * 128, 128)],
                                   wo.at[j], sem_w.at[0])
             for j in range(NG)]
    ffn_cp = [pltpu.make_async_copy(src.at[:, pl.ds(j * 128, 128)], dst.at[j],
                                    sem_w.at[1])
              for src, dst in ((wg_hbm, wg), (wu_hbm, wu), (wd_hbm, wd))
              for j in range(dst.shape[0])]
    for cp in x_cp[:1] + wqkv_cp[:W_GROUP]:
        cp.start()

    with _scope('init'):
        vts[0:2] = jnp.zeros((2,) + vts.shape[1:], BF16)
        wr[...] = wr_ref[...].astype(F32).reshape(1, D)
    with _scope('xwait'):
        x_cp[0].wait()
    for cp in wqkv_cp[W_GROUP:2 * W_GROUP] + x_cp[1:2]:
        cp.start()

    def out_copy(r0, n, slot):
        return pltpu.make_async_copy(xres.at[pl.ds(r0, n), :],
                                     out_hbm.at[0, pl.ds(r0, n), :], sem_o.at[slot])

    def layer(l, carry):
        never = jnp.full((8, 128), zero[0], I32) != 0

        with _scope('ln0'):
            _ln_stage(xres, xn, 0)

        @pl.when(l == 0)
        def _():
            def wait_group(n):
                if n % W_GROUP == 0:
                    for cp in wqkv_cp[n:n + W_GROUP]:
                        cp.wait()
                    for cp in wqkv_cp[n + 2 * W_GROUP:n + 3 * W_GROUP]:
                        cp.start()
                if n == 2 * W_GROUP:
                    x_cp[1].wait()
                if n == 3 * NG - 2 * W_GROUP:
                    for cp in x_cp[2:]:
                        cp.start()

            with _scope('p1_first'):
                _qkv_stage(xn, wqkv, qs, ks, vts, 0, wait_group)
                _ln_stage(xres, xn, 1)
            for cp in wo_cp + ffn_cp:
                cp.start()

        def wait_x(t):
            @pl.when(l == 0)
            def _():
                pltpu.make_async_copy(
                    x_hbm.at[0, pl.ds(t * TB, TB), :],
                    xres.at[pl.ds(t * TB, TB), :], sem_x.at[t]).wait()

        def p1_step(t, c):
            wait_x(t + 1)
            _qkv_stage(xn, wqkv, qs, ks, vts, t)
            _ln_stage(xres, xn, t + 1)
            return c

        with _scope('p1_loop'):
            jax.lax.fori_loop(jnp.where(l == 0, 1, 0), NTB - 1, p1_step, 0)

        best_v[...] = jnp.full((8, 1), -jnp.inf, F32)
        best_i[...] = jnp.zeros((8, 1), I32)

        def pv_all(sb):
            for g in range(NG):
                _unrotate_stage(_pv_stage(ps, ls, vts, sb, g), os_, g)

        def exp_groups(gs, after=None):
            for g in gs:
                _exp_stage(xs, ms, ps, ls, g, never, after)

        def proj(sb, exp_gs=None, **kw):
            if exp_gs is None:
                _proj_stage(os_, wo, wr, xres, xn, best_v, best_i, sb, never, **kw)
            else:
                _proj_stage(os_, wo, wr, xres, xn, best_v, best_i, sb, never,
                            overlap=lambda v: exp_groups(exp_gs, v),
                            fence=lambda: ps[zero[0], 0, 0:8, :], **kw)

        def emit_out(sb):
            @pl.when(l == N_LAYERS - 1)
            def _():
                out_copy(pl.multiple_of(sb * SB, SB), SB, sb).start()

        one = zero[0] + 1

        def p1_last(_, c):
            for g in range(NG):
                _score_stage(qs, ks, xs, ms, None, g, static_sb=0)
            exp_groups(range(NG))

            def mid(n):
                if n == P1_LAST_SCORES_AT:
                    for g in range(NG):
                        _score_stage(qs, ks, xs, ms, None, g, static_sb=1)

            _qkv_stage(xn, wqkv, qs, ks, vts, NTB - 1, mid)
            return c

        def steady(s, c):
            pv_all(s - 1)
            exp_groups([0])
            _score_stage(qs, ks, xs, ms, s + 1, 0)
            proj(s - 1, range(1, NG))
            for g in range(1, NG):
                _score_stage(qs, ks, xs, ms, s + 1, g)
            emit_out(s - 1)
            return c

        def post(_, c):
            pv_all(NSB - 2)

            def mid(j):
                if j == POST_PV_AT:
                    pv_all(NSB - 1)

            proj(NSB - 2, range(NG), fence_at=POST_PV_AT - 1, before_chunk=mid)
            proj(NSB - 1)
            return c

        with _scope('p1_last'):
            jax.lax.fori_loop(0, one, p1_last, 0)

        @pl.when(l == 0)
        def _():
            with _scope('wowait'):
                for cp in wo_cp:
                    cp.wait()

        with _scope('steady'):
            jax.lax.fori_loop(1, NSB - 1, steady, 0)
        with _scope('post'):
            jax.lax.fori_loop(0, one, post, 0)
        emit_out(NSB - 2)
        emit_out(NSB - 1)

        @pl.when(l == 0)
        def _():
            with _scope('ffnwait'):
                for cp in ffn_cp:
                    cp.wait()

        with _scope('ffn'):
            g0, upd = _router_ffn(xn, wg, wu, wd, best_v, best_i)

        @pl.when(l == N_LAYERS - 1)
        def _():
            with _scope('owait'):
                for sb in range(NSB):
                    out_copy(sb * SB, SB, sb).wait()

        xres[pl.ds(g0, 16), :] = (
            xres[pl.ds(g0, 16), :].astype(F32) + upd).astype(BF16)

        @pl.when(l == N_LAYERS - 1)
        def _():
            with _scope('ofinal'):
                cp = out_copy(g0, 16, NSB)
                cp.start()
                cp.wait()

        return carry

    jax.lax.fori_loop(0, N_LAYERS, layer, 0)


@jax.jit
def pallas_interleave_layers__sliding_block__moe_arch_mod__prompt_kernel(
    A_x: jax.Array,
    A_wqkv: jax.Array,
    A_wo: jax.Array,
    B_x: jax.Array,
    B_w_r: jax.Array,
    B_w_gate: jax.Array,
    B_w_up: jax.Array,
    B_w_down: jax.Array,
):
    del B_x
    any_spec = pl.BlockSpec(memory_space=pl.ANY)
    scratch = [
        pltpu.VMEM((S, D), BF16),
        pltpu.VMEM((NG, S, 128), BF16),
        pltpu.VMEM((NG, S, 128), BF16),
        pltpu.VMEM((NG, S, 128), BF16),
        pltpu.VMEM((NSB + 2, D, 128), BF16),
        pltpu.VMEM((NG, 4, XR, 128), F32),
        pltpu.VMEM((NG, 4, 8, 128), F32),
        pltpu.VMEM((NG, 4, XR // 2, 128), U32),
        pltpu.VMEM((NG, 4, 8, 128), F32),
        pltpu.VMEM((NG, SB, 128), BF16),
        pltpu.VMEM((3 * NG, D, 128), BF16),
        pltpu.VMEM((NG, D, 128), BF16),
        pltpu.VMEM((1, D), F32),
        pltpu.VMEM((FF // 128, D, 128), BF16),
        pltpu.VMEM((FF // 128, D, 128), BF16),
        pltpu.VMEM((NG, FF, 128), BF16),
        pltpu.VMEM((8, 1), F32),
        pltpu.VMEM((8, 1), I32),
        pltpu.SMEM((1,), I32),
        pltpu.SemaphoreType.DMA((NTB,)),
        pltpu.SemaphoreType.DMA((3 * NG // W_GROUP,)),
        pltpu.SemaphoreType.DMA((2,)),
        pltpu.SemaphoreType.DMA((NSB + 1,)),
    ]
    return pl.pallas_call(
        _kernel,
        out_shape=jax.ShapeDtypeStruct((1, S, D), BF16),
        in_specs=[any_spec, any_spec, any_spec,
                  pl.BlockSpec(memory_space=pltpu.VMEM),
                  any_spec, any_spec, any_spec],
        out_specs=any_spec,
        scratch_shapes=scratch,
        compiler_params=pltpu.CompilerParams(vmem_limit_bytes=112 * 1024 * 1024),
        name="swa_moe",
    )(A_x, A_wqkv, A_wo, B_w_r, B_w_gate, B_w_up, B_w_down)
```

```python
import math

import jax
import jax.numpy as jnp
import jax.experimental.pallas as pl
import jax.experimental.pallas.tpu as pltpu

F32 = jnp.float32
BF16 = jnp.bfloat16
U32 = jnp.uint32
I32 = jnp.int32

S = 2048
D = 1024
DH = 32
WIN = 256
FF = 3584
NG = 8
SB = 128
NSB = S // SB
QA = 32
XR = WIN + QA
TB = 256
NTB = S // TB
EPS = 1e-5
NEG = -1e30
QSCALE = (DH ** -0.5) * math.log2(math.e)
NT_DIMS = (((1,), (1,)), ((), ()))
N_LAYERS = 2
P1_LAST_SCORES_AT = 16
POST_PV_AT = 7
POST_EARLY_EXP = 1
W_GROUPS = (4, 4, 4, 4, 4, 4)
W_START = [sum(W_GROUPS[:i]) for i in range(len(W_GROUPS) + 1)]
W_AHEAD = 2


def _scope(name):
    return jax.named_scope(name)


def _layernorm(x):
    mean = jnp.sum(x, axis=1, keepdims=True) * (1.0 / D)
    xc = x - mean
    var = jnp.sum(xc * xc, axis=1, keepdims=True) * (1.0 / D)
    return xc * jax.lax.rsqrt(var + EPS)


def _packed(ref):
    return ref.bitcast(U32)


def _as_bf16(v):
    return pltpu.bitcast(v, BF16)


def _ln_stage(xres, xn, t):
    r0 = t * TB if isinstance(t, int) else pl.multiple_of(t * TB, TB)
    y = _layernorm(xres[pl.ds(r0, TB), :].astype(F32))
    for c in range(NG):
        xn[c, pl.ds(r0, TB), :] = y[:, c * 128:(c + 1) * 128].astype(BF16)


QKV_ORDER = list(range(2 * NG, 3 * NG)) + list(range(2 * NG))


def _qkv_stage(xn, wqkv, qs, ks, vts, t, before_chunk=None):
    xp = _packed(xn)
    wp = _packed(wqkv)
    if isinstance(t, int):
        r0, h0 = t * TB, t * (TB // 2)
    else:
        r0 = pl.multiple_of(t * TB, TB)
        h0 = pl.multiple_of(t * (TB // 2), TB // 2)
    kt0 = 2 + t * (TB // 128)
    lhs = _as_bf16(jnp.concatenate(
        [xp[c, pl.ds(h0, TB // 2), :] for c in range(NG)], axis=1))
    for n, j in enumerate(QKV_ORDER):
        if before_chunk is not None:
            before_chunk(n)
        y = jnp.dot(lhs, _as_bf16(wp[j]), preferred_element_type=F32)
        if j < NG:
            qs[j, pl.ds(r0, TB), :] = (y * QSCALE).astype(BF16)
        elif j < 2 * NG:
            ks[j - NG, pl.ds(r0, TB), :] = y.astype(BF16)
        else:
            c = j - 2 * NG
            for t in range(TB // 128):
                vts[kt0 + t, c * 128:(c + 1) * 128, :] = (
                    y[t * 128:(t + 1) * 128, :].T.astype(BF16))


def _score_stage(qs, ks, xs, ms, sb, g, static_sb=None, b=None):
    lane = jax.lax.broadcasted_iota(I32, (QA, 128), 1)
    li = lane % QA
    row = jax.lax.broadcasted_iota(I32, (QA, 128), 0)
    m_lo = row > li
    m_hi = row <= li
    lg = jax.lax.broadcasted_iota(I32, (QA // 2, 128), 1) // QA
    qp = _packed(qs)
    kp = _packed(ks)
    b = g if b is None else b
    for a in range(4):
        if static_sb is None:
            qa2 = pl.multiple_of(sb * (SB // 2) + (QA // 2) * a, QA // 2)
            q = qp[g, pl.ds(qa2, QA // 2), :]
            first = 0
            k = kp[g, pl.ds(qa2 - WIN // 2, XR // 2), :]
        else:
            qa = static_sb * SB + QA * a
            q = qp[g, qa // 2:(qa + QA) // 2, :]
            first = WIN - qa
            k = kp[g, 0:(XR - first) // 2, :]
        qbd = jnp.concatenate(
            [jnp.where(lg == ((a - p) % 4), q, jnp.zeros_like(q)) for p in range(4)],
            axis=0)
        x = jax.lax.dot_general(_as_bf16(k), _as_bf16(qbd), NT_DIMS,
                                preferred_element_type=F32)
        n = XR - first
        hi = jnp.where(m_hi, x[n - QA:n], NEG)
        if first == 0:
            lo = jnp.where(m_lo, x[0:QA], NEG)
            x = jnp.concatenate([lo, x[QA:n - QA], hi], axis=0)
        elif n > QA:
            x = jnp.concatenate(
                [jnp.full((first, 128), NEG, F32), x[0:n - QA], hi], axis=0)
        else:
            x = jnp.concatenate([jnp.full((first, 128), NEG, F32), hi], axis=0)
        xs[b, a] = x
        j0 = first // 16
        m0 = x[16 * j0:16 * j0 + 8]
        m1 = x[16 * j0 + 8:16 * j0 + 16]
        for j in range(j0 + 1, XR // 16):
            m0 = jnp.maximum(m0, x[16 * j:16 * j + 8])
            m1 = jnp.maximum(m1, x[16 * j + 8:16 * j + 16])
        mm = jnp.max(jnp.maximum(m0, m1), axis=0, keepdims=True)
        ms[b, a] = jnp.broadcast_to(mm, (8, 128))
    return m0


def _exp_stage(xs, ms, ps, ls, g, never, after=None):
    for a in range(4):
        m = ms[g, a]
        if after is not None:
            m = jnp.where(never, after, m)
        s0 = s1 = None
        for j in range(XR // 16):
            e0 = jnp.exp2(xs[g, a, pl.ds(16 * j, 8, stride=2), :] - m)
            e1 = jnp.exp2(xs[g, a, pl.ds(16 * j + 1, 8, stride=2), :] - m)
            s0 = e0 if s0 is None else s0 + e0
            s1 = e1 if s1 is None else s1 + e1
            if j == XR // 16 - 1:
                s = s0 + s1
                e1 = jnp.where(never, s, e1)
            ps[g, a, 8 * j:8 * j + 8, :] = pltpu.pack_elementwise(
                [e0, e1], packed_dtype=BF16).astype(U32)
        ls[g, a] = s


def _pv_stage(ps, ls, vts, sb, g, b=None):
    lg8 = jax.lax.broadcasted_iota(I32, (8, 128), 1) // QA
    odd = (lg8 % 2) == 1
    hi2 = lg8 >= 2
    zero = jnp.zeros((8, 128), U32)
    pp = ps
    vp = _packed(vts)
    b = g if b is None else b

    def sel(c, x, y):
        if x is None and y is None:
            return None
        return jnp.where(c, zero if x is None else x, zero if y is None else y)

    acc = [None] * 4
    for kt in range(3):
        yrows = [[] for _ in range(4)]
        for r in range(8 * kt, 8 * kt + 8):
            pr = []
            for a in range(4):
                j = r - 2 * a
                pr.append(pp[b, a, 8 * j:8 * j + 8, :] if 0 <= j < XR // 16 else None)
            z = [sel(odd, pr[(a + 1) % 4], pr[a]) for a in range(4)]
            for h in range(4):
                y = sel(hi2, z[(h + 2) % 4], z[h])
                yrows[h].append(zero if y is None else y)
        for h in range(4):
            y = _as_bf16(jnp.concatenate(yrows[h], axis=0))
            r0 = (g * 128 + DH * h) // 2
            vt = _as_bf16(vp[sb + kt, r0:r0 + DH // 2, :])
            ot = jnp.dot(vt, y, preferred_element_type=F32)
            acc[h] = ot if acc[h] is None else acc[h] + ot
    l = [jnp.sum(ls[b, a], axis=0, keepdims=True) for a in range(4)]
    lg1 = jax.lax.broadcasted_iota(I32, (1, 128), 1) // QA
    lz = [jnp.where((lg1 % 2) == 1, l[(a + 1) % 4], l[a]) for a in range(4)]
    ly = [jnp.where(lg1 >= 2, lz[(h + 2) % 4], lz[h]) for h in range(4)]
    return jnp.concatenate([acc[h] * (1.0 / ly[h]) for h in range(4)], axis=0)


def _unrotate_stage(ot, os_, g):
    t = ot.T
    lgrp = jax.lax.broadcasted_iota(I32, (QA, 128), 1) // QA
    odd = (lgrp % 2) == 1
    hi2 = lgrp >= 2
    tp = [t[QA * p:QA * p + QA] for p in range(4)]
    z = [jnp.where(odd, tp[(a - 1) % 4], tp[a]) for a in range(4)]
    outs = [jnp.where(hi2, z[(a - 2) % 4], z[a]) for a in range(4)]
    os_[g] = jnp.concatenate(outs, axis=0).astype(BF16)


def _proj_stage(os_, wo, wr, xres, xn, best_v, best_i, sb, never,
                overlap=None, fence=None, fence_at=NG - 1, before_chunk=None):
    op = _packed(os_)
    wp = _packed(wo)
    r0 = sb * SB if isinstance(sb, int) else pl.multiple_of(sb * SB, SB)
    lhs = jnp.concatenate([op[g] for g in range(NG)], axis=1)
    cols = []
    for j in range(NG):
        if before_chunk is not None:
            before_chunk(j)
        lj = lhs
        if overlap is not None and j == fence_at:
            head = jnp.where(never, fence(), lhs[0:8, 0:128])
            top = jnp.concatenate([head, lhs[0:8, 128:]], axis=1)
            lj = jnp.concatenate([top, lhs[8:]], axis=0)
        y = jnp.dot(_as_bf16(lj), _as_bf16(wp[j]), preferred_element_type=F32)
        cols.append(y)
        if overlap is not None and j == 0:
            overlap(y[0:8])
    x = xres[pl.ds(r0, SB), :].astype(F32) + jnp.concatenate(cols, axis=1)
    mean = jnp.sum(x, axis=1, keepdims=True) * (1.0 / D)
    xc = x - mean
    var = jnp.sum(xc * xc, axis=1, keepdims=True) * (1.0 / D)
    rstd = jax.lax.rsqrt(var + EPS)
    y = x * rstd - mean * rstd
    r = jnp.sum(y * wr[...], axis=1, keepdims=True)
    xres[pl.ds(r0, SB), :] = (x + y).astype(BF16)
    for c in range(NG):
        xn[c, pl.ds(r0, SB), :] = y[:, c * 128:(c + 1) * 128].astype(BF16)
    bv = best_v[...]
    bi = best_i[...]
    sub = jax.lax.broadcasted_iota(I32, (8, 1), 0)
    for rg in range(SB // 8):
        rr = r[8 * rg:8 * rg + 8]
        take = rr > bv
        bv = jnp.where(take, rr, bv)
        bi = jnp.where(take, sub + (r0 + 8 * rg), bi)
    best_v[...] = bv
    best_i[...] = bi


def _router_ffn(xn, wg, wu, wd, best_v, best_i):
    bv = best_v[...]
    bi = best_i[...]
    rmax = jnp.max(bv, axis=0, keepdims=True)
    idx = jnp.min(jnp.where(bv == rmax, bi, S))
    grp = idx >> 4
    xp = _packed(xn)
    h0 = pl.multiple_of(grp * 8, 8)
    lhs = _as_bf16(jnp.concatenate(
        [xp[c, pl.ds(h0, 8), :] for c in range(NG)], axis=1))
    wgp, wup, wdp = _packed(wg), _packed(wu), _packed(wd)
    act = []
    for j in range(FF // 128):
        hg = jnp.dot(lhs, _as_bf16(wgp[j]), preferred_element_type=F32)
        hu = jnp.dot(lhs, _as_bf16(wup[j]), preferred_element_type=F32)
        act.append(hg * jax.nn.sigmoid(hg) * hu)
    act = jnp.concatenate(act, axis=1).astype(BF16)
    y = jnp.concatenate(
        [jnp.dot(act, _as_bf16(wdp[j]), preferred_element_type=F32) for j in range(NG)],
        axis=1)
    row = jax.lax.broadcasted_iota(I32, (16, D), 0)
    upd = jnp.where(row == (idx & 15), y * jax.nn.sigmoid(rmax), 0.0)
    return pl.multiple_of(grp * 16, 16), upd


def _kernel(x_hbm, wqkv_hbm, wo_hbm, wr_ref, wg_hbm, wu_hbm, wd_hbm, out_hbm,
            xres, xn, qs, ks, vts, xs, ms, ps, ls, os_, wqkv, wo, wr, wg, wu, wd,
            best_v, best_i, zero, sem_x, sem_q, sem_w, sem_o):
    zero[0] = 0

    x_cp = [pltpu.make_async_copy(x_hbm.at[0, pl.ds(t * TB, TB), :],
                                  xres.at[pl.ds(t * TB, TB), :], sem_x.at[t])
            for t in range(NTB)]
    wqkv_cp = [[pltpu.make_async_copy(wqkv_hbm.at[:, pl.ds(j * 128, 128)],
                                      wqkv.at[j], sem_q.at[k])
                for j in QKV_ORDER[W_START[k]:W_START[k + 1]]]
               for k in range(len(W_GROUPS))]
    wo_cp = [pltpu.make_async_copy(wo_hbm.at[:, pl.ds(j * 128, 128)],
                                   wo.at[j], sem_w.at[0])
             for j in range(NG)]
    ffn_cp = [pltpu.make_async_copy(src.at[:, pl.ds(j * 128, 128)], dst.at[j],
                                    sem_w.at[1])
              for src, dst in ((wg_hbm, wg), (wu_hbm, wu), (wd_hbm, wd))
              for j in range(dst.shape[0])]
    for cp in x_cp[:1] + wqkv_cp[0]:
        cp.start()

    with _scope('init'):
        vts[0:2] = jnp.zeros((2,) + vts.shape[1:], BF16)
        wr[...] = wr_ref[...].astype(F32).reshape(1, D)
    with _scope('xwait'):
        x_cp[0].wait()
    for cp in sum(wqkv_cp[1:W_AHEAD], []) + x_cp[1:2]:
        cp.start()

    def out_copy(r0, n, slot):
        return pltpu.make_async_copy(xres.at[pl.ds(r0, n), :],
                                     out_hbm.at[0, pl.ds(r0, n), :], sem_o.at[slot])

    def layer(l, carry):
        never = jnp.full((8, 128), zero[0], I32) != 0

        with _scope('ln0'):
            _ln_stage(xres, xn, 0)

        @pl.when(l == 0)
        def _():
            def wait_group(n):
                if n in W_START:
                    k = W_START.index(n)
                    for cp in wqkv_cp[k]:
                        cp.wait()
                    if k + W_AHEAD < len(W_GROUPS):
                        for cp in wqkv_cp[k + W_AHEAD]:
                            cp.start()
                    if k == len(W_GROUPS) // 2:
                        x_cp[1].wait()
                    if k == len(W_GROUPS) - 1:
                        for cp in x_cp[2:]:
                            cp.start()

            with _scope('p1_first'):
                _qkv_stage(xn, wqkv, qs, ks, vts, 0, wait_group)
                _ln_stage(xres, xn, 1)

        def wait_x(t):
            @pl.when(l == 0)
            def _():
                pltpu.make_async_copy(
                    x_hbm.at[0, pl.ds(t * TB, TB), :],
                    xres.at[pl.ds(t * TB, TB), :], sem_x.at[t]).wait()

        def p1_step(t, c):
            wait_x(t + 1)

            @pl.when(jnp.logical_and(l == 0, t == 2))
            def _():
                for cp in wo_cp + ffn_cp:
                    cp.start()

            _qkv_stage(xn, wqkv, qs, ks, vts, t)
            _ln_stage(xres, xn, t + 1)
            return c

        with _scope('p1_loop'):
            jax.lax.fori_loop(jnp.where(l == 0, 1, 0), NTB - 1, p1_step, 0)

        best_v[...] = jnp.full((8, 1), -jnp.inf, F32)
        best_i[...] = jnp.zeros((8, 1), I32)

        def pv_all(sb):
            for g in range(NG):
                _unrotate_stage(_pv_stage(ps, ls, vts, sb, g), os_, g)

        def exp_groups(gs, after=None):
            for g in gs:
                _exp_stage(xs, ms, ps, ls, g, never, after)

        def proj(sb, exp_gs=None, **kw):
            if exp_gs is None:
                _proj_stage(os_, wo, wr, xres, xn, best_v, best_i, sb, never, **kw)
            else:
                _proj_stage(os_, wo, wr, xres, xn, best_v, best_i, sb, never,
                            overlap=lambda v: exp_groups(exp_gs, v),
                            fence=lambda: ps[zero[0], 0, 0:8, :], **kw)

        def emit_out(sbs):
            @pl.when(l == N_LAYERS - 1)
            def _():
                for sb in sbs:
                    out_copy(sb * SB, SB, sb).start()

        one = zero[0] + 1

        def p1_last(_, c):
            for g in range(NG):
                _score_stage(qs, ks, xs, ms, None, g, static_sb=0)
            exp_groups(range(NG))

            def mid(n):
                if n == P1_LAST_SCORES_AT:
                    for g in range(NG):
                        _score_stage(qs, ks, xs, ms, None, g, static_sb=1)

            _qkv_stage(xn, wqkv, qs, ks, vts, NTB - 1, mid)
            return c

        def steady(s, c):
            pv_all(s - 1)
            exp_groups([0])
            _score_stage(qs, ks, xs, ms, s + 1, 0)
            proj(s - 1, range(1, NG))
            for g in range(1, NG):
                _score_stage(qs, ks, xs, ms, s + 1, g)
            return c

        def post(_, c):
            pv_all(NSB - 2)

            def mid(j):
                if j == POST_PV_AT:
                    pv_all(NSB - 1)

            exp_groups(range(POST_EARLY_EXP))
            proj(NSB - 2, range(POST_EARLY_EXP, NG), fence_at=POST_PV_AT - 1,
                 before_chunk=mid)
            proj(NSB - 1)
            return c

        with _scope('p1_last'):
            jax.lax.fori_loop(0, one, p1_last, 0)

        @pl.when(l == 0)
        def _():
            with _scope('wowait'):
                for cp in wo_cp:
                    cp.wait()

        with _scope('steady'):
            jax.lax.fori_loop(1, NSB - 1, steady, 0)
        emit_out(range(NSB - 2))
        with _scope('post'):
            jax.lax.fori_loop(0, one, post, 0)
        emit_out(range(NSB - 2, NSB))

        @pl.when(l == 0)
        def _():
            with _scope('ffnwait'):
                for cp in ffn_cp:
                    cp.wait()

        with _scope('ffn'):
            g0, upd = _router_ffn(xn, wg, wu, wd, best_v, best_i)

        @pl.when(l == N_LAYERS - 1)
        def _():
            with _scope('owait'):
                for sb in range(NSB):
                    out_copy(sb * SB, SB, sb).wait()

        xres[pl.ds(g0, 16), :] = (
            xres[pl.ds(g0, 16), :].astype(F32) + upd).astype(BF16)

        @pl.when(l == N_LAYERS - 1)
        def _():
            with _scope('ofinal'):
                cp = out_copy(g0, 16, NSB)
                cp.start()
                cp.wait()

        return carry

    jax.lax.fori_loop(0, N_LAYERS, layer, 0)


@jax.jit
def pallas_interleave_layers__sliding_block__moe_arch_mod__prompt_kernel(
    A_x: jax.Array,
    A_wqkv: jax.Array,
    A_wo: jax.Array,
    B_x: jax.Array,
    B_w_r: jax.Array,
    B_w_gate: jax.Array,
    B_w_up: jax.Array,
    B_w_down: jax.Array,
):
    del B_x
    any_spec = pl.BlockSpec(memory_space=pl.ANY)
    scratch = [
        pltpu.VMEM((S, D), BF16),
        pltpu.VMEM((NG, S, 128), BF16),
        pltpu.VMEM((NG, S, 128), BF16),
        pltpu.VMEM((NG, S, 128), BF16),
        pltpu.VMEM((NSB + 2, D, 128), BF16),
        pltpu.VMEM((NG, 4, XR, 128), F32),
        pltpu.VMEM((NG, 4, 8, 128), F32),
        pltpu.VMEM((NG, 4, XR // 2, 128), U32),
        pltpu.VMEM((NG, 4, 8, 128), F32),
        pltpu.VMEM((NG, SB, 128), BF16),
        pltpu.VMEM((3 * NG, D, 128), BF16),
        pltpu.VMEM((NG, D, 128), BF16),
        pltpu.VMEM((1, D), F32),
        pltpu.VMEM((FF // 128, D, 128), BF16),
        pltpu.VMEM((FF // 128, D, 128), BF16),
        pltpu.VMEM((NG, FF, 128), BF16),
        pltpu.VMEM((8, 1), F32),
        pltpu.VMEM((8, 1), I32),
        pltpu.SMEM((1,), I32),
        pltpu.SemaphoreType.DMA((NTB,)),
        pltpu.SemaphoreType.DMA((len(W_GROUPS),)),
        pltpu.SemaphoreType.DMA((2,)),
        pltpu.SemaphoreType.DMA((NSB + 1,)),
    ]
    return pl.pallas_call(
        _kernel,
        out_shape=jax.ShapeDtypeStruct((1, S, D), BF16),
        in_specs=[any_spec, any_spec, any_spec,
                  pl.BlockSpec(memory_space=pltpu.VMEM),
                  any_spec, any_spec, any_spec],
        out_specs=any_spec,
        scratch_shapes=scratch,
        compiler_params=pltpu.CompilerParams(vmem_limit_bytes=112 * 1024 * 1024),
        name="swa_moe",
    )(A_x, A_wqkv, A_wo, B_w_r, B_w_gate, B_w_up, B_w_down)
```

```python
import math

import jax
import jax.numpy as jnp
import jax.experimental.pallas as pl
import jax.experimental.pallas.tpu as pltpu

F32 = jnp.float32
BF16 = jnp.bfloat16
U32 = jnp.uint32
I32 = jnp.int32

S = 2048
D = 1024
DH = 32
WIN = 256
FF = 3584
NG = 8
SB = 128
NSB = S // SB
QA = 32
XR = WIN + QA
TB = 256
NTB = S // TB
EPS = 1e-5
NEG = -1e30
QSCALE = (DH ** -0.5) * math.log2(math.e)
NT_DIMS = (((1,), (1,)), ((), ()))
N_LAYERS = 2
P1_LAST_SCORES_AT = 16
POST_PV_AT = 7
POST_EARLY_EXP = 1
W_GROUPS = (4, 4, 4, 4, 4, 4)
W_START = [sum(W_GROUPS[:i]) for i in range(len(W_GROUPS) + 1)]
W_AHEAD = 2


def _scope(name):
    return jax.named_scope(name)


def _layernorm(x):
    mean = jnp.sum(x, axis=1, keepdims=True) * (1.0 / D)
    xc = x - mean
    var = jnp.sum(xc * xc, axis=1, keepdims=True) * (1.0 / D)
    return xc * jax.lax.rsqrt(var + EPS)


def _packed(ref):
    return ref.bitcast(U32)


def _as_bf16(v):
    return pltpu.bitcast(v, BF16)


def _ln_stage(xres, xn, t):
    r0 = t * TB if isinstance(t, int) else pl.multiple_of(t * TB, TB)
    y = _layernorm(xres[pl.ds(r0, TB), :].astype(F32))
    for c in range(NG):
        xn[c, pl.ds(r0, TB), :] = y[:, c * 128:(c + 1) * 128].astype(BF16)


QKV_ORDER = list(range(2 * NG, 3 * NG)) + list(range(2 * NG))


def _qkv_stage(xn, wqkv, qs, ks, vts, t, before_chunk=None):
    xp = _packed(xn)
    wp = _packed(wqkv)
    if isinstance(t, int):
        r0, h0 = t * TB, t * (TB // 2)
    else:
        r0 = pl.multiple_of(t * TB, TB)
        h0 = pl.multiple_of(t * (TB // 2), TB // 2)
    kt0 = 2 + t * (TB // 128)
    lhs = _as_bf16(jnp.concatenate(
        [xp[c, pl.ds(h0, TB // 2), :] for c in range(NG)], axis=1))
    for n, j in enumerate(QKV_ORDER):
        if before_chunk is not None:
            before_chunk(n)
        y = jnp.dot(lhs, _as_bf16(wp[j]), preferred_element_type=F32)
        if j < NG:
            qs[j, pl.ds(r0, TB), :] = (y * QSCALE).astype(BF16)
        elif j < 2 * NG:
            ks[j - NG, pl.ds(r0, TB), :] = y.astype(BF16)
        else:
            c = j - 2 * NG
            for t in range(TB // 128):
                vts[kt0 + t, c * 128:(c + 1) * 128, :] = (
                    y[t * 128:(t + 1) * 128, :].T.astype(BF16))


def _score_stage(qs, ks, xs, ms, sb, g, static_sb=None, b=None):
    lane = jax.lax.broadcasted_iota(I32, (QA, 128), 1)
    li = lane % QA
    row = jax.lax.broadcasted_iota(I32, (QA, 128), 0)
    m_lo = row > li
    m_hi = row <= li
    lg = jax.lax.broadcasted_iota(I32, (QA // 2, 128), 1) // QA
    qp = _packed(qs)
    kp = _packed(ks)
    b = g if b is None else b
    for a in range(4):
        if static_sb is None:
            qa2 = pl.multiple_of(sb * (SB // 2) + (QA // 2) * a, QA // 2)
            q = qp[g, pl.ds(qa2, QA // 2), :]
            first = 0
            k = kp[g, pl.ds(qa2 - WIN // 2, XR // 2), :]
        else:
            qa = static_sb * SB + QA * a
            q = qp[g, qa // 2:(qa + QA) // 2, :]
            first = WIN - qa
            k = kp[g, 0:(XR - first) // 2, :]
        qbd = jnp.concatenate(
            [jnp.where(lg == ((a - p) % 4), q, jnp.zeros_like(q)) for p in range(4)],
            axis=0)
        x = jax.lax.dot_general(_as_bf16(k), _as_bf16(qbd), NT_DIMS,
                                preferred_element_type=F32)
        n = XR - first
        hi = jnp.where(m_hi, x[n - QA:n], NEG)
        if first == 0:
            lo = jnp.where(m_lo, x[0:QA], NEG)
            x = jnp.concatenate([lo, x[QA:n - QA], hi], axis=0)
        elif n > QA:
            x = jnp.concatenate(
                [jnp.full((first, 128), NEG, F32), x[0:n - QA], hi], axis=0)
        else:
            x = jnp.concatenate([jnp.full((first, 128), NEG, F32), hi], axis=0)
        xs[b, a] = x
        j0 = first // 16
        m0 = x[16 * j0:16 * j0 + 8]
        m1 = x[16 * j0 + 8:16 * j0 + 16]
        for j in range(j0 + 1, XR // 16):
            m0 = jnp.maximum(m0, x[16 * j:16 * j + 8])
            m1 = jnp.maximum(m1, x[16 * j + 8:16 * j + 16])
        mm = jnp.max(jnp.maximum(m0, m1), axis=0, keepdims=True)
        ms[b, a] = jnp.broadcast_to(mm, (8, 128))
    return m0


def _exp_stage(xs, ms, ps, ls, g, never, after=None):
    for a in range(4):
        m = ms[g, a]
        if after is not None:
            m = jnp.where(never, after, m)
        s0 = s1 = None
        for j in range(XR // 16):
            e0 = jnp.exp2(xs[g, a, 16 * j:16 * j + 8, :] - m)
            e1 = jnp.exp2(xs[g, a, 16 * j + 8:16 * j + 16, :] - m)
            s0 = e0 if s0 is None else s0 + e0
            s1 = e1 if s1 is None else s1 + e1
            if j == XR // 16 - 1:
                s = s0 + s1
                e1 = jnp.where(never, s, e1)
            ps[g, a, 16 * j:16 * j + 16, :] = (
                jnp.concatenate([e0, e1], axis=0).astype(BF16))
        ls[g, a] = s


def _pv_stage(ps, ls, vts, sb, g, b=None):
    lg8 = jax.lax.broadcasted_iota(I32, (8, 128), 1) // QA
    odd = (lg8 % 2) == 1
    hi2 = lg8 >= 2
    zero = jnp.zeros((8, 128), U32)
    pp = _packed(ps)
    vp = _packed(vts)
    b = g if b is None else b

    def sel(c, x, y):
        if x is None and y is None:
            return None
        return jnp.where(c, zero if x is None else x, zero if y is None else y)

    acc = [None] * 4
    for kt in range(3):
        yrows = [[] for _ in range(4)]
        for r in range(8 * kt, 8 * kt + 8):
            pr = []
            for a in range(4):
                j = r - 2 * a
                pr.append(pp[b, a, 8 * j:8 * j + 8, :] if 0 <= j < XR // 16 else None)
            z = [sel(odd, pr[(a + 1) % 4], pr[a]) for a in range(4)]
            for h in range(4):
                y = sel(hi2, z[(h + 2) % 4], z[h])
                yrows[h].append(zero if y is None else y)
        for h in range(4):
            y = _as_bf16(jnp.concatenate(yrows[h], axis=0))
            r0 = (g * 128 + DH * h) // 2
            vt = _as_bf16(vp[sb + kt, r0:r0 + DH // 2, :])
            ot = jnp.dot(vt, y, preferred_element_type=F32)
            acc[h] = ot if acc[h] is None else acc[h] + ot
    l = [jnp.sum(ls[b, a], axis=0, keepdims=True) for a in range(4)]
    lg1 = jax.lax.broadcasted_iota(I32, (1, 128), 1) // QA
    lz = [jnp.where((lg1 % 2) == 1, l[(a + 1) % 4], l[a]) for a in range(4)]
    ly = [jnp.where(lg1 >= 2, lz[(h + 2) % 4], lz[h]) for h in range(4)]
    return jnp.concatenate([acc[h] * (1.0 / ly[h]) for h in range(4)], axis=0)


def _unrotate_stage(ot, os_, g):
    t = ot.T
    lgrp = jax.lax.broadcasted_iota(I32, (QA, 128), 1) // QA
    odd = (lgrp % 2) == 1
    hi2 = lgrp >= 2
    tp = [t[QA * p:QA * p + QA] for p in range(4)]
    z = [jnp.where(odd, tp[(a - 1) % 4], tp[a]) for a in range(4)]
    outs = [jnp.where(hi2, z[(a - 2) % 4], z[a]) for a in range(4)]
    os_[g] = jnp.concatenate(outs, axis=0).astype(BF16)


def _proj_stage(os_, wo, wr, xres, xn, best_v, best_i, sb, never,
                overlap=None, fence=None, fence_at=NG - 1, before_chunk=None):
    op = _packed(os_)
    wp = _packed(wo)
    r0 = sb * SB if isinstance(sb, int) else pl.multiple_of(sb * SB, SB)
    lhs = jnp.concatenate([op[g] for g in range(NG)], axis=1)
    cols = []
    for j in range(NG):
        if before_chunk is not None:
            before_chunk(j)
        lj = lhs
        if overlap is not None and j == fence_at:
            head = jnp.where(never, fence(), lhs[0:8, 0:128])
            top = jnp.concatenate([head, lhs[0:8, 128:]], axis=1)
            lj = jnp.concatenate([top, lhs[8:]], axis=0)
        y = jnp.dot(_as_bf16(lj), _as_bf16(wp[j]), preferred_element_type=F32)
        cols.append(y)
        if overlap is not None and j == 0:
            overlap(y[0:8])
    x = xres[pl.ds(r0, SB), :].astype(F32) + jnp.concatenate(cols, axis=1)
    mean = jnp.sum(x, axis=1, keepdims=True) * (1.0 / D)
    xc = x - mean
    var = jnp.sum(xc * xc, axis=1, keepdims=True) * (1.0 / D)
    rstd = jax.lax.rsqrt(var + EPS)
    y = x * rstd - mean * rstd
    r = jnp.sum(y * wr[...], axis=1, keepdims=True)
    xres[pl.ds(r0, SB), :] = (x + y).astype(BF16)
    for c in range(NG):
        xn[c, pl.ds(r0, SB), :] = y[:, c * 128:(c + 1) * 128].astype(BF16)
    bv = best_v[...]
    bi = best_i[...]
    sub = jax.lax.broadcasted_iota(I32, (8, 1), 0)
    for rg in range(SB // 8):
        rr = r[8 * rg:8 * rg + 8]
        take = rr > bv
        bv = jnp.where(take, rr, bv)
        bi = jnp.where(take, sub + (r0 + 8 * rg), bi)
    best_v[...] = bv
    best_i[...] = bi


def _router_ffn(xn, wg, wu, wd, best_v, best_i):
    bv = best_v[...]
    bi = best_i[...]
    rmax = jnp.max(bv, axis=0, keepdims=True)
    idx = jnp.min(jnp.where(bv == rmax, bi, S))
    grp = idx >> 4
    xp = _packed(xn)
    h0 = pl.multiple_of(grp * 8, 8)
    lhs = _as_bf16(jnp.concatenate(
        [xp[c, pl.ds(h0, 8), :] for c in range(NG)], axis=1))
    wgp, wup, wdp = _packed(wg), _packed(wu), _packed(wd)
    act = []
    for j in range(FF // 128):
        hg = jnp.dot(lhs, _as_bf16(wgp[j]), preferred_element_type=F32)
        hu = jnp.dot(lhs, _as_bf16(wup[j]), preferred_element_type=F32)
        act.append(hg * jax.nn.sigmoid(hg) * hu)
    act = jnp.concatenate(act, axis=1).astype(BF16)
    y = jnp.concatenate(
        [jnp.dot(act, _as_bf16(wdp[j]), preferred_element_type=F32) for j in range(NG)],
        axis=1)
    row = jax.lax.broadcasted_iota(I32, (16, D), 0)
    upd = jnp.where(row == (idx & 15), y * jax.nn.sigmoid(rmax), 0.0)
    return pl.multiple_of(grp * 16, 16), upd


def _kernel(x_hbm, wqkv_hbm, wo_hbm, wr_ref, wg_hbm, wu_hbm, wd_hbm, out_hbm,
            xres, xn, qs, ks, vts, xs, ms, ps, ls, os_, wqkv, wo, wr, wg, wu, wd,
            best_v, best_i, zero, sem_x, sem_q, sem_w, sem_o):
    zero[0] = 0

    x_cp = [pltpu.make_async_copy(x_hbm.at[0, pl.ds(t * TB, TB), :],
                                  xres.at[pl.ds(t * TB, TB), :], sem_x.at[t])
            for t in range(NTB)]
    wqkv_cp = [[pltpu.make_async_copy(wqkv_hbm.at[:, pl.ds(j * 128, 128)],
                                      wqkv.at[j], sem_q.at[k])
                for j in QKV_ORDER[W_START[k]:W_START[k + 1]]]
               for k in range(len(W_GROUPS))]
    wo_cp = [pltpu.make_async_copy(wo_hbm.at[:, pl.ds(j * 128, 128)],
                                   wo.at[j], sem_w.at[0])
             for j in range(NG)]
    ffn_cp = [pltpu.make_async_copy(src.at[:, pl.ds(j * 128, 128)], dst.at[j],
                                    sem_w.at[1])
              for src, dst in ((wg_hbm, wg), (wu_hbm, wu), (wd_hbm, wd))
              for j in range(dst.shape[0])]
    for cp in x_cp[:1] + wqkv_cp[0]:
        cp.start()

    with _scope('init'):
        vts[0:2] = jnp.zeros((2,) + vts.shape[1:], BF16)
        wr[...] = wr_ref[...].astype(F32).reshape(1, D)
    with _scope('xwait'):
        x_cp[0].wait()
    for cp in sum(wqkv_cp[1:W_AHEAD], []) + x_cp[1:2]:
        cp.start()

    def out_copy(r0, n, slot):
        return pltpu.make_async_copy(xres.at[pl.ds(r0, n), :],
                                     out_hbm.at[0, pl.ds(r0, n), :], sem_o.at[slot])

    def layer(l, carry):
        never = jnp.full((8, 128), zero[0], I32) != 0

        with _scope('ln0'):
            _ln_stage(xres, xn, 0)

        @pl.when(l == 0)
        def _():
            def wait_group(n):
                if n in W_START:
                    k = W_START.index(n)
                    for cp in wqkv_cp[k]:
                        cp.wait()
                    if k + W_AHEAD < len(W_GROUPS):
                        for cp in wqkv_cp[k + W_AHEAD]:
                            cp.start()
                    if k == len(W_GROUPS) // 2:
                        x_cp[1].wait()
                    if k == len(W_GROUPS) - 1:
                        for cp in x_cp[2:]:
                            cp.start()

            with _scope('p1_first'):
                _qkv_stage(xn, wqkv, qs, ks, vts, 0, wait_group)
                _ln_stage(xres, xn, 1)

        def wait_x(t):
            @pl.when(l == 0)
            def _():
                pltpu.make_async_copy(
                    x_hbm.at[0, pl.ds(t * TB, TB), :],
                    xres.at[pl.ds(t * TB, TB), :], sem_x.at[t]).wait()

        def p1_step(t, c):
            wait_x(t + 1)

            @pl.when(jnp.logical_and(l == 0, t == 2))
            def _():
                for cp in wo_cp + ffn_cp:
                    cp.start()

            _qkv_stage(xn, wqkv, qs, ks, vts, t)
            _ln_stage(xres, xn, t + 1)
            return c

        with _scope('p1_loop'):
            jax.lax.fori_loop(jnp.where(l == 0, 1, 0), NTB - 1, p1_step, 0)

        best_v[...] = jnp.full((8, 1), -jnp.inf, F32)
        best_i[...] = jnp.zeros((8, 1), I32)

        def pv_all(sb):
            for g in range(NG):
                _unrotate_stage(_pv_stage(ps, ls, vts, sb, g), os_, g)

        def exp_groups(gs, after=None):
            for g in gs:
                _exp_stage(xs, ms, ps, ls, g, never, after)

        def proj(sb, exp_gs=None, **kw):
            if exp_gs is None:
                _proj_stage(os_, wo, wr, xres, xn, best_v, best_i, sb, never, **kw)
            else:
                _proj_stage(os_, wo, wr, xres, xn, best_v, best_i, sb, never,
                            overlap=lambda v: exp_groups(exp_gs, v),
                            fence=lambda: _packed(ps)[zero[0], 0, 0:8, :], **kw)

        def emit_out(sbs):
            @pl.when(l == N_LAYERS - 1)
            def _():
                for sb in sbs:
                    out_copy(sb * SB, SB, sb).start()

        one = zero[0] + 1

        def p1_last(_, c):
            for g in range(NG):
                _score_stage(qs, ks, xs, ms, None, g, static_sb=0)
            exp_groups(range(NG))

            def mid(n):
                if n == P1_LAST_SCORES_AT:
                    for g in range(NG):
                        _score_stage(qs, ks, xs, ms, None, g, static_sb=1)

            _qkv_stage(xn, wqkv, qs, ks, vts, NTB - 1, mid)
            return c

        def steady(s, c):
            pv_all(s - 1)
            exp_groups([0])
            _score_stage(qs, ks, xs, ms, s + 1, 0)
            proj(s - 1, range(1, NG))
            for g in range(1, NG):
                _score_stage(qs, ks, xs, ms, s + 1, g)
            return c

        def post(_, c):
            pv_all(NSB - 2)

            def mid(j):
                if j == POST_PV_AT:
                    pv_all(NSB - 1)

            exp_groups(range(POST_EARLY_EXP))
            proj(NSB - 2, range(POST_EARLY_EXP, NG), fence_at=POST_PV_AT - 1,
                 before_chunk=mid)
            proj(NSB - 1)
            return c

        with _scope('p1_last'):
            jax.lax.fori_loop(0, one, p1_last, 0)

        @pl.when(l == 0)
        def _():
            with _scope('wowait'):
                for cp in wo_cp:
                    cp.wait()

        with _scope('steady'):
            jax.lax.fori_loop(1, NSB - 1, steady, 0)
        emit_out(range(NSB - 2))
        with _scope('post'):
            jax.lax.fori_loop(0, one, post, 0)
        emit_out(range(NSB - 2, NSB))

        @pl.when(l == 0)
        def _():
            with _scope('ffnwait'):
                for cp in ffn_cp:
                    cp.wait()

        with _scope('ffn'):
            g0, upd = _router_ffn(xn, wg, wu, wd, best_v, best_i)

        @pl.when(l == N_LAYERS - 1)
        def _():
            with _scope('owait'):
                for sb in range(NSB):
                    out_copy(sb * SB, SB, sb).wait()

        xres[pl.ds(g0, 16), :] = (
            xres[pl.ds(g0, 16), :].astype(F32) + upd).astype(BF16)

        @pl.when(l == N_LAYERS - 1)
        def _():
            with _scope('ofinal'):
                cp = out_copy(g0, 16, NSB)
                cp.start()
                cp.wait()

        return carry

    jax.lax.fori_loop(0, N_LAYERS, layer, 0)


@jax.jit
def pallas_interleave_layers__sliding_block__moe_arch_mod__prompt_kernel(
    A_x: jax.Array,
    A_wqkv: jax.Array,
    A_wo: jax.Array,
    B_x: jax.Array,
    B_w_r: jax.Array,
    B_w_gate: jax.Array,
    B_w_up: jax.Array,
    B_w_down: jax.Array,
):
    del B_x
    any_spec = pl.BlockSpec(memory_space=pl.ANY)
    scratch = [
        pltpu.VMEM((S, D), BF16),
        pltpu.VMEM((NG, S, 128), BF16),
        pltpu.VMEM((NG, S, 128), BF16),
        pltpu.VMEM((NG, S, 128), BF16),
        pltpu.VMEM((NSB + 2, D, 128), BF16),
        pltpu.VMEM((NG, 4, XR, 128), F32),
        pltpu.VMEM((NG, 4, 8, 128), F32),
        pltpu.VMEM((NG, 4, XR, 128), BF16),
        pltpu.VMEM((NG, 4, 8, 128), F32),
        pltpu.VMEM((NG, SB, 128), BF16),
        pltpu.VMEM((3 * NG, D, 128), BF16),
        pltpu.VMEM((NG, D, 128), BF16),
        pltpu.VMEM((1, D), F32),
        pltpu.VMEM((FF // 128, D, 128), BF16),
        pltpu.VMEM((FF // 128, D, 128), BF16),
        pltpu.VMEM((NG, FF, 128), BF16),
        pltpu.VMEM((8, 1), F32),
        pltpu.VMEM((8, 1), I32),
        pltpu.SMEM((1,), I32),
        pltpu.SemaphoreType.DMA((NTB,)),
        pltpu.SemaphoreType.DMA((len(W_GROUPS),)),
        pltpu.SemaphoreType.DMA((2,)),
        pltpu.SemaphoreType.DMA((NSB + 1,)),
    ]
    return pl.pallas_call(
        _kernel,
        out_shape=jax.ShapeDtypeStruct((1, S, D), BF16),
        in_specs=[any_spec, any_spec, any_spec,
                  pl.BlockSpec(memory_space=pltpu.VMEM),
                  any_spec, any_spec, any_spec],
        out_specs=any_spec,
        scratch_shapes=scratch,
        compiler_params=pltpu.CompilerParams(vmem_limit_bytes=112 * 1024 * 1024),
        name="swa_moe",
    )(A_x, A_wqkv, A_wo, B_w_r, B_w_gate, B_w_up, B_w_down)
```

```python
import math

import jax
import jax.numpy as jnp
import jax.experimental.pallas as pl
import jax.experimental.pallas.tpu as pltpu

F32 = jnp.float32
BF16 = jnp.bfloat16
U32 = jnp.uint32
I32 = jnp.int32

S = 2048
D = 1024
DH = 32
WIN = 256
FF = 3584
NG = 8
SB = 128
NSB = S // SB
QA = 32
XR = WIN + QA
TB = 256
NTB = S // TB
EPS = 1e-5
NEG = -1e30
QSCALE = (DH ** -0.5) * math.log2(math.e)
NT_DIMS = (((1,), (1,)), ((), ()))
N_LAYERS = 2
NFC = FF // 128
KB = 4
NW = 2 * NFC + NG * KB
FS_STEPS = 5
FS_N = 20
FS_BC = 10
FS_LAG = 3
COL_DUMMY = 1 + KB
P1_LAST_SCORES_AT = 16
POST_PV_AT = 7
POST_EARLY_EXP = 1
W_GROUPS = (4, 4, 4, 4, 4, 4)
W_START = [sum(W_GROUPS[:i]) for i in range(len(W_GROUPS) + 1)]
W_AHEAD = 2


def _scope(name):
    return jax.named_scope(name)


def _layernorm(x):
    mean = jnp.sum(x, axis=1, keepdims=True) * (1.0 / D)
    xc = x - mean
    var = jnp.sum(xc * xc, axis=1, keepdims=True) * (1.0 / D)
    return xc * jax.lax.rsqrt(var + EPS)


def _packed(ref):
    return ref.bitcast(U32)


def _as_bf16(v):
    return pltpu.bitcast(v, BF16)


def _ln_stage(xres, xn, t):
    r0 = t * TB if isinstance(t, int) else pl.multiple_of(t * TB, TB)
    y = _layernorm(xres[pl.ds(r0, TB), :].astype(F32))
    for c in range(NG):
        xn[c, pl.ds(r0, TB), :] = y[:, c * 128:(c + 1) * 128].astype(BF16)


QKV_ORDER = list(range(2 * NG, 3 * NG)) + list(range(2 * NG))


def _qkv_stage(xn, wqkv, qs, ks, vts, t, before_chunk=None, after_chunk=None):
    xp = _packed(xn)
    wp = _packed(wqkv)
    if isinstance(t, int):
        r0, h0 = t * TB, t * (TB // 2)
    else:
        r0 = pl.multiple_of(t * TB, TB)
        h0 = pl.multiple_of(t * (TB // 2), TB // 2)
    kt0 = 2 + t * (TB // 128)
    lhs = _as_bf16(jnp.concatenate(
        [xp[c, pl.ds(h0, TB // 2), :] for c in range(NG)], axis=1))
    for n, j in enumerate(QKV_ORDER):
        if before_chunk is not None:
            before_chunk(n)
        y = jnp.dot(lhs, _as_bf16(wp[j]), preferred_element_type=F32)
        if after_chunk is not None:
            after_chunk(n, y[0:8])
        if j < NG:
            qs[j, pl.ds(r0, TB), :] = (y * QSCALE).astype(BF16)
        elif j < 2 * NG:
            ks[j - NG, pl.ds(r0, TB), :] = y.astype(BF16)
        else:
            c = j - 2 * NG
            for t in range(TB // 128):
                vts[kt0 + t, c * 128:(c + 1) * 128, :] = (
                    y[t * 128:(t + 1) * 128, :].T.astype(BF16))


def _score_stage(qs, ks, xs, ms, sb, g, static_sb=None, b=None):
    lane = jax.lax.broadcasted_iota(I32, (QA, 128), 1)
    li = lane % QA
    row = jax.lax.broadcasted_iota(I32, (QA, 128), 0)
    m_lo = row > li
    m_hi = row <= li
    lg = jax.lax.broadcasted_iota(I32, (QA // 2, 128), 1) // QA
    qp = _packed(qs)
    kp = _packed(ks)
    b = g if b is None else b
    for a in range(4):
        if static_sb is None:
            qa2 = pl.multiple_of(sb * (SB // 2) + (QA // 2) * a, QA // 2)
            q = qp[g, pl.ds(qa2, QA // 2), :]
            first = 0
            k = kp[g, pl.ds(qa2 - WIN // 2, XR // 2), :]
        else:
            qa = static_sb * SB + QA * a
            q = qp[g, qa // 2:(qa + QA) // 2, :]
            first = WIN - qa
            k = kp[g, 0:(XR - first) // 2, :]
        qbd = jnp.concatenate(
            [jnp.where(lg == ((a - p) % 4), q, jnp.zeros_like(q)) for p in range(4)],
            axis=0)
        x = jax.lax.dot_general(_as_bf16(k), _as_bf16(qbd), NT_DIMS,
                                preferred_element_type=F32)
        n = XR - first
        hi = jnp.where(m_hi, x[n - QA:n], NEG)
        if first == 0:
            lo = jnp.where(m_lo, x[0:QA], NEG)
            x = jnp.concatenate([lo, x[QA:n - QA], hi], axis=0)
        elif n > QA:
            x = jnp.concatenate(
                [jnp.full((first, 128), NEG, F32), x[0:n - QA], hi], axis=0)
        else:
            x = jnp.concatenate([jnp.full((first, 128), NEG, F32), hi], axis=0)
        xs[b, a] = x
        j0 = first // 16
        m0 = x[16 * j0:16 * j0 + 8]
        m1 = x[16 * j0 + 8:16 * j0 + 16]
        for j in range(j0 + 1, XR // 16):
            m0 = jnp.maximum(m0, x[16 * j:16 * j + 8])
            m1 = jnp.maximum(m1, x[16 * j + 8:16 * j + 16])
        mm = jnp.max(jnp.maximum(m0, m1), axis=0, keepdims=True)
        ms[b, a] = jnp.broadcast_to(mm, (8, 128))
    return m0


def _exp_stage(xs, ms, ps, ls, g, never, after=None):
    for a in range(4):
        m = ms[g, a]
        if after is not None:
            m = jnp.where(never, after, m)
        s0 = s1 = None
        for j in range(XR // 16):
            e0 = jnp.exp2(xs[g, a, 16 * j:16 * j + 8, :] - m)
            e1 = jnp.exp2(xs[g, a, 16 * j + 8:16 * j + 16, :] - m)
            s0 = e0 if s0 is None else s0 + e0
            s1 = e1 if s1 is None else s1 + e1
            if j == XR // 16 - 1:
                s = s0 + s1
                e1 = jnp.where(never, s, e1)
            ps[g, a, 16 * j:16 * j + 16, :] = (
                jnp.concatenate([e0, e1], axis=0).astype(BF16))
        ls[g, a] = s


def _pv_stage(ps, ls, vts, sb, g, b=None):
    lg8 = jax.lax.broadcasted_iota(I32, (8, 128), 1) // QA
    odd = (lg8 % 2) == 1
    hi2 = lg8 >= 2
    zero = jnp.zeros((8, 128), U32)
    pp = _packed(ps)
    vp = _packed(vts)
    b = g if b is None else b

    def sel(c, x, y):
        if x is None and y is None:
            return None
        return jnp.where(c, zero if x is None else x, zero if y is None else y)

    acc = [None] * 4
    for kt in range(3):
        yrows = [[] for _ in range(4)]
        for r in range(8 * kt, 8 * kt + 8):
            pr = []
            for a in range(4):
                j = r - 2 * a
                pr.append(pp[b, a, 8 * j:8 * j + 8, :] if 0 <= j < XR // 16 else None)
            z = [sel(odd, pr[(a + 1) % 4], pr[a]) for a in range(4)]
            for h in range(4):
                y = sel(hi2, z[(h + 2) % 4], z[h])
                yrows[h].append(zero if y is None else y)
        for h in range(4):
            y = _as_bf16(jnp.concatenate(yrows[h], axis=0))
            r0 = (g * 128 + DH * h) // 2
            vt = _as_bf16(vp[sb + kt, r0:r0 + DH // 2, :])
            ot = jnp.dot(vt, y, preferred_element_type=F32)
            acc[h] = ot if acc[h] is None else acc[h] + ot
    l = [jnp.sum(ls[b, a], axis=0, keepdims=True) for a in range(4)]
    lg1 = jax.lax.broadcasted_iota(I32, (1, 128), 1) // QA
    lz = [jnp.where((lg1 % 2) == 1, l[(a + 1) % 4], l[a]) for a in range(4)]
    ly = [jnp.where(lg1 >= 2, lz[(h + 2) % 4], lz[h]) for h in range(4)]
    return jnp.concatenate([acc[h] * (1.0 / ly[h]) for h in range(4)], axis=0)


def _unrotate_stage(ot, os_, g):
    t = ot.T
    lgrp = jax.lax.broadcasted_iota(I32, (QA, 128), 1) // QA
    odd = (lgrp % 2) == 1
    hi2 = lgrp >= 2
    tp = [t[QA * p:QA * p + QA] for p in range(4)]
    z = [jnp.where(odd, tp[(a - 1) % 4], tp[a]) for a in range(4)]
    outs = [jnp.where(hi2, z[(a - 2) % 4], z[a]) for a in range(4)]
    os_[g] = jnp.concatenate(outs, axis=0).astype(BF16)


def _proj_stage(os_, wo, wr, xres, xn, best_v, best_i, sb, never,
                overlap=None, fence=None, fence_at=NG - 1, before_chunk=None):
    op = _packed(os_)
    wp = _packed(wo)
    r0 = sb * SB if isinstance(sb, int) else pl.multiple_of(sb * SB, SB)
    lhs = jnp.concatenate([op[g] for g in range(NG)], axis=1)
    cols = []
    for j in range(NG):
        if before_chunk is not None:
            before_chunk(j)
        lj = lhs
        if overlap is not None and j == fence_at:
            head = jnp.where(never, fence(), lhs[0:8, 0:128])
            top = jnp.concatenate([head, lhs[0:8, 128:]], axis=1)
            lj = jnp.concatenate([top, lhs[8:]], axis=0)
        y = jnp.dot(_as_bf16(lj), _as_bf16(wp[j]), preferred_element_type=F32)
        cols.append(y)
        if overlap is not None and j == 0:
            overlap(y[0:8])
    x = xres[pl.ds(r0, SB), :].astype(F32) + jnp.concatenate(cols, axis=1)
    mean = jnp.sum(x, axis=1, keepdims=True) * (1.0 / D)
    xc = x - mean
    var = jnp.sum(xc * xc, axis=1, keepdims=True) * (1.0 / D)
    rstd = jax.lax.rsqrt(var + EPS)
    y = x * rstd - mean * rstd
    r = jnp.sum(y * wr[...], axis=1, keepdims=True)
    xres[pl.ds(r0, SB), :] = (x + y).astype(BF16)
    for c in range(NG):
        xn[c, pl.ds(r0, SB), :] = y[:, c * 128:(c + 1) * 128].astype(BF16)
    bv = best_v[...]
    bi = best_i[...]
    sub = jax.lax.broadcasted_iota(I32, (8, 1), 0)
    for rg in range(SB // 8):
        rr = r[8 * rg:8 * rg + 8]
        take = rr > bv
        bv = jnp.where(take, rr, bv)
        bi = jnp.where(take, sub + (r0 + 8 * rg), bi)
    best_v[...] = bv
    best_i[...] = bi


def _wd_idx(j, kb):
    return 2 * NFC + KB * j + kb


def _router(best_v, best_i):
    bv = best_v[...]
    rmax = jnp.max(bv, axis=0, keepdims=True)
    idx = jnp.min(jnp.where(bv == rmax, best_i[...], S))
    return rmax, idx


def _row_group(xn, idx):
    h0 = pl.multiple_of((idx >> 4) * 8, 8)
    xp = _packed(xn)
    return _as_bf16(jnp.concatenate(
        [xp[c, pl.ds(h0, 8), :] for c in range(NG)], axis=1))


def _add_to_row(xres, idx, y):
    g0 = pl.multiple_of((idx >> 4) * 16, 16)
    row = jax.lax.broadcasted_iota(I32, (16, D), 0)
    upd = jnp.where(row == (idx & 15), y, 0.0)
    xres[pl.ds(g0, 16), :] = (xres[pl.ds(g0, 16), :].astype(F32) + upd).astype(BF16)
    return g0


def _ffn_mxu(lhs, wffn):
    wp = _packed(wffn)
    act = []
    for j in range(NFC):
        hg = jnp.dot(lhs, _as_bf16(wp[j]), preferred_element_type=F32)
        hu = jnp.dot(lhs, _as_bf16(wp[NFC + j]), preferred_element_type=F32)
        act.append(hg * jax.nn.sigmoid(hg) * hu)
    act = jnp.concatenate(act, axis=1).astype(BF16)
    cols = []
    for j in range(NG):
        w = jnp.concatenate(
            [wp[_wd_idx(j, kb), 0:(min(FF, (kb + 1) * D) - kb * D) // 2, :]
             for kb in range(KB)], axis=0)
        cols.append(jnp.dot(act, _as_bf16(w), preferred_element_type=F32))
    return jnp.concatenate(cols, axis=1)


def _bcast_cols(row):
    return jnp.broadcast_to(row, (128, 128)).T


def _matvec_chunk(wffn, w, col, c, never, after):
    wp = _packed(wffn)
    acc = None
    for g in range(D // 16):
        v = wp[w, 8 * g:8 * g + 8, :]
        if g == 0:
            v = jnp.where(never, pltpu.bitcast(after, U32), v)
        t = _as_bf16(v).astype(F32) * col[c, 16 * g:16 * g + 16, :]
        acc = t if acc is None else acc + t
    return acc[0:8] + acc[8:16]


def _fs_tables():
    mv, bc = [], []
    for k in range(FS_STEPS):
        for n in range(FS_N):
            if k < 3:
                j = FS_BC * k + n % FS_BC
                w = min(j, NFC - 1) + (NFC if n >= FS_BC else 0)
                mv.append((w, 0, w if j < NFC else NW))
            else:
                j, kb = (n % 16) // 2, 2 * (k - 3) + n % 2
                w = _wd_idx(j, kb)
                mv.append((w, 1 + kb, w if n < 16 else NW))
        for m in range(FS_BC):
            j = FS_BC * (k - 1) + m
            if 1 <= k <= 3 and j < NFC:
                bc.append((j, 1 + j // NG, j % NG))
            else:
                bc.append((m, COL_DUMMY, m % NG))
    return mv, bc


def _kernel(x_hbm, wqkv_hbm, wo_hbm, wr_ref, wg_hbm, wu_hbm, wd_hbm, out_hbm,
            xres, xn, qs, ks, vts, xs, ms, ps, ls, os_, wqkv, wo, wr, wffn, col, hp, gate,
            best_v, best_i, zero, order, sel, tab, sem_x, sem_q, sem_w, sem_o):
    zero[0] = 0

    x_cp = [pltpu.make_async_copy(x_hbm.at[0, pl.ds(t * TB, TB), :],
                                  xres.at[pl.ds(t * TB, TB), :], sem_x.at[t])
            for t in range(NTB)]
    wqkv_cp = [[pltpu.make_async_copy(wqkv_hbm.at[:, pl.ds(j * 128, 128)],
                                      wqkv.at[j], sem_q.at[k])
                for j in QKV_ORDER[W_START[k]:W_START[k + 1]]]
               for k in range(len(W_GROUPS))]
    wo_cp = [pltpu.make_async_copy(wo_hbm.at[:, pl.ds(j * 128, 128)],
                                   wo.at[j], sem_w.at[0])
             for j in range(NG)]
    ffn_cp = [pltpu.make_async_copy(src.at[:, pl.ds(j * 128, 128)],
                                    wffn.at[off + j], sem_w.at[1])
              for src, off in ((wg_hbm, 0), (wu_hbm, NFC)) for j in range(NFC)]
    for j in range(NG):
        for kb in range(KB):
            rows = min(FF, (kb + 1) * D) - kb * D
            ffn_cp.append(pltpu.make_async_copy(
                wd_hbm.at[pl.ds(kb * D, rows), pl.ds(j * 128, 128)],
                wffn.at[_wd_idx(j, kb), pl.ds(0, rows), :], sem_w.at[1]))
    for cp in x_cp[:1] + wqkv_cp[0]:
        cp.start()

    with _scope('init'):
        vts[0:2] = jnp.zeros((2,) + vts.shape[1:], BF16)
        wr[...] = wr_ref[...].astype(F32).reshape(1, D)
        pad = KB * D - FF
        for j in range(NG):
            wffn[_wd_idx(j, KB - 1), D - pad:D, :] = jnp.zeros((pad, 128), BF16)
        col[KB, D - pad:D, :] = jnp.zeros((pad, 128), F32)
        hp[...] = jnp.zeros(hp.shape, F32)
        for t in range(NTB):
            order[t] = t
        mv_tab, bc_tab = _fs_tables()
        for i, v in enumerate(sum(mv_tab + bc_tab, ())):
            tab[i] = v
    with _scope('xwait'):
        x_cp[0].wait()
    for cp in sum(wqkv_cp[1:W_AHEAD], []) + x_cp[1:2]:
        cp.start()

    def out_copy(r0, n, slot):
        return pltpu.make_async_copy(xres.at[pl.ds(r0, n), :],
                                     out_hbm.at[0, pl.ds(r0, n), :], sem_o.at[slot])

    def layer(l, carry):
        never = jnp.full((8, 128), zero[0], I32) != 0

        with _scope('ln0'):
            _ln_stage(xres, xn, order[0])

        @pl.when(l == 0)
        def _():
            def wait_group(n):
                if n in W_START:
                    k = W_START.index(n)
                    for cp in wqkv_cp[k]:
                        cp.wait()
                    if k + W_AHEAD < len(W_GROUPS):
                        for cp in wqkv_cp[k + W_AHEAD]:
                            cp.start()
                    if k == len(W_GROUPS) // 2:
                        x_cp[1].wait()
                    if k == len(W_GROUPS) - 1:
                        for cp in x_cp[2:]:
                            cp.start()

            with _scope('p1_first'):
                _qkv_stage(xn, wqkv, qs, ks, vts, 0, wait_group)
                _ln_stage(xres, xn, 1)

        def wait_x(t):
            @pl.when(l == 0)
            def _():
                pltpu.make_async_copy(
                    x_hbm.at[0, pl.ds(t * TB, TB), :],
                    xres.at[pl.ds(t * TB, TB), :], sem_x.at[t]).wait()

        def p1_step(k, c):
            wait_x(k + 1)

            @pl.when(jnp.logical_and(l == 0, k == 2))
            def _():
                for cp in wo_cp + ffn_cp[:2 * NFC]:
                    cp.start()

            @pl.when(jnp.logical_and(l == 0, k == 5))
            def _():
                for cp in ffn_cp[2 * NFC:]:
                    cp.start()

            _qkv_stage(xn, wqkv, qs, ks, vts, order[k])
            _ln_stage(xres, xn, order[k + 1])
            return c

        def fs_step(k, c):
            b0 = 3 * (FS_STEPS * FS_N + k * FS_BC)
            for m in range(FS_BC):
                j, cs, rb = (tab[b0 + 3 * m + i] for i in range(3))
                hg = jnp.sum(hp[j], axis=0, keepdims=True)
                hu = jnp.sum(hp[NFC + j], axis=0, keepdims=True)
                a = (hg * jax.nn.sigmoid(hg) * hu).astype(BF16).astype(F32)
                col[cs, pl.ds(pl.multiple_of(rb * 128, 128), 128), :] = _bcast_cols(a)

            def matvec(n, y):
                n -= FS_LAG
                if 0 <= n < FS_N:
                    w, cs, slot = (tab[3 * (k * FS_N + n) + i] for i in range(3))
                    hp[slot] = _matvec_chunk(wffn, w, col, cs, never, y)

            _qkv_stage(xn, wqkv, qs, ks, vts, order[k], after_chunk=matvec)
            _ln_stage(xres, xn, order[k + 1])
            return c

        @pl.when(l == 1)
        def _():
            with _scope('fs_loop'):
                jax.lax.fori_loop(0, FS_STEPS, fs_step, 0)
            with _scope('fs_fin'):
                y = jnp.concatenate(
                    [jnp.sum(sum(hp[_wd_idx(j, kb)] for kb in range(KB)),
                             axis=0, keepdims=True) for j in range(NG)], axis=1)
                _add_to_row(xres, sel[0], y * gate[...])

        with _scope('p1_loop'):
            jax.lax.fori_loop(jnp.where(l == 0, 1, FS_STEPS), NTB - 1, p1_step, 0)

        best_v[...] = jnp.full((8, 1), -jnp.inf, F32)
        best_i[...] = jnp.zeros((8, 1), I32)

        def pv_all(sb):
            for g in range(NG):
                _unrotate_stage(_pv_stage(ps, ls, vts, sb, g), os_, g)

        def exp_groups(gs, after=None):
            for g in gs:
                _exp_stage(xs, ms, ps, ls, g, never, after)

        def proj(sb, exp_gs=None, **kw):
            if exp_gs is None:
                _proj_stage(os_, wo, wr, xres, xn, best_v, best_i, sb, never, **kw)
            else:
                _proj_stage(os_, wo, wr, xres, xn, best_v, best_i, sb, never,
                            overlap=lambda v: exp_groups(exp_gs, v),
                            fence=lambda: _packed(ps)[zero[0], 0, 0:8, :], **kw)

        def emit_out(sbs):
            @pl.when(l == N_LAYERS - 1)
            def _():
                for sb in sbs:
                    out_copy(sb * SB, SB, sb).start()

        one = zero[0] + 1

        def p1_last(_, c):
            for g in range(NG):
                _score_stage(qs, ks, xs, ms, None, g, static_sb=0)
            exp_groups(range(NG))

            def mid(n):
                if n == P1_LAST_SCORES_AT:
                    for g in range(NG):
                        _score_stage(qs, ks, xs, ms, None, g, static_sb=1)

            _qkv_stage(xn, wqkv, qs, ks, vts, NTB - 1, mid)
            return c

        def steady(s, c):
            pv_all(s - 1)
            exp_groups([0])
            _score_stage(qs, ks, xs, ms, s + 1, 0)
            proj(s - 1, range(1, NG))
            for g in range(1, NG):
                _score_stage(qs, ks, xs, ms, s + 1, g)
            return c

        def post(_, c):
            pv_all(NSB - 2)

            def mid(j):
                if j == POST_PV_AT:
                    pv_all(NSB - 1)

            exp_groups(range(POST_EARLY_EXP))
            proj(NSB - 2, range(POST_EARLY_EXP, NG), fence_at=POST_PV_AT - 1,
                 before_chunk=mid)
            proj(NSB - 1)
            return c

        with _scope('p1_last'):
            jax.lax.fori_loop(0, one, p1_last, 0)

        @pl.when(l == 0)
        def _():
            with _scope('wowait'):
                for cp in wo_cp:
                    cp.wait()

        with _scope('steady'):
            jax.lax.fori_loop(1, NSB - 1, steady, 0)
        emit_out(range(NSB - 2))
        with _scope('post'):
            jax.lax.fori_loop(0, one, post, 0)
        emit_out(range(NSB - 2, NSB))

        rmax, idx = _router(best_v, best_i)
        lhs = _row_group(xn, idx)

        @pl.when(l == 0)
        def _():
            with _scope('route'):
                for cp in ffn_cp:
                    cp.wait()
                sel[0] = idx
                gate[...] = jax.nn.sigmoid(rmax)
                row = jax.lax.broadcasted_iota(I32, (16, D), 0)
                x = jnp.sum(jnp.where(row == (idx & 15), lhs.astype(F32), 0.0),
                            axis=0, keepdims=True)
                for c in range(NG):
                    col[0, c * 128:(c + 1) * 128, :] = _bcast_cols(
                        x[:, c * 128:(c + 1) * 128])
                t_idx = idx // TB
                for p in range(NTB - 2):
                    order[p] = p + (p >= t_idx).astype(I32)
                order[NTB - 2] = jnp.minimum(t_idx, NTB - 2)

        @pl.when(l == N_LAYERS - 1)
        def _():
            with _scope('ffn'):
                y = _ffn_mxu(lhs, wffn) * jax.nn.sigmoid(rmax)
                for sb in range(NSB):
                    out_copy(sb * SB, SB, sb).wait()
                g0 = _add_to_row(xres, idx, y)
            with _scope('ofinal'):
                cp = out_copy(g0, 16, NSB)
                cp.start()
                cp.wait()

        return carry

    jax.lax.fori_loop(0, N_LAYERS, layer, 0)


@jax.jit
def pallas_interleave_layers__sliding_block__moe_arch_mod__prompt_kernel(
    A_x: jax.Array,
    A_wqkv: jax.Array,
    A_wo: jax.Array,
    B_x: jax.Array,
    B_w_r: jax.Array,
    B_w_gate: jax.Array,
    B_w_up: jax.Array,
    B_w_down: jax.Array,
):
    del B_x
    any_spec = pl.BlockSpec(memory_space=pl.ANY)
    scratch = [
        pltpu.VMEM((S, D), BF16),
        pltpu.VMEM((NG, S, 128), BF16),
        pltpu.VMEM((NG, S, 128), BF16),
        pltpu.VMEM((NG, S, 128), BF16),
        pltpu.VMEM((NSB + 2, D, 128), BF16),
        pltpu.VMEM((NG, 4, XR, 128), F32),
        pltpu.VMEM((NG, 4, 8, 128), F32),
        pltpu.VMEM((NG, 4, XR, 128), BF16),
        pltpu.VMEM((NG, 4, 8, 128), F32),
        pltpu.VMEM((NG, SB, 128), BF16),
        pltpu.VMEM((3 * NG, D, 128), BF16),
        pltpu.VMEM((NG, D, 128), BF16),
        pltpu.VMEM((1, D), F32),
        pltpu.VMEM((NW, D, 128), BF16),
        pltpu.VMEM((COL_DUMMY + 1, D, 128), F32),
        pltpu.VMEM((NW + 1, 8, 128), F32),
        pltpu.VMEM((1, 1), F32),
        pltpu.VMEM((8, 1), F32),
        pltpu.VMEM((8, 1), I32),
        pltpu.SMEM((1,), I32),
        pltpu.SMEM((NTB,), I32),
        pltpu.SMEM((1,), I32),
        pltpu.SMEM((3 * FS_STEPS * (FS_N + FS_BC),), I32),
        pltpu.SemaphoreType.DMA((NTB,)),
        pltpu.SemaphoreType.DMA((len(W_GROUPS),)),
        pltpu.SemaphoreType.DMA((2,)),
        pltpu.SemaphoreType.DMA((NSB + 1,)),
    ]
    return pl.pallas_call(
        _kernel,
        out_shape=jax.ShapeDtypeStruct((1, S, D), BF16),
        in_specs=[any_spec, any_spec, any_spec,
                  pl.BlockSpec(memory_space=pltpu.VMEM),
                  any_spec, any_spec, any_spec],
        out_specs=any_spec,
        scratch_shapes=scratch,
        compiler_params=pltpu.CompilerParams(vmem_limit_bytes=112 * 1024 * 1024),
        name="swa_moe",
    )(A_x, A_wqkv, A_wo, B_w_r, B_w_gate, B_w_up, B_w_down)
```

```python
import math

import jax
import jax.numpy as jnp
import jax.experimental.pallas as pl
import jax.experimental.pallas.tpu as pltpu

F32 = jnp.float32
BF16 = jnp.bfloat16
U32 = jnp.uint32
I32 = jnp.int32

S = 2048
D = 1024
DH = 32
WIN = 256
FF = 3584
NG = 8
SB = 128
NSB = S // SB
QA = 32
XR = WIN + QA
TB = 256
NTB = S // TB
EPS = 1e-5
NEG = -1e30
QSCALE = (DH ** -0.5) * math.log2(math.e)
NT_DIMS = (((1,), (1,)), ((), ()))
N_LAYERS = 2
NFC = FF // 128
KB = 4
NW = 2 * NFC + NG * KB
FS_STEPS = 5
FS_N = 20
FS_BC = 10
FS_LAG = 3
COL_DUMMY = 1 + KB
P1_LAST_SCORES_AT = 16
POST_PV_AT = 7
POST_EARLY_EXP = 1
W_GROUPS = (4, 4, 4, 4, 4, 4)
W_START = [sum(W_GROUPS[:i]) for i in range(len(W_GROUPS) + 1)]
W_AHEAD = 2


def _scope(name):
    return jax.named_scope(name)


def _layernorm(x):
    mean = jnp.sum(x, axis=1, keepdims=True) * (1.0 / D)
    xc = x - mean
    var = jnp.sum(xc * xc, axis=1, keepdims=True) * (1.0 / D)
    return xc * jax.lax.rsqrt(var + EPS)


def _packed(ref):
    return ref.bitcast(U32)


def _as_bf16(v):
    return pltpu.bitcast(v, BF16)


def _ln_stage(xres, xn, t):
    r0 = t * TB if isinstance(t, int) else pl.multiple_of(t * TB, TB)
    y = _layernorm(xres[pl.ds(r0, TB), :].astype(F32))
    for c in range(NG):
        xn[c, pl.ds(r0, TB), :] = y[:, c * 128:(c + 1) * 128].astype(BF16)


QKV_ORDER = list(range(2 * NG, 3 * NG)) + list(range(2 * NG))


FIRST_ORDER = sum(([2 * NG + 2 * i, 2 * NG + 2 * i + 1, 2 * i, 2 * i + 1]
                   for i in range(NG // 2)), []) + list(range(NG, 2 * NG))


def _qkv_stage(xn, wqkv, qs, ks, vts, t, before_chunk=None, after_chunk=None,
               chunk_order=QKV_ORDER):
    xp = _packed(xn)
    wp = _packed(wqkv)
    if isinstance(t, int):
        r0, h0 = t * TB, t * (TB // 2)
    else:
        r0 = pl.multiple_of(t * TB, TB)
        h0 = pl.multiple_of(t * (TB // 2), TB // 2)
    kt0 = 2 + t * (TB // 128)
    lhs = _as_bf16(jnp.concatenate(
        [xp[c, pl.ds(h0, TB // 2), :] for c in range(NG)], axis=1))
    for n, j in enumerate(chunk_order):
        if before_chunk is not None:
            before_chunk(n)
        y = jnp.dot(lhs, _as_bf16(wp[j]), preferred_element_type=F32)
        if after_chunk is not None:
            after_chunk(n, y[0:8])
        if j < NG:
            qs[j, pl.ds(r0, TB), :] = (y * QSCALE).astype(BF16)
        elif j < 2 * NG:
            ks[j - NG, pl.ds(r0, TB), :] = y.astype(BF16)
        else:
            c = j - 2 * NG
            for t in range(TB // 128):
                vts[kt0 + t, c * 128:(c + 1) * 128, :] = (
                    y[t * 128:(t + 1) * 128, :].T.astype(BF16))


def _score_stage(qs, ks, xs, ms, sb, g, static_sb=None, b=None):
    lane = jax.lax.broadcasted_iota(I32, (QA, 128), 1)
    li = lane % QA
    row = jax.lax.broadcasted_iota(I32, (QA, 128), 0)
    m_lo = row > li
    m_hi = row <= li
    lg = jax.lax.broadcasted_iota(I32, (QA // 2, 128), 1) // QA
    qp = _packed(qs)
    kp = _packed(ks)
    b = g if b is None else b
    for a in range(4):
        if static_sb is None:
            qa2 = pl.multiple_of(sb * (SB // 2) + (QA // 2) * a, QA // 2)
            q = qp[g, pl.ds(qa2, QA // 2), :]
            first = 0
            k = kp[g, pl.ds(qa2 - WIN // 2, XR // 2), :]
        else:
            qa = static_sb * SB + QA * a
            q = qp[g, qa // 2:(qa + QA) // 2, :]
            first = WIN - qa
            k = kp[g, 0:(XR - first) // 2, :]
        qbd = jnp.concatenate(
            [jnp.where(lg == ((a - p) % 4), q, jnp.zeros_like(q)) for p in range(4)],
            axis=0)
        x = jax.lax.dot_general(_as_bf16(k), _as_bf16(qbd), NT_DIMS,
                                preferred_element_type=F32)
        n = XR - first
        hi = jnp.where(m_hi, x[n - QA:n], NEG)
        if first == 0:
            lo = jnp.where(m_lo, x[0:QA], NEG)
            x = jnp.concatenate([lo, x[QA:n - QA], hi], axis=0)
        elif n > QA:
            x = jnp.concatenate(
                [jnp.full((first, 128), NEG, F32), x[0:n - QA], hi], axis=0)
        else:
            x = jnp.concatenate([jnp.full((first, 128), NEG, F32), hi], axis=0)
        xs[b, a] = x
        j0 = first // 16
        m0 = x[16 * j0:16 * j0 + 8]
        m1 = x[16 * j0 + 8:16 * j0 + 16]
        for j in range(j0 + 1, XR // 16):
            m0 = jnp.maximum(m0, x[16 * j:16 * j + 8])
            m1 = jnp.maximum(m1, x[16 * j + 8:16 * j + 16])
        mm = jnp.max(jnp.maximum(m0, m1), axis=0, keepdims=True)
        ms[b, a] = jnp.broadcast_to(mm, (8, 128))
    return m0


def _exp_stage(xs, ms, ps, ls, g, never, after=None):
    for a in range(4):
        m = ms[g, a]
        if after is not None:
            m = jnp.where(never, after, m)
        s0 = s1 = None
        for j in range(XR // 16):
            e0 = jnp.exp2(xs[g, a, 16 * j:16 * j + 8, :] - m)
            e1 = jnp.exp2(xs[g, a, 16 * j + 8:16 * j + 16, :] - m)
            s0 = e0 if s0 is None else s0 + e0
            s1 = e1 if s1 is None else s1 + e1
            if j == XR // 16 - 1:
                s = s0 + s1
                e1 = jnp.where(never, s, e1)
            ps[g, a, 16 * j:16 * j + 16, :] = (
                jnp.concatenate([e0, e1], axis=0).astype(BF16))
        ls[g, a] = s


def _pv_stage(ps, ls, vts, sb, g, b=None):
    lg8 = jax.lax.broadcasted_iota(I32, (8, 128), 1) // QA
    odd = (lg8 % 2) == 1
    hi2 = lg8 >= 2
    zero = jnp.zeros((8, 128), U32)
    pp = _packed(ps)
    vp = _packed(vts)
    b = g if b is None else b

    def sel(c, x, y):
        if x is None and y is None:
            return None
        return jnp.where(c, zero if x is None else x, zero if y is None else y)

    acc = [None] * 4
    for kt in range(3):
        yrows = [[] for _ in range(4)]
        for r in range(8 * kt, 8 * kt + 8):
            pr = []
            for a in range(4):
                j = r - 2 * a
                pr.append(pp[b, a, 8 * j:8 * j + 8, :] if 0 <= j < XR // 16 else None)
            z = [sel(odd, pr[(a + 1) % 4], pr[a]) for a in range(4)]
            for h in range(4):
                y = sel(hi2, z[(h + 2) % 4], z[h])
                yrows[h].append(zero if y is None else y)
        for h in range(4):
            y = _as_bf16(jnp.concatenate(yrows[h], axis=0))
            r0 = (g * 128 + DH * h) // 2
            vt = _as_bf16(vp[sb + kt, r0:r0 + DH // 2, :])
            ot = jnp.dot(vt, y, preferred_element_type=F32)
            acc[h] = ot if acc[h] is None else acc[h] + ot
    l = [jnp.sum(ls[b, a], axis=0, keepdims=True) for a in range(4)]
    lg1 = jax.lax.broadcasted_iota(I32, (1, 128), 1) // QA
    lz = [jnp.where((lg1 % 2) == 1, l[(a + 1) % 4], l[a]) for a in range(4)]
    ly = [jnp.where(lg1 >= 2, lz[(h + 2) % 4], lz[h]) for h in range(4)]
    return jnp.concatenate([acc[h] * (1.0 / ly[h]) for h in range(4)], axis=0)


def _unrotate_stage(ot, os_, g):
    t = ot.T
    lgrp = jax.lax.broadcasted_iota(I32, (QA, 128), 1) // QA
    odd = (lgrp % 2) == 1
    hi2 = lgrp >= 2
    tp = [t[QA * p:QA * p + QA] for p in range(4)]
    z = [jnp.where(odd, tp[(a - 1) % 4], tp[a]) for a in range(4)]
    outs = [jnp.where(hi2, z[(a - 2) % 4], z[a]) for a in range(4)]
    os_[g] = jnp.concatenate(outs, axis=0).astype(BF16)


def _proj_stage(os_, wo, wr, xres, xn, best_v, best_i, sb, never,
                overlap=None, fence=None, fence_at=NG - 1, before_chunk=None):
    op = _packed(os_)
    wp = _packed(wo)
    r0 = sb * SB if isinstance(sb, int) else pl.multiple_of(sb * SB, SB)
    lhs = jnp.concatenate([op[g] for g in range(NG)], axis=1)
    cols = []
    for j in range(NG):
        if before_chunk is not None:
            before_chunk(j)
        lj = lhs
        if overlap is not None and j == fence_at:
            head = jnp.where(never, fence(), lhs[0:8, 0:128])
            top = jnp.concatenate([head, lhs[0:8, 128:]], axis=1)
            lj = jnp.concatenate([top, lhs[8:]], axis=0)
        y = jnp.dot(_as_bf16(lj), _as_bf16(wp[j]), preferred_element_type=F32)
        cols.append(y)
        if overlap is not None and j == 0:
            overlap(y[0:8])
    x = xres[pl.ds(r0, SB), :].astype(F32) + jnp.concatenate(cols, axis=1)
    mean = jnp.sum(x, axis=1, keepdims=True) * (1.0 / D)
    xc = x - mean
    var = jnp.sum(xc * xc, axis=1, keepdims=True) * (1.0 / D)
    rstd = jax.lax.rsqrt(var + EPS)
    y = x * rstd - mean * rstd
    r = jnp.sum(y * wr[...], axis=1, keepdims=True)
    xres[pl.ds(r0, SB), :] = (x + y).astype(BF16)
    for c in range(NG):
        xn[c, pl.ds(r0, SB), :] = y[:, c * 128:(c + 1) * 128].astype(BF16)
    bv = best_v[...]
    bi = best_i[...]
    sub = jax.lax.broadcasted_iota(I32, (8, 1), 0)
    for rg in range(SB // 8):
        rr = r[8 * rg:8 * rg + 8]
        take = rr > bv
        bv = jnp.where(take, rr, bv)
        bi = jnp.where(take, sub + (r0 + 8 * rg), bi)
    best_v[...] = bv
    best_i[...] = bi


def _wd_idx(j, kb):
    return 2 * NFC + KB * j + kb


def _router(best_v, best_i):
    bv = best_v[...]
    rmax = jnp.max(bv, axis=0, keepdims=True)
    idx = jnp.min(jnp.where(bv == rmax, best_i[...], S))
    return rmax, idx


def _row_group(xn, idx):
    h0 = pl.multiple_of((idx >> 4) * 8, 8)
    xp = _packed(xn)
    return _as_bf16(jnp.concatenate(
        [xp[c, pl.ds(h0, 8), :] for c in range(NG)], axis=1))


def _add_to_row(xres, idx, y):
    g0 = pl.multiple_of((idx >> 4) * 16, 16)
    row = jax.lax.broadcasted_iota(I32, (16, D), 0)
    upd = jnp.where(row == (idx & 15), y, 0.0)
    xres[pl.ds(g0, 16), :] = (xres[pl.ds(g0, 16), :].astype(F32) + upd).astype(BF16)
    return g0


def _ffn_mxu(lhs, wffn):
    wp = _packed(wffn)
    act = []
    for j in range(NFC):
        hg = jnp.dot(lhs, _as_bf16(wp[j]), preferred_element_type=F32)
        hu = jnp.dot(lhs, _as_bf16(wp[NFC + j]), preferred_element_type=F32)
        act.append(hg * jax.nn.sigmoid(hg) * hu)
    act = jnp.concatenate(act, axis=1).astype(BF16)
    cols = []
    for j in range(NG):
        w = jnp.concatenate(
            [wp[_wd_idx(j, kb), 0:(min(FF, (kb + 1) * D) - kb * D) // 2, :]
             for kb in range(KB)], axis=0)
        cols.append(jnp.dot(act, _as_bf16(w), preferred_element_type=F32))
    return jnp.concatenate(cols, axis=1)


def _bcast_cols(row):
    return jnp.broadcast_to(row, (128, 128)).T


def _matvec_chunk(wffn, w, col, c, never, after):
    wp = _packed(wffn)
    acc = None
    for g in range(D // 16):
        v = wp[w, 8 * g:8 * g + 8, :]
        if g == 0:
            v = jnp.where(never, pltpu.bitcast(after, U32), v)
        t = _as_bf16(v).astype(F32) * col[c, 16 * g:16 * g + 16, :]
        acc = t if acc is None else acc + t
    return acc[0:8] + acc[8:16]


def _fs_tables():
    mv, bc = [], []
    for k in range(FS_STEPS):
        for n in range(FS_N):
            if k < 3:
                j = FS_BC * k + n % FS_BC
                w = min(j, NFC - 1) + (NFC if n >= FS_BC else 0)
                mv.append((w, 0, w if j < NFC else NW))
            else:
                j, kb = (n % 16) // 2, 2 * (k - 3) + n % 2
                w = _wd_idx(j, kb)
                mv.append((w, 1 + kb, w if n < 16 else NW))
        for m in range(FS_BC):
            j = FS_BC * (k - 1) + m
            if 1 <= k <= 3 and j < NFC:
                bc.append((j, 1 + j // NG, j % NG))
            else:
                bc.append((m, COL_DUMMY, m % NG))
    return mv, bc


def _kernel(x_hbm, wqkv_hbm, wo_hbm, wr_ref, wg_hbm, wu_hbm, wd_hbm, out_hbm,
            xres, xn, qs, ks, vts, xs, ms, ps, ls, os_, wqkv, wo, wr, wffn, col, hp, gate,
            best_v, best_i, zero, order, sel, tab, sem_x, sem_q, sem_w, sem_o):
    zero[0] = 0

    x_cp = [pltpu.make_async_copy(x_hbm.at[0, pl.ds(t * TB, TB), :],
                                  xres.at[pl.ds(t * TB, TB), :], sem_x.at[t])
            for t in range(NTB)]
    wqkv_cp = [[pltpu.make_async_copy(wqkv_hbm.at[:, pl.ds(j * 128, 128)],
                                      wqkv.at[j], sem_q.at[k])
                for j in FIRST_ORDER[W_START[k]:W_START[k + 1]]]
               for k in range(len(W_GROUPS))]
    wo_cp = [pltpu.make_async_copy(wo_hbm.at[:, pl.ds(j * 128, 128)],
                                   wo.at[j], sem_w.at[0])
             for j in range(NG)]
    ffn_cp = [pltpu.make_async_copy(src.at[:, pl.ds(j * 128, 128)],
                                    wffn.at[off + j], sem_w.at[1])
              for src, off in ((wg_hbm, 0), (wu_hbm, NFC)) for j in range(NFC)]
    for j in range(NG):
        for kb in range(KB):
            rows = min(FF, (kb + 1) * D) - kb * D
            ffn_cp.append(pltpu.make_async_copy(
                wd_hbm.at[pl.ds(kb * D, rows), pl.ds(j * 128, 128)],
                wffn.at[_wd_idx(j, kb), pl.ds(0, rows), :], sem_w.at[1]))
    for cp in x_cp[:1] + wqkv_cp[0]:
        cp.start()

    with _scope('init'):
        vts[0:2] = jnp.zeros((2,) + vts.shape[1:], BF16)
        wr[...] = wr_ref[...].astype(F32).reshape(1, D)
        pad = KB * D - FF
        for j in range(NG):
            wffn[_wd_idx(j, KB - 1), D - pad:D, :] = jnp.zeros((pad, 128), BF16)
        col[KB, D - pad:D, :] = jnp.zeros((pad, 128), F32)
        hp[...] = jnp.zeros(hp.shape, F32)
        for t in range(NTB):
            order[t] = t
        mv_tab, bc_tab = _fs_tables()
        for i, v in enumerate(sum(mv_tab + bc_tab, ())):
            tab[i] = v
    with _scope('xwait'):
        x_cp[0].wait()
    for cp in sum(wqkv_cp[1:W_AHEAD], []) + x_cp[1:2]:
        cp.start()

    def out_copy(r0, n, slot):
        return pltpu.make_async_copy(xres.at[pl.ds(r0, n), :],
                                     out_hbm.at[0, pl.ds(r0, n), :], sem_o.at[slot])

    def layer(l, carry):
        never = jnp.full((8, 128), zero[0], I32) != 0

        with _scope('ln0'):
            _ln_stage(xres, xn, order[0])

        @pl.when(l == 0)
        def _():
            def wait_group(n):
                if n in W_START:
                    k = W_START.index(n)
                    for cp in wqkv_cp[k]:
                        cp.wait()
                    if k + W_AHEAD < len(W_GROUPS):
                        for cp in wqkv_cp[k + W_AHEAD]:
                            cp.start()
                    if k == len(W_GROUPS) // 2:
                        x_cp[1].wait()
                        _ln_stage(xres, xn, 1)
                    if k == len(W_GROUPS) - 1:
                        for cp in x_cp[2:]:
                            cp.start()

            with _scope('p1_first'):
                _qkv_stage(xn, wqkv, qs, ks, vts, 0, wait_group,
                           chunk_order=FIRST_ORDER)

        def wait_x(t):
            @pl.when(l == 0)
            def _():
                pltpu.make_async_copy(
                    x_hbm.at[0, pl.ds(t * TB, TB), :],
                    xres.at[pl.ds(t * TB, TB), :], sem_x.at[t]).wait()

        def p1_step(k, c):
            wait_x(k + 1)

            @pl.when(jnp.logical_and(l == 0, k == 2))
            def _():
                for cp in wo_cp + ffn_cp[:2 * NFC]:
                    cp.start()

            @pl.when(jnp.logical_and(l == 0, k == 5))
            def _():
                for cp in ffn_cp[2 * NFC:]:
                    cp.start()

            _qkv_stage(xn, wqkv, qs, ks, vts, order[k])
            _ln_stage(xres, xn, order[k + 1])
            return c

        def fs_step(k, c):
            b0 = 3 * (FS_STEPS * FS_N + k * FS_BC)
            for m in range(FS_BC):
                j, cs, rb = (tab[b0 + 3 * m + i] for i in range(3))
                hg = jnp.sum(hp[j], axis=0, keepdims=True)
                hu = jnp.sum(hp[NFC + j], axis=0, keepdims=True)
                a = (hg * jax.nn.sigmoid(hg) * hu).astype(BF16).astype(F32)
                col[cs, pl.ds(pl.multiple_of(rb * 128, 128), 128), :] = _bcast_cols(a)

            def matvec(n, y):
                n -= FS_LAG
                if 0 <= n < FS_N:
                    w, cs, slot = (tab[3 * (k * FS_N + n) + i] for i in range(3))
                    hp[slot] = _matvec_chunk(wffn, w, col, cs, never, y)

            _qkv_stage(xn, wqkv, qs, ks, vts, order[k], after_chunk=matvec)
            _ln_stage(xres, xn, order[k + 1])
            return c

        @pl.when(l == 1)
        def _():
            with _scope('fs_loop'):
                jax.lax.fori_loop(0, FS_STEPS, fs_step, 0)
            with _scope('fs_fin'):
                y = jnp.concatenate(
                    [jnp.sum(sum(hp[_wd_idx(j, kb)] for kb in range(KB)),
                             axis=0, keepdims=True) for j in range(NG)], axis=1)
                _add_to_row(xres, sel[0], y * gate[...])

        with _scope('p1_loop'):
            jax.lax.fori_loop(jnp.where(l == 0, 1, FS_STEPS), NTB - 1, p1_step, 0)

        best_v[...] = jnp.full((8, 1), -jnp.inf, F32)
        best_i[...] = jnp.zeros((8, 1), I32)

        def pv_all(sb):
            for g in range(NG):
                _unrotate_stage(_pv_stage(ps, ls, vts, sb, g), os_, g)

        def exp_groups(gs, after=None):
            for g in gs:
                _exp_stage(xs, ms, ps, ls, g, never, after)

        def proj(sb, exp_gs=None, **kw):
            if exp_gs is None:
                _proj_stage(os_, wo, wr, xres, xn, best_v, best_i, sb, never, **kw)
            else:
                _proj_stage(os_, wo, wr, xres, xn, best_v, best_i, sb, never,
                            overlap=lambda v: exp_groups(exp_gs, v),
                            fence=lambda: _packed(ps)[zero[0], 0, 0:8, :], **kw)

        def emit_out(sbs):
            @pl.when(l == N_LAYERS - 1)
            def _():
                for sb in sbs:
                    out_copy(sb * SB, SB, sb).start()

        one = zero[0] + 1

        def p1_last(_, c):
            for g in range(NG):
                _score_stage(qs, ks, xs, ms, None, g, static_sb=0)
            exp_groups(range(NG))

            def mid(n):
                if n == P1_LAST_SCORES_AT:
                    for g in range(NG):
                        _score_stage(qs, ks, xs, ms, None, g, static_sb=1)

            _qkv_stage(xn, wqkv, qs, ks, vts, NTB - 1, mid)
            return c

        def steady(s, c):
            pv_all(s - 1)
            exp_groups([0])
            _score_stage(qs, ks, xs, ms, s + 1, 0)
            proj(s - 1, range(1, NG))
            for g in range(1, NG):
                _score_stage(qs, ks, xs, ms, s + 1, g)
            return c

        def post(_, c):
            pv_all(NSB - 2)

            def mid(j):
                if j == POST_PV_AT:
                    pv_all(NSB - 1)

            exp_groups(range(POST_EARLY_EXP))
            proj(NSB - 2, range(POST_EARLY_EXP, NG), fence_at=POST_PV_AT - 1,
                 before_chunk=mid)
            proj(NSB - 1)
            return c

        with _scope('p1_last'):
            jax.lax.fori_loop(0, one, p1_last, 0)

        @pl.when(l == 0)
        def _():
            with _scope('wowait'):
                for cp in wo_cp:
                    cp.wait()

        with _scope('steady'):
            jax.lax.fori_loop(1, NSB - 1, steady, 0)
        emit_out(range(NSB - 2))
        with _scope('post'):
            jax.lax.fori_loop(0, one, post, 0)
        emit_out(range(NSB - 2, NSB))

        rmax, idx = _router(best_v, best_i)
        lhs = _row_group(xn, idx)

        @pl.when(l == 0)
        def _():
            with _scope('route'):
                for cp in ffn_cp:
                    cp.wait()
                sel[0] = idx
                gate[...] = jax.nn.sigmoid(rmax)
                row = jax.lax.broadcasted_iota(I32, (16, D), 0)
                x = jnp.sum(jnp.where(row == (idx & 15), lhs.astype(F32), 0.0),
                            axis=0, keepdims=True)
                for c in range(NG):
                    col[0, c * 128:(c + 1) * 128, :] = _bcast_cols(
                        x[:, c * 128:(c + 1) * 128])
                t_idx = idx // TB
                for p in range(NTB - 2):
                    order[p] = p + (p >= t_idx).astype(I32)
                order[NTB - 2] = jnp.minimum(t_idx, NTB - 2)

        @pl.when(l == N_LAYERS - 1)
        def _():
            with _scope('ffn'):
                y = _ffn_mxu(lhs, wffn) * jax.nn.sigmoid(rmax)
                for sb in range(NSB):
                    out_copy(sb * SB, SB, sb).wait()
                g0 = _add_to_row(xres, idx, y)
            with _scope('ofinal'):
                cp = out_copy(g0, 16, NSB)
                cp.start()
                cp.wait()

        return carry

    jax.lax.fori_loop(0, N_LAYERS, layer, 0)


@jax.jit
def pallas_interleave_layers__sliding_block__moe_arch_mod__prompt_kernel(
    A_x: jax.Array,
    A_wqkv: jax.Array,
    A_wo: jax.Array,
    B_x: jax.Array,
    B_w_r: jax.Array,
    B_w_gate: jax.Array,
    B_w_up: jax.Array,
    B_w_down: jax.Array,
):
    del B_x
    any_spec = pl.BlockSpec(memory_space=pl.ANY)
    scratch = [
        pltpu.VMEM((S, D), BF16),
        pltpu.VMEM((NG, S, 128), BF16),
        pltpu.VMEM((NG, S, 128), BF16),
        pltpu.VMEM((NG, S, 128), BF16),
        pltpu.VMEM((NSB + 2, D, 128), BF16),
        pltpu.VMEM((NG, 4, XR, 128), F32),
        pltpu.VMEM((NG, 4, 8, 128), F32),
        pltpu.VMEM((NG, 4, XR, 128), BF16),
        pltpu.VMEM((NG, 4, 8, 128), F32),
        pltpu.VMEM((NG, SB, 128), BF16),
        pltpu.VMEM((3 * NG, D, 128), BF16),
        pltpu.VMEM((NG, D, 128), BF16),
        pltpu.VMEM((1, D), F32),
        pltpu.VMEM((NW, D, 128), BF16),
        pltpu.VMEM((COL_DUMMY + 1, D, 128), F32),
        pltpu.VMEM((NW + 1, 8, 128), F32),
        pltpu.VMEM((1, 1), F32),
        pltpu.VMEM((8, 1), F32),
        pltpu.VMEM((8, 1), I32),
        pltpu.SMEM((1,), I32),
        pltpu.SMEM((NTB,), I32),
        pltpu.SMEM((1,), I32),
        pltpu.SMEM((3 * FS_STEPS * (FS_N + FS_BC),), I32),
        pltpu.SemaphoreType.DMA((NTB,)),
        pltpu.SemaphoreType.DMA((len(W_GROUPS),)),
        pltpu.SemaphoreType.DMA((2,)),
        pltpu.SemaphoreType.DMA((NSB + 1,)),
    ]
    return pl.pallas_call(
        _kernel,
        out_shape=jax.ShapeDtypeStruct((1, S, D), BF16),
        in_specs=[any_spec, any_spec, any_spec,
                  pl.BlockSpec(memory_space=pltpu.VMEM),
                  any_spec, any_spec, any_spec],
        out_specs=any_spec,
        scratch_shapes=scratch,
        compiler_params=pltpu.CompilerParams(vmem_limit_bytes=112 * 1024 * 1024),
        name="swa_moe",
    )(A_x, A_wqkv, A_wo, B_w_r, B_w_gate, B_w_up, B_w_down)
```

```python
import math

import jax
import jax.numpy as jnp
import jax.experimental.pallas as pl
import jax.experimental.pallas.tpu as pltpu

F32 = jnp.float32
BF16 = jnp.bfloat16
U32 = jnp.uint32
I32 = jnp.int32

S = 2048
D = 1024
DH = 32
WIN = 256
FF = 3584
NG = 8
SB = 128
NSB = S // SB
QA = 32
XR = WIN + QA
TB = 256
NTB = S // TB
EPS = 1e-5
NEG = -1e30
QSCALE = (DH ** -0.5) * math.log2(math.e)
NT_DIMS = (((1,), (1,)), ((), ()))
N_LAYERS = 2
NFC = FF // 128
KB = 4
NW = 2 * NFC + NG * KB
FS_STEPS = 5
FS_N = 20
FS_BC = 10
FS_LAG = 3
COL_DUMMY = 1 + KB
FFN_VPU = 8
P1_LAST_SCORES_AT = 16
POST_PV_AT = 7
POST_EARLY_EXP = 1
W_GROUPS = (4, 4, 4, 4, 4, 4)
W_START = [sum(W_GROUPS[:i]) for i in range(len(W_GROUPS) + 1)]
W_AHEAD = 2


def _scope(name):
    return jax.named_scope(name)


def _layernorm(x):
    mean = jnp.sum(x, axis=1, keepdims=True) * (1.0 / D)
    xc = x - mean
    var = jnp.sum(xc * xc, axis=1, keepdims=True) * (1.0 / D)
    return xc * jax.lax.rsqrt(var + EPS)


def _packed(ref):
    return ref.bitcast(U32)


def _as_bf16(v):
    return pltpu.bitcast(v, BF16)


def _ln_stage(xres, xn, t):
    r0 = t * TB if isinstance(t, int) else pl.multiple_of(t * TB, TB)
    y = _layernorm(xres[pl.ds(r0, TB), :].astype(F32))
    for c in range(NG):
        xn[c, pl.ds(r0, TB), :] = y[:, c * 128:(c + 1) * 128].astype(BF16)


QKV_ORDER = list(range(2 * NG, 3 * NG)) + list(range(2 * NG))


FIRST_ORDER = sum(([2 * NG + 2 * i, 2 * NG + 2 * i + 1, 2 * i, 2 * i + 1]
                   for i in range(NG // 2)), []) + list(range(NG, 2 * NG))


def _qkv_stage(xn, wqkv, qs, ks, vts, t, before_chunk=None, after_chunk=None,
               chunk_order=QKV_ORDER):
    xp = _packed(xn)
    wp = _packed(wqkv)
    if isinstance(t, int):
        r0, h0 = t * TB, t * (TB // 2)
    else:
        r0 = pl.multiple_of(t * TB, TB)
        h0 = pl.multiple_of(t * (TB // 2), TB // 2)
    kt0 = 2 + t * (TB // 128)
    lhs = _as_bf16(jnp.concatenate(
        [xp[c, pl.ds(h0, TB // 2), :] for c in range(NG)], axis=1))
    for n, j in enumerate(chunk_order):
        if before_chunk is not None:
            before_chunk(n)
        y = jnp.dot(lhs, _as_bf16(wp[j]), preferred_element_type=F32)
        if after_chunk is not None:
            after_chunk(n, y[0:8])
        if j < NG:
            qs[j, pl.ds(r0, TB), :] = (y * QSCALE).astype(BF16)
        elif j < 2 * NG:
            ks[j - NG, pl.ds(r0, TB), :] = y.astype(BF16)
        else:
            c = j - 2 * NG
            for t in range(TB // 128):
                vts[kt0 + t, c * 128:(c + 1) * 128, :] = (
                    y[t * 128:(t + 1) * 128, :].T.astype(BF16))


def _score_stage(qs, ks, xs, ms, sb, g, static_sb=None, b=None):
    lane = jax.lax.broadcasted_iota(I32, (QA, 128), 1)
    li = lane % QA
    row = jax.lax.broadcasted_iota(I32, (QA, 128), 0)
    m_lo = row > li
    m_hi = row <= li
    lg = jax.lax.broadcasted_iota(I32, (QA // 2, 128), 1) // QA
    qp = _packed(qs)
    kp = _packed(ks)
    b = g if b is None else b
    for a in range(4):
        if static_sb is None:
            qa2 = pl.multiple_of(sb * (SB // 2) + (QA // 2) * a, QA // 2)
            q = qp[g, pl.ds(qa2, QA // 2), :]
            first = 0
            k = kp[g, pl.ds(qa2 - WIN // 2, XR // 2), :]
        else:
            qa = static_sb * SB + QA * a
            q = qp[g, qa // 2:(qa + QA) // 2, :]
            first = WIN - qa
            k = kp[g, 0:(XR - first) // 2, :]
        qbd = jnp.concatenate(
            [jnp.where(lg == ((a - p) % 4), q, jnp.zeros_like(q)) for p in range(4)],
            axis=0)
        x = jax.lax.dot_general(_as_bf16(k), _as_bf16(qbd), NT_DIMS,
                                preferred_element_type=F32)
        n = XR - first
        hi = jnp.where(m_hi, x[n - QA:n], NEG)
        if first == 0:
            lo = jnp.where(m_lo, x[0:QA], NEG)
            x = jnp.concatenate([lo, x[QA:n - QA], hi], axis=0)
        elif n > QA:
            x = jnp.concatenate(
                [jnp.full((first, 128), NEG, F32), x[0:n - QA], hi], axis=0)
        else:
            x = jnp.concatenate([jnp.full((first, 128), NEG, F32), hi], axis=0)
        xs[b, a] = x
        j0 = first // 16
        m0 = x[16 * j0:16 * j0 + 8]
        m1 = x[16 * j0 + 8:16 * j0 + 16]
        for j in range(j0 + 1, XR // 16):
            m0 = jnp.maximum(m0, x[16 * j:16 * j + 8])
            m1 = jnp.maximum(m1, x[16 * j + 8:16 * j + 16])
        mm = jnp.max(jnp.maximum(m0, m1), axis=0, keepdims=True)
        ms[b, a] = jnp.broadcast_to(mm, (8, 128))
    return m0


def _exp_stage(xs, ms, ps, ls, g, never, after=None):
    for a in range(4):
        m = ms[g, a]
        if after is not None:
            m = jnp.where(never, after, m)
        s0 = s1 = None
        for j in range(XR // 16):
            e0 = jnp.exp2(xs[g, a, 16 * j:16 * j + 8, :] - m)
            e1 = jnp.exp2(xs[g, a, 16 * j + 8:16 * j + 16, :] - m)
            s0 = e0 if s0 is None else s0 + e0
            s1 = e1 if s1 is None else s1 + e1
            if j == XR // 16 - 1:
                s = s0 + s1
                e1 = jnp.where(never, s, e1)
            ps[g, a, 16 * j:16 * j + 16, :] = (
                jnp.concatenate([e0, e1], axis=0).astype(BF16))
        ls[g, a] = s


def _pv_stage(ps, ls, vts, sb, g, b=None):
    lg8 = jax.lax.broadcasted_iota(I32, (8, 128), 1) // QA
    odd = (lg8 % 2) == 1
    hi2 = lg8 >= 2
    zero = jnp.zeros((8, 128), U32)
    pp = _packed(ps)
    vp = _packed(vts)
    b = g if b is None else b

    def sel(c, x, y):
        if x is None and y is None:
            return None
        return jnp.where(c, zero if x is None else x, zero if y is None else y)

    acc = [None] * 4
    for kt in range(3):
        yrows = [[] for _ in range(4)]
        for r in range(8 * kt, 8 * kt + 8):
            pr = []
            for a in range(4):
                j = r - 2 * a
                pr.append(pp[b, a, 8 * j:8 * j + 8, :] if 0 <= j < XR // 16 else None)
            z = [sel(odd, pr[(a + 1) % 4], pr[a]) for a in range(4)]
            for h in range(4):
                y = sel(hi2, z[(h + 2) % 4], z[h])
                yrows[h].append(zero if y is None else y)
        for h in range(4):
            y = _as_bf16(jnp.concatenate(yrows[h], axis=0))
            r0 = (g * 128 + DH * h) // 2
            vt = _as_bf16(vp[sb + kt, r0:r0 + DH // 2, :])
            ot = jnp.dot(vt, y, preferred_element_type=F32)
            acc[h] = ot if acc[h] is None else acc[h] + ot
    l = [jnp.sum(ls[b, a], axis=0, keepdims=True) for a in range(4)]
    lg1 = jax.lax.broadcasted_iota(I32, (1, 128), 1) // QA
    lz = [jnp.where((lg1 % 2) == 1, l[(a + 1) % 4], l[a]) for a in range(4)]
    ly = [jnp.where(lg1 >= 2, lz[(h + 2) % 4], lz[h]) for h in range(4)]
    return jnp.concatenate([acc[h] * (1.0 / ly[h]) for h in range(4)], axis=0)


def _unrotate_stage(ot, os_, g):
    t = ot.T
    lgrp = jax.lax.broadcasted_iota(I32, (QA, 128), 1) // QA
    odd = (lgrp % 2) == 1
    hi2 = lgrp >= 2
    tp = [t[QA * p:QA * p + QA] for p in range(4)]
    z = [jnp.where(odd, tp[(a - 1) % 4], tp[a]) for a in range(4)]
    outs = [jnp.where(hi2, z[(a - 2) % 4], z[a]) for a in range(4)]
    os_[g] = jnp.concatenate(outs, axis=0).astype(BF16)


def _proj_stage(os_, wo, wr, xres, xn, best_v, best_i, sb, never,
                overlap=None, fence=None, fence_at=NG - 1, before_chunk=None):
    op = _packed(os_)
    wp = _packed(wo)
    r0 = sb * SB if isinstance(sb, int) else pl.multiple_of(sb * SB, SB)
    lhs = jnp.concatenate([op[g] for g in range(NG)], axis=1)
    cols = []
    for j in range(NG):
        if before_chunk is not None:
            before_chunk(j)
        lj = lhs
        if overlap is not None and j == fence_at:
            head = jnp.where(never, fence(), lhs[0:8, 0:128])
            top = jnp.concatenate([head, lhs[0:8, 128:]], axis=1)
            lj = jnp.concatenate([top, lhs[8:]], axis=0)
        y = jnp.dot(_as_bf16(lj), _as_bf16(wp[j]), preferred_element_type=F32)
        cols.append(y)
        if overlap is not None and j == 0:
            overlap(y[0:8])
    x = xres[pl.ds(r0, SB), :].astype(F32) + jnp.concatenate(cols, axis=1)
    mean = jnp.sum(x, axis=1, keepdims=True) * (1.0 / D)
    xc = x - mean
    var = jnp.sum(xc * xc, axis=1, keepdims=True) * (1.0 / D)
    rstd = jax.lax.rsqrt(var + EPS)
    y = x * rstd - mean * rstd
    r = jnp.sum(y * wr[...], axis=1, keepdims=True)
    xres[pl.ds(r0, SB), :] = (x + y).astype(BF16)
    for c in range(NG):
        xn[c, pl.ds(r0, SB), :] = y[:, c * 128:(c + 1) * 128].astype(BF16)
    bv = best_v[...]
    bi = best_i[...]
    sub = jax.lax.broadcasted_iota(I32, (8, 1), 0)
    for rg in range(SB // 8):
        rr = r[8 * rg:8 * rg + 8]
        take = rr > bv
        bv = jnp.where(take, rr, bv)
        bi = jnp.where(take, sub + (r0 + 8 * rg), bi)
    best_v[...] = bv
    best_i[...] = bi


def _wd_idx(j, kb):
    return 2 * NFC + KB * j + kb


def _router(best_v, best_i):
    bv = best_v[...]
    rmax = jnp.max(bv, axis=0, keepdims=True)
    idx = jnp.min(jnp.where(bv == rmax, best_i[...], S))
    return rmax, idx


def _row_group(xn, idx):
    h0 = pl.multiple_of((idx >> 4) * 8, 8)
    xp = _packed(xn)
    return _as_bf16(jnp.concatenate(
        [xp[c, pl.ds(h0, 8), :] for c in range(NG)], axis=1))


def _add_to_row(xres, idx, y):
    g0 = pl.multiple_of((idx >> 4) * 16, 16)
    row = jax.lax.broadcasted_iota(I32, (16, D), 0)
    upd = jnp.where(row == (idx & 15), y, 0.0)
    xres[pl.ds(g0, 16), :] = (xres[pl.ds(g0, 16), :].astype(F32) + upd).astype(BF16)
    return g0


def _select_row(v, idx):
    row = jax.lax.broadcasted_iota(I32, v.shape, 0)
    return jnp.sum(jnp.where(row == (idx & 15), v, 0.0), axis=0, keepdims=True)


def _store_x_cols(col, lhs, idx):
    x = _select_row(lhs.astype(F32), idx)
    for c in range(NG):
        col[0, c * 128:(c + 1) * 128, :] = _bcast_cols(x[:, c * 128:(c + 1) * 128])


def _ffn_last(lhs, idx, wffn, col, never):
    wp = _packed(wffn)
    _store_x_cols(col, lhs, idx)
    todo = [(j, u) for j in range(NFC - FFN_VPU, NFC) for u in range(2)]
    h = {}
    n = 0
    for j in range(NFC - FFN_VPU):
        for u in range(2):
            y = jnp.dot(lhs, _as_bf16(wp[u * NFC + j]), preferred_element_type=F32)
            h[j, u] = _select_row(y, idx)
            if n >= 4 and n % 2 == 0 and todo:
                jj, uu = todo.pop(0)
                part = _matvec_chunk(wffn, uu * NFC + jj, col, 0, never, y[0:8])
                h[jj, uu] = jnp.sum(part, axis=0, keepdims=True)
            n += 1
    assert not todo
    act = jnp.concatenate(
        [h[j, 0] * jax.nn.sigmoid(h[j, 0]) * h[j, 1] for j in range(NFC)], axis=1)
    act = jnp.broadcast_to(act, (16, FF)).astype(BF16)
    cols = []
    for j in range(NG):
        w = jnp.concatenate(
            [wp[_wd_idx(j, kb), 0:(min(FF, (kb + 1) * D) - kb * D) // 2, :]
             for kb in range(KB)], axis=0)
        cols.append(jnp.dot(act, _as_bf16(w), preferred_element_type=F32)[0:1])
    return jnp.concatenate(cols, axis=1)


def _bcast_cols(row):
    return jnp.broadcast_to(row, (128, 128)).T


def _matvec_chunk(wffn, w, col, c, never, after):
    wp = _packed(wffn)
    acc = None
    for g in range(D // 16):
        v = wp[w, 8 * g:8 * g + 8, :]
        if g == 0:
            v = jnp.where(never, pltpu.bitcast(after, U32), v)
        t = _as_bf16(v).astype(F32) * col[c, 16 * g:16 * g + 16, :]
        acc = t if acc is None else acc + t
    return acc[0:8] + acc[8:16]


def _fs_tables():
    mv, bc = [], []
    for k in range(FS_STEPS):
        for n in range(FS_N):
            if k < 3:
                j = FS_BC * k + n % FS_BC
                w = min(j, NFC - 1) + (NFC if n >= FS_BC else 0)
                mv.append((w, 0, w if j < NFC else NW))
            else:
                j, kb = (n % 16) // 2, 2 * (k - 3) + n % 2
                w = _wd_idx(j, kb)
                mv.append((w, 1 + kb, w if n < 16 else NW))
        for m in range(FS_BC):
            j = FS_BC * (k - 1) + m
            if 1 <= k <= 3 and j < NFC:
                bc.append((j, 1 + j // NG, j % NG))
            else:
                bc.append((m, COL_DUMMY, m % NG))
    return mv, bc


def _kernel(x_hbm, wqkv_hbm, wo_hbm, wr_ref, wg_hbm, wu_hbm, wd_hbm, out_hbm,
            xres, xn, qs, ks, vts, xs, ms, ps, ls, os_, wqkv, wo, wr, wffn, col, hp, gate,
            best_v, best_i, zero, order, sel, tab, sem_x, sem_q, sem_w, sem_o):
    zero[0] = 0

    x_cp = [pltpu.make_async_copy(x_hbm.at[0, pl.ds(t * TB, TB), :],
                                  xres.at[pl.ds(t * TB, TB), :], sem_x.at[t])
            for t in range(NTB)]
    wqkv_cp = [[pltpu.make_async_copy(wqkv_hbm.at[:, pl.ds(j * 128, 128)],
                                      wqkv.at[j], sem_q.at[k])
                for j in FIRST_ORDER[W_START[k]:W_START[k + 1]]]
               for k in range(len(W_GROUPS))]
    wo_cp = [pltpu.make_async_copy(wo_hbm.at[:, pl.ds(j * 128, 128)],
                                   wo.at[j], sem_w.at[0])
             for j in range(NG)]
    ffn_cp = [pltpu.make_async_copy(src.at[:, pl.ds(j * 128, 128)],
                                    wffn.at[off + j], sem_w.at[1])
              for src, off in ((wg_hbm, 0), (wu_hbm, NFC)) for j in range(NFC)]
    for j in range(NG):
        for kb in range(KB):
            rows = min(FF, (kb + 1) * D) - kb * D
            ffn_cp.append(pltpu.make_async_copy(
                wd_hbm.at[pl.ds(kb * D, rows), pl.ds(j * 128, 128)],
                wffn.at[_wd_idx(j, kb), pl.ds(0, rows), :], sem_w.at[1]))
    for cp in x_cp[:1] + wqkv_cp[0]:
        cp.start()

    with _scope('init'):
        vts[0:2] = jnp.zeros((2,) + vts.shape[1:], BF16)
        wr[...] = wr_ref[...].astype(F32).reshape(1, D)
        pad = KB * D - FF
        for j in range(NG):
            wffn[_wd_idx(j, KB - 1), D - pad:D, :] = jnp.zeros((pad, 128), BF16)
        col[KB, D - pad:D, :] = jnp.zeros((pad, 128), F32)
        hp[...] = jnp.zeros(hp.shape, F32)
        for t in range(NTB):
            order[t] = t
        mv_tab, bc_tab = _fs_tables()
        for i, v in enumerate(sum(mv_tab + bc_tab, ())):
            tab[i] = v
    with _scope('xwait'):
        x_cp[0].wait()
    for cp in sum(wqkv_cp[1:W_AHEAD], []) + x_cp[1:2]:
        cp.start()

    def out_copy(r0, n, slot):
        return pltpu.make_async_copy(xres.at[pl.ds(r0, n), :],
                                     out_hbm.at[0, pl.ds(r0, n), :], sem_o.at[slot])

    def layer(l, carry):
        never = jnp.full((8, 128), zero[0], I32) != 0

        with _scope('ln0'):
            _ln_stage(xres, xn, order[0])

        @pl.when(l == 0)
        def _():
            def wait_group(n):
                if n in W_START:
                    k = W_START.index(n)
                    for cp in wqkv_cp[k]:
                        cp.wait()
                    if k + W_AHEAD < len(W_GROUPS):
                        for cp in wqkv_cp[k + W_AHEAD]:
                            cp.start()
                    if k == len(W_GROUPS) // 2:
                        x_cp[1].wait()
                        _ln_stage(xres, xn, 1)
                    if k == len(W_GROUPS) - 1:
                        for cp in x_cp[2:]:
                            cp.start()

            with _scope('p1_first'):
                _qkv_stage(xn, wqkv, qs, ks, vts, 0, wait_group,
                           chunk_order=FIRST_ORDER)

        def wait_x(t):
            @pl.when(l == 0)
            def _():
                pltpu.make_async_copy(
                    x_hbm.at[0, pl.ds(t * TB, TB), :],
                    xres.at[pl.ds(t * TB, TB), :], sem_x.at[t]).wait()

        def p1_step(k, c):
            wait_x(k + 1)

            @pl.when(jnp.logical_and(l == 0, k == 2))
            def _():
                for cp in wo_cp + ffn_cp[:2 * NFC]:
                    cp.start()

            @pl.when(jnp.logical_and(l == 0, k == 5))
            def _():
                for cp in ffn_cp[2 * NFC:]:
                    cp.start()

            _qkv_stage(xn, wqkv, qs, ks, vts, order[k])
            _ln_stage(xres, xn, order[k + 1])
            return c

        def fs_step(k, c):
            b0 = 3 * (FS_STEPS * FS_N + k * FS_BC)
            for m in range(FS_BC):
                j, cs, rb = (tab[b0 + 3 * m + i] for i in range(3))
                hg = jnp.sum(hp[j], axis=0, keepdims=True)
                hu = jnp.sum(hp[NFC + j], axis=0, keepdims=True)
                a = (hg * jax.nn.sigmoid(hg) * hu).astype(BF16).astype(F32)
                col[cs, pl.ds(pl.multiple_of(rb * 128, 128), 128), :] = _bcast_cols(a)

            def matvec(n, y):
                n -= FS_LAG
                if 0 <= n < FS_N:
                    w, cs, slot = (tab[3 * (k * FS_N + n) + i] for i in range(3))
                    hp[slot] = _matvec_chunk(wffn, w, col, cs, never, y)

            _qkv_stage(xn, wqkv, qs, ks, vts, order[k], after_chunk=matvec)
            _ln_stage(xres, xn, order[k + 1])
            return c

        @pl.when(l == 1)
        def _():
            with _scope('fs_loop'):
                jax.lax.fori_loop(0, FS_STEPS, fs_step, 0)
            with _scope('fs_fin'):
                y = jnp.concatenate(
                    [jnp.sum(sum(hp[_wd_idx(j, kb)] for kb in range(KB)),
                             axis=0, keepdims=True) for j in range(NG)], axis=1)
                _add_to_row(xres, sel[0], y * gate[...])

        with _scope('p1_loop'):
            jax.lax.fori_loop(jnp.where(l == 0, 1, FS_STEPS), NTB - 1, p1_step, 0)

        best_v[...] = jnp.full((8, 1), -jnp.inf, F32)
        best_i[...] = jnp.zeros((8, 1), I32)

        def pv_all(sb):
            for g in range(NG):
                _unrotate_stage(_pv_stage(ps, ls, vts, sb, g), os_, g)

        def exp_groups(gs, after=None):
            for g in gs:
                _exp_stage(xs, ms, ps, ls, g, never, after)

        def proj(sb, exp_gs=None, **kw):
            if exp_gs is None:
                _proj_stage(os_, wo, wr, xres, xn, best_v, best_i, sb, never, **kw)
            else:
                _proj_stage(os_, wo, wr, xres, xn, best_v, best_i, sb, never,
                            overlap=lambda v: exp_groups(exp_gs, v),
                            fence=lambda: _packed(ps)[zero[0], 0, 0:8, :], **kw)

        def emit_out(sbs):
            @pl.when(l == N_LAYERS - 1)
            def _():
                for sb in sbs:
                    out_copy(sb * SB, SB, sb).start()

        one = zero[0] + 1

        def p1_last(_, c):
            for g in range(NG):
                _score_stage(qs, ks, xs, ms, None, g, static_sb=0)
            exp_groups(range(NG))

            def mid(n):
                if n == P1_LAST_SCORES_AT:
                    for g in range(NG):
                        _score_stage(qs, ks, xs, ms, None, g, static_sb=1)

            _qkv_stage(xn, wqkv, qs, ks, vts, NTB - 1, mid)
            return c

        def steady(s, c):
            pv_all(s - 1)
            exp_groups([0])
            _score_stage(qs, ks, xs, ms, s + 1, 0)
            proj(s - 1, range(1, NG))
            for g in range(1, NG):
                _score_stage(qs, ks, xs, ms, s + 1, g)
            return c

        def post(_, c):
            pv_all(NSB - 2)

            def mid(j):
                if j == POST_PV_AT:
                    pv_all(NSB - 1)

            exp_groups(range(POST_EARLY_EXP))
            proj(NSB - 2, range(POST_EARLY_EXP, NG), fence_at=POST_PV_AT - 1,
                 before_chunk=mid)
            proj(NSB - 1)
            return c

        with _scope('p1_last'):
            jax.lax.fori_loop(0, one, p1_last, 0)

        @pl.when(l == 0)
        def _():
            with _scope('wowait'):
                for cp in wo_cp:
                    cp.wait()

        with _scope('steady'):
            jax.lax.fori_loop(1, NSB - 1, steady, 0)
        emit_out(range(NSB - 2))
        with _scope('post'):
            jax.lax.fori_loop(0, one, post, 0)
        emit_out(range(NSB - 2, NSB))

        rmax, idx = _router(best_v, best_i)
        lhs = _row_group(xn, idx)

        @pl.when(l == 0)
        def _():
            with _scope('route'):
                for cp in ffn_cp:
                    cp.wait()
                sel[0] = idx
                gate[...] = jax.nn.sigmoid(rmax)
                _store_x_cols(col, lhs, idx)
                t_idx = idx // TB
                for p in range(NTB - 2):
                    order[p] = p + (p >= t_idx).astype(I32)
                order[NTB - 2] = jnp.minimum(t_idx, NTB - 2)

        @pl.when(l == N_LAYERS - 1)
        def _():
            with _scope('ffn'):
                y = _ffn_last(lhs, idx, wffn, col, never) * jax.nn.sigmoid(rmax)
                for sb in range(NSB):
                    out_copy(sb * SB, SB, sb).wait()
                g0 = _add_to_row(xres, idx, y)
            with _scope('ofinal'):
                cp = out_copy(g0, 16, NSB)
                cp.start()
                cp.wait()

        return carry

    jax.lax.fori_loop(0, N_LAYERS, layer, 0)


@jax.jit
def pallas_interleave_layers__sliding_block__moe_arch_mod__prompt_kernel(
    A_x: jax.Array,
    A_wqkv: jax.Array,
    A_wo: jax.Array,
    B_x: jax.Array,
    B_w_r: jax.Array,
    B_w_gate: jax.Array,
    B_w_up: jax.Array,
    B_w_down: jax.Array,
):
    del B_x
    any_spec = pl.BlockSpec(memory_space=pl.ANY)
    scratch = [
        pltpu.VMEM((S, D), BF16),
        pltpu.VMEM((NG, S, 128), BF16),
        pltpu.VMEM((NG, S, 128), BF16),
        pltpu.VMEM((NG, S, 128), BF16),
        pltpu.VMEM((NSB + 2, D, 128), BF16),
        pltpu.VMEM((NG, 4, XR, 128), F32),
        pltpu.VMEM((NG, 4, 8, 128), F32),
        pltpu.VMEM((NG, 4, XR, 128), BF16),
        pltpu.VMEM((NG, 4, 8, 128), F32),
        pltpu.VMEM((NG, SB, 128), BF16),
        pltpu.VMEM((3 * NG, D, 128), BF16),
        pltpu.VMEM((NG, D, 128), BF16),
        pltpu.VMEM((1, D), F32),
        pltpu.VMEM((NW, D, 128), BF16),
        pltpu.VMEM((COL_DUMMY + 1, D, 128), F32),
        pltpu.VMEM((NW + 1, 8, 128), F32),
        pltpu.VMEM((1, 1), F32),
        pltpu.VMEM((8, 1), F32),
        pltpu.VMEM((8, 1), I32),
        pltpu.SMEM((1,), I32),
        pltpu.SMEM((NTB,), I32),
        pltpu.SMEM((1,), I32),
        pltpu.SMEM((3 * FS_STEPS * (FS_N + FS_BC),), I32),
        pltpu.SemaphoreType.DMA((NTB,)),
        pltpu.SemaphoreType.DMA((len(W_GROUPS),)),
        pltpu.SemaphoreType.DMA((2,)),
        pltpu.SemaphoreType.DMA((NSB + 1,)),
    ]
    return pl.pallas_call(
        _kernel,
        out_shape=jax.ShapeDtypeStruct((1, S, D), BF16),
        in_specs=[any_spec, any_spec, any_spec,
                  pl.BlockSpec(memory_space=pltpu.VMEM),
                  any_spec, any_spec, any_spec],
        out_specs=any_spec,
        scratch_shapes=scratch,
        compiler_params=pltpu.CompilerParams(vmem_limit_bytes=112 * 1024 * 1024),
        name="swa_moe",
    )(A_x, A_wqkv, A_wo, B_w_r, B_w_gate, B_w_up, B_w_down)
```

```python
import math

import jax
import jax.numpy as jnp
import jax.experimental.pallas as pl
import jax.experimental.pallas.tpu as pltpu

F32 = jnp.float32
BF16 = jnp.bfloat16
U32 = jnp.uint32
I32 = jnp.int32

S = 2048
D = 1024
DH = 32
WIN = 256
FF = 3584
NG = 8
SB = 128
NSB = S // SB
QA = 32
XR = WIN + QA
TB = 256
NTB = S // TB
EPS = 1e-5
NEG = -1e30
QSCALE = (DH ** -0.5) * math.log2(math.e)
NT_DIMS = (((1,), (1,)), ((), ()))
N_LAYERS = 2
NFC = FF // 128
KB = 4
NW = 2 * NFC + NG * KB
FS_STEPS = 5
FS_N = 20
FS_BC = 10
FS_LAG = 3
COL_DUMMY = 1 + KB
NORM_AFTER = (0,)
FFN_VPU = 8
P1_LAST_SCORES_AT = 16
POST_PV_AT = 7
POST_EARLY_EXP = 1
W_GROUPS = (4, 4, 4, 4, 4, 4)
W_START = [sum(W_GROUPS[:i]) for i in range(len(W_GROUPS) + 1)]
W_AHEAD = 2


def _scope(name):
    return jax.named_scope(name)


def _layernorm(x):
    mean = jnp.sum(x, axis=1, keepdims=True) * (1.0 / D)
    xc = x - mean
    var = jnp.sum(xc * xc, axis=1, keepdims=True) * (1.0 / D)
    return xc * jax.lax.rsqrt(var + EPS)


def _packed(ref):
    return ref.bitcast(U32)


def _as_bf16(v):
    return pltpu.bitcast(v, BF16)


def _ln_stage(xres, xn, t):
    r0 = t * TB if isinstance(t, int) else pl.multiple_of(t * TB, TB)
    y = _layernorm(xres[pl.ds(r0, TB), :].astype(F32))
    for c in range(NG):
        xn[c, pl.ds(r0, TB), :] = y[:, c * 128:(c + 1) * 128].astype(BF16)


QKV_ORDER = list(range(2 * NG, 3 * NG)) + list(range(2 * NG))


FIRST_ORDER = sum(([2 * NG + 2 * i, 2 * NG + 2 * i + 1, 2 * i, 2 * i + 1]
                   for i in range(NG // 2)), []) + list(range(NG, 2 * NG))


def _qkv_stage(xn, wqkv, qs, ks, vts, t, before_chunk=None, after_chunk=None,
               chunk_order=QKV_ORDER):
    xp = _packed(xn)
    wp = _packed(wqkv)
    if isinstance(t, int):
        r0, h0 = t * TB, t * (TB // 2)
    else:
        r0 = pl.multiple_of(t * TB, TB)
        h0 = pl.multiple_of(t * (TB // 2), TB // 2)
    kt0 = 2 + t * (TB // 128)
    lhs = _as_bf16(jnp.concatenate(
        [xp[c, pl.ds(h0, TB // 2), :] for c in range(NG)], axis=1))
    for n, j in enumerate(chunk_order):
        if before_chunk is not None:
            before_chunk(n)
        y = jnp.dot(lhs, _as_bf16(wp[j]), preferred_element_type=F32)
        if after_chunk is not None:
            after_chunk(n, y[0:8])
        if j < NG:
            qs[j, pl.ds(r0, TB), :] = (y * QSCALE).astype(BF16)
        elif j < 2 * NG:
            ks[j - NG, pl.ds(r0, TB), :] = y.astype(BF16)
        else:
            c = j - 2 * NG
            for t in range(TB // 128):
                vts[kt0 + t, c * 128:(c + 1) * 128, :] = (
                    y[t * 128:(t + 1) * 128, :].T.astype(BF16))


def _score_stage(qs, ks, xs, ms, sb, g, static_sb=None, b=None):
    lane = jax.lax.broadcasted_iota(I32, (QA, 128), 1)
    li = lane % QA
    row = jax.lax.broadcasted_iota(I32, (QA, 128), 0)
    m_lo = row > li
    m_hi = row <= li
    lg = jax.lax.broadcasted_iota(I32, (QA // 2, 128), 1) // QA
    qp = _packed(qs)
    kp = _packed(ks)
    b = g if b is None else b
    for a in range(4):
        if static_sb is None:
            qa2 = pl.multiple_of(sb * (SB // 2) + (QA // 2) * a, QA // 2)
            q = qp[g, pl.ds(qa2, QA // 2), :]
            first = 0
            k = kp[g, pl.ds(qa2 - WIN // 2, XR // 2), :]
        else:
            qa = static_sb * SB + QA * a
            q = qp[g, qa // 2:(qa + QA) // 2, :]
            first = WIN - qa
            k = kp[g, 0:(XR - first) // 2, :]
        qbd = jnp.concatenate(
            [jnp.where(lg == ((a - p) % 4), q, jnp.zeros_like(q)) for p in range(4)],
            axis=0)
        x = jax.lax.dot_general(_as_bf16(k), _as_bf16(qbd), NT_DIMS,
                                preferred_element_type=F32)
        n = XR - first
        hi = jnp.where(m_hi, x[n - QA:n], NEG)
        if first == 0:
            lo = jnp.where(m_lo, x[0:QA], NEG)
            x = jnp.concatenate([lo, x[QA:n - QA], hi], axis=0)
        elif n > QA:
            x = jnp.concatenate(
                [jnp.full((first, 128), NEG, F32), x[0:n - QA], hi], axis=0)
        else:
            x = jnp.concatenate([jnp.full((first, 128), NEG, F32), hi], axis=0)
        xs[b, a] = x
        j0 = first // 16
        m0 = x[16 * j0:16 * j0 + 8]
        m1 = x[16 * j0 + 8:16 * j0 + 16]
        for j in range(j0 + 1, XR // 16):
            m0 = jnp.maximum(m0, x[16 * j:16 * j + 8])
            m1 = jnp.maximum(m1, x[16 * j + 8:16 * j + 16])
        mm = jnp.max(jnp.maximum(m0, m1), axis=0, keepdims=True)
        ms[b, a] = jnp.broadcast_to(mm, (8, 128))
    return m0


def _exp_stage(xs, ms, ps, ls, g, never, after=None):
    for a in range(4):
        m = ms[g, a]
        if after is not None:
            m = jnp.where(never, after, m)
        s0 = s1 = None
        for j in range(XR // 16):
            e0 = jnp.exp2(xs[g, a, 16 * j:16 * j + 8, :] - m)
            e1 = jnp.exp2(xs[g, a, 16 * j + 8:16 * j + 16, :] - m)
            s0 = e0 if s0 is None else s0 + e0
            s1 = e1 if s1 is None else s1 + e1
            if j == XR // 16 - 1:
                s = s0 + s1
                e1 = jnp.where(never, s, e1)
            ps[g, a, 16 * j:16 * j + 16, :] = (
                jnp.concatenate([e0, e1], axis=0).astype(BF16))
        ls[g, a] = s


def _pv_stage(ps, ls, vts, sb, g, b=None):
    lg8 = jax.lax.broadcasted_iota(I32, (8, 128), 1) // QA
    odd = (lg8 % 2) == 1
    hi2 = lg8 >= 2
    zero = jnp.zeros((8, 128), U32)
    pp = _packed(ps)
    vp = _packed(vts)
    b = g if b is None else b

    def sel(c, x, y):
        if x is None and y is None:
            return None
        return jnp.where(c, zero if x is None else x, zero if y is None else y)

    acc = [None] * 4
    for kt in range(3):
        yrows = [[] for _ in range(4)]
        for r in range(8 * kt, 8 * kt + 8):
            pr = []
            for a in range(4):
                j = r - 2 * a
                pr.append(pp[b, a, 8 * j:8 * j + 8, :] if 0 <= j < XR // 16 else None)
            z = [sel(odd, pr[(a + 1) % 4], pr[a]) for a in range(4)]
            for h in range(4):
                y = sel(hi2, z[(h + 2) % 4], z[h])
                yrows[h].append(zero if y is None else y)
        for h in range(4):
            y = _as_bf16(jnp.concatenate(yrows[h], axis=0))
            r0 = (g * 128 + DH * h) // 2
            vt = _as_bf16(vp[sb + kt, r0:r0 + DH // 2, :])
            ot = jnp.dot(vt, y, preferred_element_type=F32)
            acc[h] = ot if acc[h] is None else acc[h] + ot
    l = [jnp.sum(ls[b, a], axis=0, keepdims=True) for a in range(4)]
    lg1 = jax.lax.broadcasted_iota(I32, (1, 128), 1) // QA
    lz = [jnp.where((lg1 % 2) == 1, l[(a + 1) % 4], l[a]) for a in range(4)]
    ly = [jnp.where(lg1 >= 2, lz[(h + 2) % 4], lz[h]) for h in range(4)]
    return jnp.concatenate([acc[h] * (1.0 / ly[h]) for h in range(4)], axis=0)


def _unrotate_stage(ot, os_, g):
    t = ot.T
    lgrp = jax.lax.broadcasted_iota(I32, (QA, 128), 1) // QA
    odd = (lgrp % 2) == 1
    hi2 = lgrp >= 2
    tp = [t[QA * p:QA * p + QA] for p in range(4)]
    z = [jnp.where(odd, tp[(a - 1) % 4], tp[a]) for a in range(4)]
    outs = [jnp.where(hi2, z[(a - 2) % 4], z[a]) for a in range(4)]
    os_[g] = jnp.concatenate(outs, axis=0).astype(BF16)


def _proj_matmul(os_, wo, never, overlap=None, fence=None, fence_at=NG - 1,
                 before_chunk=None):
    op = _packed(os_)
    wp = _packed(wo)
    lhs = jnp.concatenate([op[g] for g in range(NG)], axis=1)
    cols = []
    for j in range(NG):
        if before_chunk is not None:
            before_chunk(j)
        lj = lhs
        if overlap is not None and j == fence_at:
            head = jnp.where(never, fence(), lhs[0:8, 0:128])
            top = jnp.concatenate([head, lhs[0:8, 128:]], axis=1)
            lj = jnp.concatenate([top, lhs[8:]], axis=0)
        y = jnp.dot(_as_bf16(lj), _as_bf16(wp[j]), preferred_element_type=F32)
        cols.append(y)
        if overlap is not None and j == 0:
            overlap(y[0:8])
    return jnp.concatenate(cols, axis=1)


def _norm_stage(acc, wr, xres, xn, best_v, best_i, sb, lo, hi, never, after=None):
    r0 = (sb * SB if isinstance(sb, int) else pl.multiple_of(sb * SB, SB)) + lo
    n = hi - lo
    x = xres[pl.ds(r0, n), :].astype(F32) + acc[lo:hi]
    mean = jnp.sum(x, axis=1, keepdims=True) * (1.0 / D)
    if after is not None:
        mean = jnp.where(never[0:1, 0:1], after[0:1, 0:1], mean)
    xc = x - mean
    var = jnp.sum(xc * xc, axis=1, keepdims=True) * (1.0 / D)
    rstd = jax.lax.rsqrt(var + EPS)
    y = x * rstd - mean * rstd
    r = jnp.sum(y * wr[...], axis=1, keepdims=True)
    xres[pl.ds(r0, n), :] = (x + y).astype(BF16)
    for c in range(NG):
        xn[c, pl.ds(r0, n), :] = y[:, c * 128:(c + 1) * 128].astype(BF16)
    bv = best_v[...]
    bi = best_i[...]
    sub = jax.lax.broadcasted_iota(I32, (8, 1), 0)
    for rg in range(n // 8):
        rr = r[8 * rg:8 * rg + 8]
        take = rr > bv
        bv = jnp.where(take, rr, bv)
        bi = jnp.where(take, sub + (r0 + 8 * rg), bi)
    best_v[...] = bv
    best_i[...] = bi


def _wd_idx(j, kb):
    return 2 * NFC + KB * j + kb


def _router(best_v, best_i):
    bv = best_v[...]
    rmax = jnp.max(bv, axis=0, keepdims=True)
    idx = jnp.min(jnp.where(bv == rmax, best_i[...], S))
    return rmax, idx


def _row_group(xn, idx):
    h0 = pl.multiple_of((idx >> 4) * 8, 8)
    xp = _packed(xn)
    return _as_bf16(jnp.concatenate(
        [xp[c, pl.ds(h0, 8), :] for c in range(NG)], axis=1))


def _add_to_row(xres, idx, y):
    g0 = pl.multiple_of((idx >> 4) * 16, 16)
    row = jax.lax.broadcasted_iota(I32, (16, D), 0)
    upd = jnp.where(row == (idx & 15), y, 0.0)
    xres[pl.ds(g0, 16), :] = (xres[pl.ds(g0, 16), :].astype(F32) + upd).astype(BF16)
    return g0


def _select_row(v, idx):
    row = jax.lax.broadcasted_iota(I32, v.shape, 0)
    return jnp.sum(jnp.where(row == (idx & 15), v, 0.0), axis=0, keepdims=True)


def _store_x_cols(col, lhs, idx):
    x = _select_row(lhs.astype(F32), idx)
    for c in range(NG):
        col[0, c * 128:(c + 1) * 128, :] = _bcast_cols(x[:, c * 128:(c + 1) * 128])


def _ffn_last(lhs, idx, wffn, col, never):
    wp = _packed(wffn)
    _store_x_cols(col, lhs, idx)
    todo = [(j, u) for j in range(NFC - FFN_VPU, NFC) for u in range(2)]
    h = {}
    n = 0
    for j in range(NFC - FFN_VPU):
        for u in range(2):
            y = jnp.dot(lhs, _as_bf16(wp[u * NFC + j]), preferred_element_type=F32)
            h[j, u] = _select_row(y, idx)
            if n >= 4 and n % 2 == 0 and todo:
                jj, uu = todo.pop(0)
                part = _matvec_chunk(wffn, uu * NFC + jj, col, 0, never, y[0:8])
                h[jj, uu] = jnp.sum(part, axis=0, keepdims=True)
            n += 1
    assert not todo
    act = jnp.concatenate(
        [h[j, 0] * jax.nn.sigmoid(h[j, 0]) * h[j, 1] for j in range(NFC)], axis=1)
    act = jnp.broadcast_to(act, (16, FF)).astype(BF16)
    cols = []
    for j in range(NG):
        w = jnp.concatenate(
            [wp[_wd_idx(j, kb), 0:(min(FF, (kb + 1) * D) - kb * D) // 2, :]
             for kb in range(KB)], axis=0)
        cols.append(jnp.dot(act, _as_bf16(w), preferred_element_type=F32)[0:1])
    return jnp.concatenate(cols, axis=1)


def _bcast_cols(row):
    return jnp.broadcast_to(row, (128, 128)).T


def _matvec_chunk(wffn, w, col, c, never, after):
    wp = _packed(wffn)
    acc = None
    for g in range(D // 16):
        v = wp[w, 8 * g:8 * g + 8, :]
        if g == 0:
            v = jnp.where(never, pltpu.bitcast(after, U32), v)
        t = _as_bf16(v).astype(F32) * col[c, 16 * g:16 * g + 16, :]
        acc = t if acc is None else acc + t
    return acc[0:8] + acc[8:16]


def _fs_tables():
    mv, bc = [], []
    for k in range(FS_STEPS):
        for n in range(FS_N):
            if k < 3:
                j = FS_BC * k + n % FS_BC
                w = min(j, NFC - 1) + (NFC if n >= FS_BC else 0)
                mv.append((w, 0, w if j < NFC else NW))
            else:
                j, kb = (n % 16) // 2, 2 * (k - 3) + n % 2
                w = _wd_idx(j, kb)
                mv.append((w, 1 + kb, w if n < 16 else NW))
        for m in range(FS_BC):
            j = FS_BC * (k - 1) + m
            if 1 <= k <= 3 and j < NFC:
                bc.append((j, 1 + j // NG, j % NG))
            else:
                bc.append((m, COL_DUMMY, m % NG))
    return mv, bc


def _kernel(x_hbm, wqkv_hbm, wo_hbm, wr_ref, wg_hbm, wu_hbm, wd_hbm, out_hbm,
            xres, xn, qs, ks, vts, xs, ms, ps, ls, os_, wqkv, wo, wr, wffn, col, hp, gate,
            best_v, best_i, zero, order, sel, tab, sem_x, sem_q, sem_w, sem_o):
    zero[0] = 0

    x_cp = [pltpu.make_async_copy(x_hbm.at[0, pl.ds(t * TB, TB), :],
                                  xres.at[pl.ds(t * TB, TB), :], sem_x.at[t])
            for t in range(NTB)]
    wqkv_cp = [[pltpu.make_async_copy(wqkv_hbm.at[:, pl.ds(j * 128, 128)],
                                      wqkv.at[j], sem_q.at[k])
                for j in FIRST_ORDER[W_START[k]:W_START[k + 1]]]
               for k in range(len(W_GROUPS))]
    wo_cp = [pltpu.make_async_copy(wo_hbm.at[:, pl.ds(j * 128, 128)],
                                   wo.at[j], sem_w.at[0])
             for j in range(NG)]
    ffn_cp = [pltpu.make_async_copy(src.at[:, pl.ds(j * 128, 128)],
                                    wffn.at[off + j], sem_w.at[1])
              for src, off in ((wg_hbm, 0), (wu_hbm, NFC)) for j in range(NFC)]
    for j in range(NG):
        for kb in range(KB):
            rows = min(FF, (kb + 1) * D) - kb * D
            ffn_cp.append(pltpu.make_async_copy(
                wd_hbm.at[pl.ds(kb * D, rows), pl.ds(j * 128, 128)],
                wffn.at[_wd_idx(j, kb), pl.ds(0, rows), :], sem_w.at[1]))
    x_cp[0].start()

    with _scope('init'):
        vts[0:2] = jnp.zeros((2,) + vts.shape[1:], BF16)
        wr[...] = wr_ref[...].astype(F32).reshape(1, D)
        pad = KB * D - FF
        for j in range(NG):
            wffn[_wd_idx(j, KB - 1), D - pad:D, :] = jnp.zeros((pad, 128), BF16)
        col[KB, D - pad:D, :] = jnp.zeros((pad, 128), F32)
        hp[...] = jnp.zeros(hp.shape, F32)
        for t in range(NTB):
            order[t] = t
        mv_tab, bc_tab = _fs_tables()
        for i, v in enumerate(sum(mv_tab + bc_tab, ())):
            tab[i] = v
    for cp in wqkv_cp[0]:
        cp.start()
    with _scope('xwait'):
        x_cp[0].wait()
    for cp in sum(wqkv_cp[1:W_AHEAD], []) + x_cp[1:2]:
        cp.start()

    def out_copy(r0, n, slot):
        return pltpu.make_async_copy(xres.at[pl.ds(r0, n), :],
                                     out_hbm.at[0, pl.ds(r0, n), :], sem_o.at[slot])

    def layer(l, carry):
        hint = [None]

        def new_hint():
            hint[0] = jnp.full((8, 128), zero[0], I32) != 0


        @pl.when(l == 0)
        def _():
            with _scope('ln0'):
                _ln_stage(xres, xn, 0)

            def wait_group(n):
                if n in W_START:
                    k = W_START.index(n)
                    for cp in wqkv_cp[k]:
                        cp.wait()
                    if k + W_AHEAD < len(W_GROUPS):
                        for cp in wqkv_cp[k + W_AHEAD]:
                            cp.start()
                    if k == len(W_GROUPS) // 2:
                        x_cp[1].wait()
                        _ln_stage(xres, xn, 1)
                    if k == len(W_GROUPS) - 1:
                        for cp in x_cp[2:]:
                            cp.start()

            with _scope('p1_first'):
                _qkv_stage(xn, wqkv, qs, ks, vts, 0, wait_group,
                           chunk_order=FIRST_ORDER)

        def wait_x(t):
            @pl.when(l == 0)
            def _():
                pltpu.make_async_copy(
                    x_hbm.at[0, pl.ds(t * TB, TB), :],
                    xres.at[pl.ds(t * TB, TB), :], sem_x.at[t]).wait()

        def p1_step(k, c):
            wait_x(k + 1)

            @pl.when(jnp.logical_and(l == 0, k == 2))
            def _():
                for cp in wo_cp + ffn_cp[:2 * NFC]:
                    cp.start()

            @pl.when(jnp.logical_and(l == 0, k == 5))
            def _():
                for cp in ffn_cp[2 * NFC:]:
                    cp.start()

            _qkv_stage(xn, wqkv, qs, ks, vts, order[k])
            _ln_stage(xres, xn, order[k + 1])
            return c

        def fs_step(k, c):
            new_hint()
            b0 = 3 * (FS_STEPS * FS_N + k * FS_BC)
            for m in range(FS_BC):
                j, cs, rb = (tab[b0 + 3 * m + i] for i in range(3))
                hg = jnp.sum(hp[j], axis=0, keepdims=True)
                hu = jnp.sum(hp[NFC + j], axis=0, keepdims=True)
                a = (hg * jax.nn.sigmoid(hg) * hu).astype(BF16).astype(F32)
                col[cs, pl.ds(pl.multiple_of(rb * 128, 128), 128), :] = _bcast_cols(a)

            def matvec(n, y):
                n -= FS_LAG
                if 0 <= n < FS_N:
                    w, cs, slot = (tab[3 * (k * FS_N + n) + i] for i in range(3))
                    hp[slot] = _matvec_chunk(wffn, w, col, cs, hint[0], y)

            _qkv_stage(xn, wqkv, qs, ks, vts, order[k], after_chunk=matvec)
            _ln_stage(xres, xn, order[k + 1])
            return c

        @pl.when(l == 1)
        def _():
            with _scope('fs_loop'):
                jax.lax.fori_loop(0, FS_STEPS, fs_step, 0)
            with _scope('fs_fin'):
                y = jnp.concatenate(
                    [jnp.sum(sum(hp[_wd_idx(j, kb)] for kb in range(KB)),
                             axis=0, keepdims=True) for j in range(NG)], axis=1)
                _add_to_row(xres, sel[0], y * gate[...])

        with _scope('p1_loop'):
            jax.lax.fori_loop(jnp.where(l == 0, 1, FS_STEPS), NTB - 1, p1_step, 0)

        best_v[...] = jnp.full((8, 1), -jnp.inf, F32)
        best_i[...] = jnp.zeros((8, 1), I32)

        def pv_all(sb):
            for g in range(NG):
                _unrotate_stage(_pv_stage(ps, ls, vts, sb, g), os_, g)

        def exp_groups(gs, after=None):
            for g in gs:
                _exp_stage(xs, ms, ps, ls, g, hint[0], after)

        def proj(exp_gs=None, **kw):
            if exp_gs is None:
                return _proj_matmul(os_, wo, hint[0], **kw)
            return _proj_matmul(os_, wo, hint[0],
                                overlap=lambda v: exp_groups(exp_gs, v),
                                fence=lambda: _packed(ps)[zero[0], 0, 0:8, :], **kw)

        def norm(acc, sb, lo=0, hi=SB, after=None):
            _norm_stage(acc, wr, xres, xn, best_v, best_i, sb, lo, hi, hint[0], after)

        def emit_out(sbs):
            @pl.when(l == N_LAYERS - 1)
            def _():
                for sb in sbs:
                    out_copy(sb * SB, SB, sb).start()

        one = zero[0] + 1

        def p1_last(_, c):
            new_hint()
            for g in range(NG):
                _score_stage(qs, ks, xs, ms, None, g, static_sb=0)
            exp_groups(range(NG))

            def mid(n):
                if n == P1_LAST_SCORES_AT:
                    for g in range(NG):
                        _score_stage(qs, ks, xs, ms, None, g, static_sb=1)

            _qkv_stage(xn, wqkv, qs, ks, vts, NTB - 1, mid)
            return c

        def steady(s, c):
            new_hint()
            pv_all(s - 1)
            exp_groups([0])
            _score_stage(qs, ks, xs, ms, s + 1, 0)
            acc = proj(range(1, NG))
            rows = SB // len(NORM_AFTER)
            for g in range(NG):
                v = None
                if g > 0:
                    v = _score_stage(qs, ks, xs, ms, s + 1, g)
                for i, a in enumerate(NORM_AFTER):
                    if a == g:
                        norm(acc, s - 1, i * rows, (i + 1) * rows, v)
            return c

        def post(_, c):
            new_hint()
            pv_all(NSB - 2)

            def mid(j):
                if j == POST_PV_AT:
                    pv_all(NSB - 1)

            exp_groups(range(POST_EARLY_EXP))
            norm(proj(range(POST_EARLY_EXP, NG), fence_at=POST_PV_AT - 1,
                      before_chunk=mid), NSB - 2)
            norm(proj(), NSB - 1)
            return c

        with _scope('p1_last'):
            jax.lax.fori_loop(0, one, p1_last, 0)

        @pl.when(l == 0)
        def _():
            with _scope('wowait'):
                for cp in wo_cp:
                    cp.wait()

        with _scope('steady'):
            jax.lax.fori_loop(1, NSB - 1, steady, 0)
        emit_out(range(NSB - 2))
        with _scope('post'):
            jax.lax.fori_loop(0, one, post, 0)
        emit_out(range(NSB - 2, NSB))

        rmax, idx = _router(best_v, best_i)
        lhs = _row_group(xn, idx)

        @pl.when(l == 0)
        def _():
            with _scope('route'):
                for cp in ffn_cp:
                    cp.wait()
                sel[0] = idx
                gate[...] = jax.nn.sigmoid(rmax)
                _store_x_cols(col, lhs, idx)
                t_idx = idx // TB
                for p in range(NTB - 2):
                    order[p] = p + (p >= t_idx).astype(I32)
                order[NTB - 2] = jnp.minimum(t_idx, NTB - 2)
                _ln_stage(xres, xn, (t_idx == 0).astype(I32))

        @pl.when(l == N_LAYERS - 1)
        def _():
            with _scope('ffn'):
                new_hint()
                y = _ffn_last(lhs, idx, wffn, col, hint[0]) * jax.nn.sigmoid(rmax)
                for sb in range(NSB):
                    out_copy(sb * SB, SB, sb).wait()
                g0 = _add_to_row(xres, idx, y)
            with _scope('ofinal'):
                cp = out_copy(g0, 16, NSB)
                cp.start()
                cp.wait()

        return carry

    jax.lax.fori_loop(0, N_LAYERS, layer, 0)


@jax.jit
def pallas_interleave_layers__sliding_block__moe_arch_mod__prompt_kernel(
    A_x: jax.Array,
    A_wqkv: jax.Array,
    A_wo: jax.Array,
    B_x: jax.Array,
    B_w_r: jax.Array,
    B_w_gate: jax.Array,
    B_w_up: jax.Array,
    B_w_down: jax.Array,
):
    del B_x
    any_spec = pl.BlockSpec(memory_space=pl.ANY)
    scratch = [
        pltpu.VMEM((S, D), BF16),
        pltpu.VMEM((NG, S, 128), BF16),
        pltpu.VMEM((NG, S, 128), BF16),
        pltpu.VMEM((NG, S, 128), BF16),
        pltpu.VMEM((NSB + 2, D, 128), BF16),
        pltpu.VMEM((NG, 4, XR, 128), F32),
        pltpu.VMEM((NG, 4, 8, 128), F32),
        pltpu.VMEM((NG, 4, XR, 128), BF16),
        pltpu.VMEM((NG, 4, 8, 128), F32),
        pltpu.VMEM((NG, SB, 128), BF16),
        pltpu.VMEM((3 * NG, D, 128), BF16),
        pltpu.VMEM((NG, D, 128), BF16),
        pltpu.VMEM((1, D), F32),
        pltpu.VMEM((NW, D, 128), BF16),
        pltpu.VMEM((COL_DUMMY + 1, D, 128), F32),
        pltpu.VMEM((NW + 1, 8, 128), F32),
        pltpu.VMEM((1, 1), F32),
        pltpu.VMEM((8, 1), F32),
        pltpu.VMEM((8, 1), I32),
        pltpu.SMEM((1,), I32),
        pltpu.SMEM((NTB,), I32),
        pltpu.SMEM((1,), I32),
        pltpu.SMEM((3 * FS_STEPS * (FS_N + FS_BC),), I32),
        pltpu.SemaphoreType.DMA((NTB,)),
        pltpu.SemaphoreType.DMA((len(W_GROUPS),)),
        pltpu.SemaphoreType.DMA((2,)),
        pltpu.SemaphoreType.DMA((NSB + 1,)),
    ]
    return pl.pallas_call(
        _kernel,
        out_shape=jax.ShapeDtypeStruct((1, S, D), BF16),
        in_specs=[any_spec, any_spec, any_spec,
                  pl.BlockSpec(memory_space=pltpu.VMEM),
                  any_spec, any_spec, any_spec],
        out_specs=any_spec,
        scratch_shapes=scratch,
        compiler_params=pltpu.CompilerParams(vmem_limit_bytes=112 * 1024 * 1024),
        name="swa_moe",
    )(A_x, A_wqkv, A_wo, B_w_r, B_w_gate, B_w_up, B_w_down)
```

```python
import math

import jax
import jax.numpy as jnp
import jax.experimental.pallas as pl
import jax.experimental.pallas.tpu as pltpu

F32 = jnp.float32
BF16 = jnp.bfloat16
U32 = jnp.uint32
I32 = jnp.int32

S = 2048
D = 1024
DH = 32
WIN = 256
FF = 3584
NG = 8
SB = 128
NSB = S // SB
QA = 32
XR = WIN + QA
TB = 256
NTB = S // TB
EPS = 1e-5
NEG = -1e30
QSCALE = (DH ** -0.5) * math.log2(math.e)
NT_DIMS = (((1,), (1,)), ((), ()))
N_LAYERS = 2
NFC = FF // 128
KB = 4
NW = 2 * NFC + NG * KB
FS_STEPS = 5
FS_N = 20
FS_BC = 10
FS_LAG = 3
COL_DUMMY = 1 + KB
NORM_AFTER = (0,)
FFN_VPU = 8
P1_LAST_SCORES_AT = 16
POST_PV_AT = 7
POST_EARLY_EXP = 1
W_GROUP = 4


def _scope(name):
    return jax.named_scope(name)


def _layernorm(x):
    mean = jnp.sum(x, axis=1, keepdims=True) * (1.0 / D)
    xc = x - mean
    var = jnp.sum(xc * xc, axis=1, keepdims=True) * (1.0 / D)
    return xc * jax.lax.rsqrt(var + EPS)


def _packed(ref):
    return ref.bitcast(U32)


def _as_bf16(v):
    return pltpu.bitcast(v, BF16)


def _ln_stage(xres, xn, t, rows=TB):
    r0 = t * rows if isinstance(t, int) else pl.multiple_of(t * rows, rows)
    y = _layernorm(xres[pl.ds(r0, rows), :].astype(F32))
    for c in range(NG):
        xn[c, pl.ds(r0, rows), :] = y[:, c * 128:(c + 1) * 128].astype(BF16)


QKV_ORDER = list(range(2 * NG, 3 * NG)) + list(range(2 * NG))


def _qkv_lhs(xn, h0):
    xp = _packed(xn)
    return _as_bf16(jnp.concatenate(
        [xp[c, pl.ds(h0, TB // 2), :] for c in range(NG)], axis=1))


def _first_group_chunk(k, n):
    if isinstance(k, int):
        if k < 4:
            return (2 * NG + 2 * k + n) if n < 2 else (2 * k + n - 2)
        return NG + 4 * (k - 4) + n
    a = (2 * NG + 2 * k + n) if n < 2 else (2 * k + n - 2)
    return jnp.where(k < 4, a, NG + 4 * (k - 4) + n)


def _qkv_stage(xn, wqkv, qs, ks, vts, t, before_chunk=None, after_chunk=None):
    wp = _packed(wqkv)
    if isinstance(t, int):
        r0, h0 = t * TB, t * (TB // 2)
    else:
        r0 = pl.multiple_of(t * TB, TB)
        h0 = pl.multiple_of(t * (TB // 2), TB // 2)
    kt0 = 2 + t * (TB // 128)
    lhs = _qkv_lhs(xn, h0)
    for n, j in enumerate(QKV_ORDER):
        if before_chunk is not None:
            before_chunk(n)
        y = jnp.dot(lhs, _as_bf16(wp[j]), preferred_element_type=F32)
        if after_chunk is not None:
            after_chunk(n, y[0:8])
        if j < NG:
            qs[j, pl.ds(r0, TB), :] = (y * QSCALE).astype(BF16)
        elif j < 2 * NG:
            ks[j - NG, pl.ds(r0, TB), :] = y.astype(BF16)
        else:
            c = j - 2 * NG
            for t in range(TB // 128):
                vts[kt0 + t, c * 128:(c + 1) * 128, :] = (
                    y[t * 128:(t + 1) * 128, :].T.astype(BF16))


def _score_stage(qs, ks, xs, ms, sb, g, static_sb=None, b=None):
    lane = jax.lax.broadcasted_iota(I32, (QA, 128), 1)
    li = lane % QA
    row = jax.lax.broadcasted_iota(I32, (QA, 128), 0)
    m_lo = row > li
    m_hi = row <= li
    lg = jax.lax.broadcasted_iota(I32, (QA // 2, 128), 1) // QA
    qp = _packed(qs)
    kp = _packed(ks)
    b = g if b is None else b
    for a in range(4):
        if static_sb is None:
            qa2 = pl.multiple_of(sb * (SB // 2) + (QA // 2) * a, QA // 2)
            q = qp[g, pl.ds(qa2, QA // 2), :]
            first = 0
            k = kp[g, pl.ds(qa2 - WIN // 2, XR // 2), :]
        else:
            qa = static_sb * SB + QA * a
            q = qp[g, qa // 2:(qa + QA) // 2, :]
            first = WIN - qa
            k = kp[g, 0:(XR - first) // 2, :]
        qbd = jnp.concatenate(
            [jnp.where(lg == ((a - p) % 4), q, jnp.zeros_like(q)) for p in range(4)],
            axis=0)
        x = jax.lax.dot_general(_as_bf16(k), _as_bf16(qbd), NT_DIMS,
                                preferred_element_type=F32)
        n = XR - first
        hi = jnp.where(m_hi, x[n - QA:n], NEG)
        if first == 0:
            lo = jnp.where(m_lo, x[0:QA], NEG)
            x = jnp.concatenate([lo, x[QA:n - QA], hi], axis=0)
        elif n > QA:
            x = jnp.concatenate(
                [jnp.full((first, 128), NEG, F32), x[0:n - QA], hi], axis=0)
        else:
            x = jnp.concatenate([jnp.full((first, 128), NEG, F32), hi], axis=0)
        xs[b, a] = x
        j0 = first // 16
        m0 = x[16 * j0:16 * j0 + 8]
        m1 = x[16 * j0 + 8:16 * j0 + 16]
        for j in range(j0 + 1, XR // 16):
            m0 = jnp.maximum(m0, x[16 * j:16 * j + 8])
            m1 = jnp.maximum(m1, x[16 * j + 8:16 * j + 16])
        mm = jnp.max(jnp.maximum(m0, m1), axis=0, keepdims=True)
        ms[b, a] = jnp.broadcast_to(mm, (8, 128))
    return m0


def _exp_stage(xs, ms, ps, ls, g, never, after=None):
    for a in range(4):
        m = ms[g, a]
        if after is not None:
            m = jnp.where(never, after, m)
        s0 = s1 = None
        for j in range(XR // 16):
            e0 = jnp.exp2(xs[g, a, 16 * j:16 * j + 8, :] - m)
            e1 = jnp.exp2(xs[g, a, 16 * j + 8:16 * j + 16, :] - m)
            s0 = e0 if s0 is None else s0 + e0
            s1 = e1 if s1 is None else s1 + e1
            if j == XR // 16 - 1:
                s = s0 + s1
                e1 = jnp.where(never, s, e1)
            ps[g, a, 16 * j:16 * j + 16, :] = (
                jnp.concatenate([e0, e1], axis=0).astype(BF16))
        ls[g, a] = s


def _pv_stage(ps, ls, vts, sb, g, b=None):
    lg8 = jax.lax.broadcasted_iota(I32, (8, 128), 1) // QA
    odd = (lg8 % 2) == 1
    hi2 = lg8 >= 2
    zero = jnp.zeros((8, 128), U32)
    pp = _packed(ps)
    vp = _packed(vts)
    b = g if b is None else b

    def sel(c, x, y):
        if x is None and y is None:
            return None
        return jnp.where(c, zero if x is None else x, zero if y is None else y)

    acc = [None] * 4
    for kt in range(3):
        yrows = [[] for _ in range(4)]
        for r in range(8 * kt, 8 * kt + 8):
            pr = []
            for a in range(4):
                j = r - 2 * a
                pr.append(pp[b, a, 8 * j:8 * j + 8, :] if 0 <= j < XR // 16 else None)
            z = [sel(odd, pr[(a + 1) % 4], pr[a]) for a in range(4)]
            for h in range(4):
                y = sel(hi2, z[(h + 2) % 4], z[h])
                yrows[h].append(zero if y is None else y)
        for h in range(4):
            y = _as_bf16(jnp.concatenate(yrows[h], axis=0))
            r0 = (g * 128 + DH * h) // 2
            vt = _as_bf16(vp[sb + kt, r0:r0 + DH // 2, :])
            ot = jnp.dot(vt, y, preferred_element_type=F32)
            acc[h] = ot if acc[h] is None else acc[h] + ot
    l = [jnp.sum(ls[b, a], axis=0, keepdims=True) for a in range(4)]
    lg1 = jax.lax.broadcasted_iota(I32, (1, 128), 1) // QA
    lz = [jnp.where((lg1 % 2) == 1, l[(a + 1) % 4], l[a]) for a in range(4)]
    ly = [jnp.where(lg1 >= 2, lz[(h + 2) % 4], lz[h]) for h in range(4)]
    return jnp.concatenate([acc[h] * (1.0 / ly[h]) for h in range(4)], axis=0)


def _unrotate_stage(ot, os_, g):
    t = ot.T
    lgrp = jax.lax.broadcasted_iota(I32, (QA, 128), 1) // QA
    odd = (lgrp % 2) == 1
    hi2 = lgrp >= 2
    tp = [t[QA * p:QA * p + QA] for p in range(4)]
    z = [jnp.where(odd, tp[(a - 1) % 4], tp[a]) for a in range(4)]
    outs = [jnp.where(hi2, z[(a - 2) % 4], z[a]) for a in range(4)]
    os_[g] = jnp.concatenate(outs, axis=0).astype(BF16)


def _proj_matmul(os_, wo, never, overlap=None, fence=None, fence_at=NG - 1,
                 before_chunk=None):
    op = _packed(os_)
    wp = _packed(wo)
    lhs = jnp.concatenate([op[g] for g in range(NG)], axis=1)
    cols = []
    for j in range(NG):
        if before_chunk is not None:
            before_chunk(j)
        lj = lhs
        if overlap is not None and j == fence_at:
            head = jnp.where(never, fence(), lhs[0:8, 0:128])
            top = jnp.concatenate([head, lhs[0:8, 128:]], axis=1)
            lj = jnp.concatenate([top, lhs[8:]], axis=0)
        y = jnp.dot(_as_bf16(lj), _as_bf16(wp[j]), preferred_element_type=F32)
        cols.append(y)
        if overlap is not None and j == 0:
            overlap(y[0:8])
    return jnp.concatenate(cols, axis=1)


def _norm_stage(acc, wr, xres, xn, best_v, best_i, sb, lo, hi, never, after=None):
    r0 = (sb * SB if isinstance(sb, int) else pl.multiple_of(sb * SB, SB)) + lo
    n = hi - lo
    x = xres[pl.ds(r0, n), :].astype(F32) + acc[lo:hi]
    mean = jnp.sum(x, axis=1, keepdims=True) * (1.0 / D)
    if after is not None:
        mean = jnp.where(never[0:1, 0:1], after[0:1, 0:1], mean)
    xc = x - mean
    var = jnp.sum(xc * xc, axis=1, keepdims=True) * (1.0 / D)
    rstd = jax.lax.rsqrt(var + EPS)
    y = x * rstd - mean * rstd
    r = jnp.sum(y * wr[...], axis=1, keepdims=True)
    xres[pl.ds(r0, n), :] = (x + y).astype(BF16)
    for c in range(NG):
        xn[c, pl.ds(r0, n), :] = y[:, c * 128:(c + 1) * 128].astype(BF16)
    bv = best_v[...]
    bi = best_i[...]
    sub = jax.lax.broadcasted_iota(I32, (8, 1), 0)
    for rg in range(n // 8):
        rr = r[8 * rg:8 * rg + 8]
        take = rr > bv
        bv = jnp.where(take, rr, bv)
        bi = jnp.where(take, sub + (r0 + 8 * rg), bi)
    best_v[...] = bv
    best_i[...] = bi


def _wd_idx(j, kb):
    return 2 * NFC + KB * j + kb


def _router(best_v, best_i):
    bv = best_v[...]
    rmax = jnp.max(bv, axis=0, keepdims=True)
    idx = jnp.min(jnp.where(bv == rmax, best_i[...], S))
    return rmax, idx


def _row_group(xn, idx):
    h0 = pl.multiple_of((idx >> 4) * 8, 8)
    xp = _packed(xn)
    return _as_bf16(jnp.concatenate(
        [xp[c, pl.ds(h0, 8), :] for c in range(NG)], axis=1))


def _add_to_row(xres, idx, y):
    g0 = pl.multiple_of((idx >> 4) * 16, 16)
    row = jax.lax.broadcasted_iota(I32, (16, D), 0)
    upd = jnp.where(row == (idx & 15), y, 0.0)
    xres[pl.ds(g0, 16), :] = (xres[pl.ds(g0, 16), :].astype(F32) + upd).astype(BF16)
    return g0


def _select_row(v, idx):
    row = jax.lax.broadcasted_iota(I32, v.shape, 0)
    return jnp.sum(jnp.where(row == (idx & 15), v, 0.0), axis=0, keepdims=True)


def _store_x_cols(col, lhs, idx):
    x = _select_row(lhs.astype(F32), idx)
    for c in range(NG):
        col[0, c * 128:(c + 1) * 128, :] = _bcast_cols(x[:, c * 128:(c + 1) * 128])


def _ffn_last(lhs, idx, wffn, col, never):
    wp = _packed(wffn)
    _store_x_cols(col, lhs, idx)
    todo = [(j, u) for j in range(NFC - FFN_VPU, NFC) for u in range(2)]
    h = {}
    n = 0
    for j in range(NFC - FFN_VPU):
        for u in range(2):
            y = jnp.dot(lhs, _as_bf16(wp[u * NFC + j]), preferred_element_type=F32)
            h[j, u] = _select_row(y, idx)
            if n >= 4 and n % 2 == 0 and todo:
                jj, uu = todo.pop(0)
                part = _matvec_chunk(wffn, uu * NFC + jj, col, 0, never, y[0:8])
                h[jj, uu] = jnp.sum(part, axis=0, keepdims=True)
            n += 1
    assert not todo
    act = jnp.concatenate(
        [h[j, 0] * jax.nn.sigmoid(h[j, 0]) * h[j, 1] for j in range(NFC)], axis=1)
    act = jnp.broadcast_to(act, (16, FF)).astype(BF16)
    cols = []
    for j in range(NG):
        w = jnp.concatenate(
            [wp[_wd_idx(j, kb), 0:(min(FF, (kb + 1) * D) - kb * D) // 2, :]
             for kb in range(KB)], axis=0)
        cols.append(jnp.dot(act, _as_bf16(w), preferred_element_type=F32)[0:1])
    return jnp.concatenate(cols, axis=1)


def _bcast_cols(row):
    return jnp.broadcast_to(row, (128, 128)).T


def _matvec_chunk(wffn, w, col, c, never, after):
    wp = _packed(wffn)
    acc = None
    for g in range(D // 16):
        v = wp[w, 8 * g:8 * g + 8, :]
        if g == 0:
            v = jnp.where(never, pltpu.bitcast(after, U32), v)
        t = _as_bf16(v).astype(F32) * col[c, 16 * g:16 * g + 16, :]
        acc = t if acc is None else acc + t
    return acc[0:8] + acc[8:16]


def _fs_tables():
    mv, bc = [], []
    for k in range(FS_STEPS):
        for n in range(FS_N):
            if k < 3:
                j = FS_BC * k + n % FS_BC
                w = min(j, NFC - 1) + (NFC if n >= FS_BC else 0)
                mv.append((w, 0, w if j < NFC else NW))
            else:
                j, kb = (n % 16) // 2, 2 * (k - 3) + n % 2
                w = _wd_idx(j, kb)
                mv.append((w, 1 + kb, w if n < 16 else NW))
        for m in range(FS_BC):
            j = FS_BC * (k - 1) + m
            if 1 <= k <= 3 and j < NFC:
                bc.append((j, 1 + j // NG, j % NG))
            else:
                bc.append((m, COL_DUMMY, m % NG))
    return mv, bc


def _kernel(x_hbm, wqkv_hbm, wo_hbm, wr_ref, wg_hbm, wu_hbm, wd_hbm, out_hbm,
            xres, xn, qs, ks, vts, xs, ms, ps, ls, os_, wqkv, wo, wr, wffn, col, hp, gate,
            best_v, best_i, zero, order, sel, tab, sem_x, sem_q, sem_w, sem_o):
    zero[0] = 0

    x_cp = [pltpu.make_async_copy(x_hbm.at[0, pl.ds(t * TB, TB), :],
                                  xres.at[pl.ds(t * TB, TB), :], sem_x.at[t])
            for t in range(NTB)]
    def wqkv_group(k):
        cps = []
        for n in range(W_GROUP):
            j = _first_group_chunk(k, n)
            c0 = j * 128 if isinstance(j, int) else pl.multiple_of(j * 128, 128)
            cps.append(pltpu.make_async_copy(wqkv_hbm.at[:, pl.ds(c0, 128)],
                                             wqkv.at[j], sem_q.at[k]))
        return cps

    wo_cp = [pltpu.make_async_copy(wo_hbm.at[:, pl.ds(j * 128, 128)],
                                   wo.at[j], sem_w.at[0])
             for j in range(NG)]
    ffn_cp = [pltpu.make_async_copy(src.at[:, pl.ds(j * 128, 128)],
                                    wffn.at[off + j], sem_w.at[1])
              for src, off in ((wg_hbm, 0), (wu_hbm, NFC)) for j in range(NFC)]
    for j in range(NG):
        for kb in range(KB):
            rows = min(FF, (kb + 1) * D) - kb * D
            ffn_cp.append(pltpu.make_async_copy(
                wd_hbm.at[pl.ds(kb * D, rows), pl.ds(j * 128, 128)],
                wffn.at[_wd_idx(j, kb), pl.ds(0, rows), :], sem_w.at[1]))
    x_cp[0].start()

    with _scope('init'):
        vts[0:2] = jnp.zeros((2,) + vts.shape[1:], BF16)
        wr[...] = wr_ref[...].astype(F32).reshape(1, D)
        pad = KB * D - FF
        for j in range(NG):
            wffn[_wd_idx(j, KB - 1), D - pad:D, :] = jnp.zeros((pad, 128), BF16)
        col[KB, D - pad:D, :] = jnp.zeros((pad, 128), F32)
        hp[...] = jnp.zeros(hp.shape, F32)
        for t in range(NTB):
            order[t] = t
        mv_tab, bc_tab = _fs_tables()
        for i, v in enumerate(sum(mv_tab + bc_tab, ())):
            tab[i] = v
    for cp in wqkv_group(0):
        cp.start()
    with _scope('xwait'):
        x_cp[0].wait()
    for cp in wqkv_group(1) + x_cp[1:2]:
        cp.start()

    def out_copy(r0, n, slot):
        return pltpu.make_async_copy(xres.at[pl.ds(r0, n), :],
                                     out_hbm.at[0, pl.ds(r0, n), :], sem_o.at[slot])

    def layer(l, carry):
        hint = [None]

        def new_hint():
            hint[0] = jnp.full((8, 128), zero[0], I32) != 0


        @pl.when(l == 0)
        def _():
            with _scope('ln0'):
                _ln_stage(xres, xn, 0)

            wp = _packed(wqkv)

            def vq_group(k, c):
                for cp in wqkv_group(k):
                    cp.wait()
                for cp in wqkv_group(k + 2):
                    cp.start()
                lhs = _qkv_lhs(xn, 0)
                for n in range(W_GROUP):
                    j = _first_group_chunk(k, n)
                    y = jnp.dot(lhs, _as_bf16(wp[j]), preferred_element_type=F32)
                    if n < 2:
                        c0 = pl.multiple_of((j - 2 * NG) * 128, 128)
                        for t in range(TB // 128):
                            vts[2 + t, pl.ds(c0, 128), :] = (
                                y[t * 128:(t + 1) * 128, :].T.astype(BF16))
                    else:
                        qs[j, 0:TB, :] = (y * QSCALE).astype(BF16)
                return c

            def k_group(i, c):
                for cp in wqkv_group(4 + i):
                    cp.wait()

                @pl.when(i == 0)
                def _():
                    x_cp[1].wait()

                @pl.when(i == 1)
                def _():
                    for cp in x_cp[2:]:
                        cp.start()

                lhs = _qkv_lhs(xn, 0)
                for n in range(W_GROUP):
                    j = NG + W_GROUP * i + n
                    y = jnp.dot(lhs, _as_bf16(wp[j]), preferred_element_type=F32)
                    ks[j - NG, 0:TB, :] = y.astype(BF16)
                _ln_stage(xres, xn, TB // 128 + i, rows=128)
                return c

            with _scope('p1_first'):
                jax.lax.fori_loop(0, 4, vq_group, 0)
                jax.lax.fori_loop(0, 2, k_group, 0)

        def wait_x(t):
            @pl.when(l == 0)
            def _():
                pltpu.make_async_copy(
                    x_hbm.at[0, pl.ds(t * TB, TB), :],
                    xres.at[pl.ds(t * TB, TB), :], sem_x.at[t]).wait()

        def p1_step(k, c):
            wait_x(k + 1)

            @pl.when(jnp.logical_and(l == 0, k == 2))
            def _():
                for cp in wo_cp + ffn_cp[:2 * NFC]:
                    cp.start()

            @pl.when(jnp.logical_and(l == 0, k == 5))
            def _():
                for cp in ffn_cp[2 * NFC:]:
                    cp.start()

            _qkv_stage(xn, wqkv, qs, ks, vts, order[k])
            _ln_stage(xres, xn, order[k + 1])
            return c

        def fs_step(k, c):
            new_hint()
            b0 = 3 * (FS_STEPS * FS_N + k * FS_BC)
            for m in range(FS_BC):
                j, cs, rb = (tab[b0 + 3 * m + i] for i in range(3))
                hg = jnp.sum(hp[j], axis=0, keepdims=True)
                hu = jnp.sum(hp[NFC + j], axis=0, keepdims=True)
                a = (hg * jax.nn.sigmoid(hg) * hu).astype(BF16).astype(F32)
                col[cs, pl.ds(pl.multiple_of(rb * 128, 128), 128), :] = _bcast_cols(a)

            def matvec(n, y):
                n -= FS_LAG
                if 0 <= n < FS_N:
                    w, cs, slot = (tab[3 * (k * FS_N + n) + i] for i in range(3))
                    hp[slot] = _matvec_chunk(wffn, w, col, cs, hint[0], y)

            _qkv_stage(xn, wqkv, qs, ks, vts, order[k], after_chunk=matvec)
            _ln_stage(xres, xn, order[k + 1])
            return c

        @pl.when(l == 1)
        def _():
            with _scope('fs_loop'):
                jax.lax.fori_loop(0, FS_STEPS, fs_step, 0)
            with _scope('fs_fin'):
                y = jnp.concatenate(
                    [jnp.sum(sum(hp[_wd_idx(j, kb)] for kb in range(KB)),
                             axis=0, keepdims=True) for j in range(NG)], axis=1)
                _add_to_row(xres, sel[0], y * gate[...])

        with _scope('p1_loop'):
            jax.lax.fori_loop(jnp.where(l == 0, 1, FS_STEPS), NTB - 1, p1_step, 0)

        best_v[...] = jnp.full((8, 1), -jnp.inf, F32)
        best_i[...] = jnp.zeros((8, 1), I32)

        def pv_all(sb):
            for g in range(NG):
                _unrotate_stage(_pv_stage(ps, ls, vts, sb, g), os_, g)

        def exp_groups(gs, after=None):
            for g in gs:
                _exp_stage(xs, ms, ps, ls, g, hint[0], after)

        def proj(exp_gs=None, **kw):
            if exp_gs is None:
                return _proj_matmul(os_, wo, hint[0], **kw)
            return _proj_matmul(os_, wo, hint[0],
                                overlap=lambda v: exp_groups(exp_gs, v),
                                fence=lambda: _packed(ps)[zero[0], 0, 0:8, :], **kw)

        def norm(acc, sb, lo=0, hi=SB, after=None):
            _norm_stage(acc, wr, xres, xn, best_v, best_i, sb, lo, hi, hint[0], after)

        def emit_out(sbs):
            @pl.when(l == N_LAYERS - 1)
            def _():
                for sb in sbs:
                    out_copy(sb * SB, SB, sb).start()

        one = zero[0] + 1

        def p1_last(_, c):
            new_hint()
            for g in range(NG):
                _score_stage(qs, ks, xs, ms, None, g, static_sb=0)
            exp_groups(range(NG))

            def mid(n):
                if n == P1_LAST_SCORES_AT:
                    for g in range(NG):
                        _score_stage(qs, ks, xs, ms, None, g, static_sb=1)

            _qkv_stage(xn, wqkv, qs, ks, vts, NTB - 1, mid)
            return c

        def steady(s, c):
            new_hint()
            pv_all(s - 1)
            exp_groups([0])
            _score_stage(qs, ks, xs, ms, s + 1, 0)
            acc = proj(range(1, NG))
            rows = SB // len(NORM_AFTER)
            for g in range(NG):
                v = None
                if g > 0:
                    v = _score_stage(qs, ks, xs, ms, s + 1, g)
                for i, a in enumerate(NORM_AFTER):
                    if a == g:
                        norm(acc, s - 1, i * rows, (i + 1) * rows, v)
            return c

        def post(_, c):
            new_hint()
            pv_all(NSB - 2)

            def mid(j):
                if j == POST_PV_AT:
                    pv_all(NSB - 1)

            exp_groups(range(POST_EARLY_EXP))
            norm(proj(range(POST_EARLY_EXP, NG), fence_at=POST_PV_AT - 1,
                      before_chunk=mid), NSB - 2)
            norm(proj(), NSB - 1)
            return c

        with _scope('p1_last'):
            jax.lax.fori_loop(0, one, p1_last, 0)

        @pl.when(l == 0)
        def _():
            with _scope('wowait'):
                for cp in wo_cp:
                    cp.wait()

        with _scope('steady'):
            jax.lax.fori_loop(1, NSB - 1, steady, 0)
        emit_out(range(NSB - 2))
        with _scope('post'):
            jax.lax.fori_loop(0, one, post, 0)
        emit_out(range(NSB - 2, NSB))

        rmax, idx = _router(best_v, best_i)
        lhs = _row_group(xn, idx)

        @pl.when(l == 0)
        def _():
            with _scope('route'):
                for cp in ffn_cp:
                    cp.wait()
                sel[0] = idx
                gate[...] = jax.nn.sigmoid(rmax)
                _store_x_cols(col, lhs, idx)
                t_idx = idx // TB
                for p in range(NTB - 2):
                    order[p] = p + (p >= t_idx).astype(I32)
                order[NTB - 2] = jnp.minimum(t_idx, NTB - 2)
                _ln_stage(xres, xn, (t_idx == 0).astype(I32))

        @pl.when(l == N_LAYERS - 1)
        def _():
            with _scope('ffn'):
                new_hint()
                y = _ffn_last(lhs, idx, wffn, col, hint[0]) * jax.nn.sigmoid(rmax)
                for sb in range(NSB):
                    out_copy(sb * SB, SB, sb).wait()
                g0 = _add_to_row(xres, idx, y)
            with _scope('ofinal'):
                cp = out_copy(g0, 16, NSB)
                cp.start()
                cp.wait()

        return carry

    jax.lax.fori_loop(0, N_LAYERS, layer, 0)


@jax.jit
def pallas_interleave_layers__sliding_block__moe_arch_mod__prompt_kernel(
    A_x: jax.Array,
    A_wqkv: jax.Array,
    A_wo: jax.Array,
    B_x: jax.Array,
    B_w_r: jax.Array,
    B_w_gate: jax.Array,
    B_w_up: jax.Array,
    B_w_down: jax.Array,
):
    del B_x
    any_spec = pl.BlockSpec(memory_space=pl.ANY)
    scratch = [
        pltpu.VMEM((S, D), BF16),
        pltpu.VMEM((NG, S, 128), BF16),
        pltpu.VMEM((NG, S, 128), BF16),
        pltpu.VMEM((NG, S, 128), BF16),
        pltpu.VMEM((NSB + 2, D, 128), BF16),
        pltpu.VMEM((NG, 4, XR, 128), F32),
        pltpu.VMEM((NG, 4, 8, 128), F32),
        pltpu.VMEM((NG, 4, XR, 128), BF16),
        pltpu.VMEM((NG, 4, 8, 128), F32),
        pltpu.VMEM((NG, SB, 128), BF16),
        pltpu.VMEM((3 * NG, D, 128), BF16),
        pltpu.VMEM((NG, D, 128), BF16),
        pltpu.VMEM((1, D), F32),
        pltpu.VMEM((NW, D, 128), BF16),
        pltpu.VMEM((COL_DUMMY + 1, D, 128), F32),
        pltpu.VMEM((NW + 1, 8, 128), F32),
        pltpu.VMEM((1, 1), F32),
        pltpu.VMEM((8, 1), F32),
        pltpu.VMEM((8, 1), I32),
        pltpu.SMEM((1,), I32),
        pltpu.SMEM((NTB,), I32),
        pltpu.SMEM((1,), I32),
        pltpu.SMEM((3 * FS_STEPS * (FS_N + FS_BC),), I32),
        pltpu.SemaphoreType.DMA((NTB,)),
        pltpu.SemaphoreType.DMA((3 * NG // W_GROUP,)),
        pltpu.SemaphoreType.DMA((2,)),
        pltpu.SemaphoreType.DMA((NSB + 1,)),
    ]
    return pl.pallas_call(
        _kernel,
        out_shape=jax.ShapeDtypeStruct((1, S, D), BF16),
        in_specs=[any_spec, any_spec, any_spec,
                  pl.BlockSpec(memory_space=pltpu.VMEM),
                  any_spec, any_spec, any_spec],
        out_specs=any_spec,
        scratch_shapes=scratch,
        compiler_params=pltpu.CompilerParams(vmem_limit_bytes=112 * 1024 * 1024),
        name="swa_moe",
    )(A_x, A_wqkv, A_wo, B_w_r, B_w_gate, B_w_up, B_w_down)
```

```python
import math

import jax
import jax.numpy as jnp
import jax.experimental.pallas as pl
import jax.experimental.pallas.tpu as pltpu

F32 = jnp.float32
BF16 = jnp.bfloat16
U32 = jnp.uint32
I32 = jnp.int32

S = 2048
D = 1024
DH = 32
WIN = 256
FF = 3584
NG = 8
SB = 128
NSB = S // SB
QA = 32
XR = WIN + QA
TB = 256
NTB = S // TB
EPS = 1e-5
NEG = -1e30
QSCALE = (DH ** -0.5) * math.log2(math.e)
NT_DIMS = (((1,), (1,)), ((), ()))
N_LAYERS = 2
NFC = FF // 128
KB = 4
NW = 2 * NFC + NG * KB
FS_STEPS = 5
FS_N = 20
FS_BC = 10
FS_LAG = 3
COL_DUMMY = 1 + KB
FFN_VPU = 8
P1_LAST_SCORES_AT = 16
POST_PV_AT = 7
POST_EARLY_EXP = 1
W_GROUP = 4


def _scope(name):
    return jax.named_scope(name)


def _layernorm(x):
    mean = jnp.sum(x, axis=1, keepdims=True) * (1.0 / D)
    xc = x - mean
    var = jnp.sum(xc * xc, axis=1, keepdims=True) * (1.0 / D)
    return xc * jax.lax.rsqrt(var + EPS)


def _packed(ref):
    return ref.bitcast(U32)


def _as_bf16(v):
    return pltpu.bitcast(v, BF16)


def _ln_stage(xres, xn, t, rows=TB):
    r0 = t * rows if isinstance(t, int) else pl.multiple_of(t * rows, rows)
    y = _layernorm(xres[pl.ds(r0, rows), :].astype(F32))
    for c in range(NG):
        xn[c, pl.ds(r0, rows), :] = y[:, c * 128:(c + 1) * 128].astype(BF16)


QKV_ORDER = list(range(2 * NG, 3 * NG)) + list(range(2 * NG))


def _qkv_lhs(xn, h0):
    xp = _packed(xn)
    return _as_bf16(jnp.concatenate(
        [xp[c, pl.ds(h0, TB // 2), :] for c in range(NG)], axis=1))


def _first_group_chunk(k, n):
    if isinstance(k, int):
        if k < 4:
            return (2 * NG + 2 * k + n) if n < 2 else (2 * k + n - 2)
        return NG + 4 * (k - 4) + n
    a = (2 * NG + 2 * k + n) if n < 2 else (2 * k + n - 2)
    return jnp.where(k < 4, a, NG + 4 * (k - 4) + n)


def _qkv_stage(xn, wqkv, qs, ks, vts, t, before_chunk=None, after_chunk=None):
    wp = _packed(wqkv)
    if isinstance(t, int):
        r0, h0 = t * TB, t * (TB // 2)
    else:
        r0 = pl.multiple_of(t * TB, TB)
        h0 = pl.multiple_of(t * (TB // 2), TB // 2)
    kt0 = 2 + t * (TB // 128)
    lhs = _qkv_lhs(xn, h0)
    for n, j in enumerate(QKV_ORDER):
        if before_chunk is not None:
            before_chunk(n)
        y = jnp.dot(lhs, _as_bf16(wp[j]), preferred_element_type=F32)
        if after_chunk is not None:
            after_chunk(n, y[0:8])
        if j < NG:
            qs[j, pl.ds(r0, TB), :] = (y * QSCALE).astype(BF16)
        elif j < 2 * NG:
            ks[j - NG, pl.ds(r0, TB), :] = y.astype(BF16)
        else:
            c = j - 2 * NG
            for t in range(TB // 128):
                vts[kt0 + t, c * 128:(c + 1) * 128, :] = (
                    y[t * 128:(t + 1) * 128, :].T.astype(BF16))


def _score_stage(qs, ks, xs, ms, sb, g, static_sb=None, b=None):
    lane = jax.lax.broadcasted_iota(I32, (QA, 128), 1)
    li = lane % QA
    row = jax.lax.broadcasted_iota(I32, (QA, 128), 0)
    m_lo = row > li
    m_hi = row <= li
    lg = jax.lax.broadcasted_iota(I32, (QA // 2, 128), 1) // QA
    qp = _packed(qs)
    kp = _packed(ks)
    b = g if b is None else b
    for a in range(4):
        if static_sb is None:
            qa2 = pl.multiple_of(sb * (SB // 2) + (QA // 2) * a, QA // 2)
            q = qp[g, pl.ds(qa2, QA // 2), :]
            first = 0
            k = kp[g, pl.ds(qa2 - WIN // 2, XR // 2), :]
        else:
            qa = static_sb * SB + QA * a
            q = qp[g, qa // 2:(qa + QA) // 2, :]
            first = WIN - qa
            k = kp[g, 0:(XR - first) // 2, :]
        qbd = jnp.concatenate(
            [jnp.where(lg == ((a - p) % 4), q, jnp.zeros_like(q)) for p in range(4)],
            axis=0)
        x = jax.lax.dot_general(_as_bf16(k), _as_bf16(qbd), NT_DIMS,
                                preferred_element_type=F32)
        n = XR - first
        hi = jnp.where(m_hi, x[n - QA:n], NEG)
        if first == 0:
            lo = jnp.where(m_lo, x[0:QA], NEG)
            x = jnp.concatenate([lo, x[QA:n - QA], hi], axis=0)
        elif n > QA:
            x = jnp.concatenate(
                [jnp.full((first, 128), NEG, F32), x[0:n - QA], hi], axis=0)
        else:
            x = jnp.concatenate([jnp.full((first, 128), NEG, F32), hi], axis=0)
        xs[b, a] = x
        j0 = first // 16
        m0 = x[16 * j0:16 * j0 + 8]
        m1 = x[16 * j0 + 8:16 * j0 + 16]
        for j in range(j0 + 1, XR // 16):
            m0 = jnp.maximum(m0, x[16 * j:16 * j + 8])
            m1 = jnp.maximum(m1, x[16 * j + 8:16 * j + 16])
        mm = jnp.max(jnp.maximum(m0, m1), axis=0, keepdims=True)
        ms[b, a] = jnp.broadcast_to(mm, (8, 128))
    return m0


def _exp_stage(xs, ms, ps, ls, g, never, after=None):
    for a in range(4):
        m = ms[g, a]
        if after is not None:
            m = jnp.where(never, after, m)
        s0 = s1 = None
        for j in range(XR // 16):
            e0 = jnp.exp2(xs[g, a, 16 * j:16 * j + 8, :] - m)
            e1 = jnp.exp2(xs[g, a, 16 * j + 8:16 * j + 16, :] - m)
            s0 = e0 if s0 is None else s0 + e0
            s1 = e1 if s1 is None else s1 + e1
            if j == XR // 16 - 1:
                s = s0 + s1
                e1 = jnp.where(never, s, e1)
            ps[g, a, 16 * j:16 * j + 16, :] = (
                jnp.concatenate([e0, e1], axis=0).astype(BF16))
        ls[g, a] = s


def _pv_stage(ps, ls, vts, sb, g, b=None):
    lg8 = jax.lax.broadcasted_iota(I32, (8, 128), 1) // QA
    odd = (lg8 % 2) == 1
    hi2 = lg8 >= 2
    zero = jnp.zeros((8, 128), U32)
    pp = _packed(ps)
    vp = _packed(vts)
    b = g if b is None else b

    def sel(c, x, y):
        if x is None and y is None:
            return None
        return jnp.where(c, zero if x is None else x, zero if y is None else y)

    acc = [None] * 4
    for kt in range(3):
        yrows = [[] for _ in range(4)]
        for r in range(8 * kt, 8 * kt + 8):
            pr = []
            for a in range(4):
                j = r - 2 * a
                pr.append(pp[b, a, 8 * j:8 * j + 8, :] if 0 <= j < XR // 16 else None)
            z = [sel(odd, pr[(a + 1) % 4], pr[a]) for a in range(4)]
            for h in range(4):
                y = sel(hi2, z[(h + 2) % 4], z[h])
                yrows[h].append(zero if y is None else y)
        for h in range(4):
            y = _as_bf16(jnp.concatenate(yrows[h], axis=0))
            r0 = (g * 128 + DH * h) // 2
            vt = _as_bf16(vp[sb + kt, r0:r0 + DH // 2, :])
            ot = jnp.dot(vt, y, preferred_element_type=F32)
            acc[h] = ot if acc[h] is None else acc[h] + ot
    l = [jnp.sum(ls[b, a], axis=0, keepdims=True) for a in range(4)]
    lg1 = jax.lax.broadcasted_iota(I32, (1, 128), 1) // QA
    lz = [jnp.where((lg1 % 2) == 1, l[(a + 1) % 4], l[a]) for a in range(4)]
    ly = [jnp.where(lg1 >= 2, lz[(h + 2) % 4], lz[h]) for h in range(4)]
    return jnp.concatenate([acc[h] * (1.0 / ly[h]) for h in range(4)], axis=0)


def _unrotate_stage(ot, os_, g):
    t = ot.T
    lgrp = jax.lax.broadcasted_iota(I32, (QA, 128), 1) // QA
    odd = (lgrp % 2) == 1
    hi2 = lgrp >= 2
    tp = [t[QA * p:QA * p + QA] for p in range(4)]
    z = [jnp.where(odd, tp[(a - 1) % 4], tp[a]) for a in range(4)]
    outs = [jnp.where(hi2, z[(a - 2) % 4], z[a]) for a in range(4)]
    os_[g] = jnp.concatenate(outs, axis=0).astype(BF16)


def _proj_matmul(os_, wo, never, overlap=None, fence=None, fence_at=NG - 1,
                 before_chunk=None):
    op = _packed(os_)
    wp = _packed(wo)
    lhs = jnp.concatenate([op[g] for g in range(NG)], axis=1)
    cols = []
    for j in range(NG):
        if before_chunk is not None:
            before_chunk(j)
        lj = lhs
        if overlap is not None and j == fence_at:
            head = jnp.where(never, fence(), lhs[0:8, 0:128])
            top = jnp.concatenate([head, lhs[0:8, 128:]], axis=1)
            lj = jnp.concatenate([top, lhs[8:]], axis=0)
        y = jnp.dot(_as_bf16(lj), _as_bf16(wp[j]), preferred_element_type=F32)
        cols.append(y)
        if overlap is not None and j == 0:
            overlap(y[0:8])
    return jnp.concatenate(cols, axis=1)


def _norm_stage(acc, wr, xres, xn, best_v, best_i, sb, lo, hi, never, after=None):
    r0 = (sb * SB if isinstance(sb, int) else pl.multiple_of(sb * SB, SB)) + lo
    n = hi - lo
    x = xres[pl.ds(r0, n), :].astype(F32) + acc[lo:hi]
    mean = jnp.sum(x, axis=1, keepdims=True) * (1.0 / D)
    if after is not None:
        mean = jnp.where(never[0:1, 0:1], after[0:1, 0:1], mean)
    xc = x - mean
    var = jnp.sum(xc * xc, axis=1, keepdims=True) * (1.0 / D)
    rstd = jax.lax.rsqrt(var + EPS)
    y = x * rstd - mean * rstd
    r = jnp.sum(y * wr[...], axis=1, keepdims=True)
    xres[pl.ds(r0, n), :] = (x + y).astype(BF16)
    for c in range(NG):
        xn[c, pl.ds(r0, n), :] = y[:, c * 128:(c + 1) * 128].astype(BF16)
    bv = best_v[...]
    bi = best_i[...]
    sub = jax.lax.broadcasted_iota(I32, (8, 1), 0)
    for rg in range(n // 8):
        rr = r[8 * rg:8 * rg + 8]
        take = rr > bv
        bv = jnp.where(take, rr, bv)
        bi = jnp.where(take, sub + (r0 + 8 * rg), bi)
    best_v[...] = bv
    best_i[...] = bi


def _wd_idx(j, kb):
    return 2 * NFC + KB * j + kb


def _router(best_v, best_i):
    bv = best_v[...]
    rmax = jnp.max(bv, axis=0, keepdims=True)
    idx = jnp.min(jnp.where(bv == rmax, best_i[...], S))
    return rmax, idx


def _row_group(xn, idx):
    h0 = pl.multiple_of((idx >> 4) * 8, 8)
    xp = _packed(xn)
    return _as_bf16(jnp.concatenate(
        [xp[c, pl.ds(h0, 8), :] for c in range(NG)], axis=1))


def _add_to_row(xres, idx, y):
    g0 = pl.multiple_of((idx >> 4) * 16, 16)
    row = jax.lax.broadcasted_iota(I32, (16, D), 0)
    upd = jnp.where(row == (idx & 15), y, 0.0)
    xres[pl.ds(g0, 16), :] = (xres[pl.ds(g0, 16), :].astype(F32) + upd).astype(BF16)
    return g0


def _select_row(v, idx):
    row = jax.lax.broadcasted_iota(I32, v.shape, 0)
    return jnp.sum(jnp.where(row == (idx & 15), v, 0.0), axis=0, keepdims=True)


def _store_x_cols(col, lhs, idx):
    x = _select_row(lhs.astype(F32), idx)
    for c in range(NG):
        col[0, c * 128:(c + 1) * 128, :] = _bcast_cols(x[:, c * 128:(c + 1) * 128])


def _ffn_last(lhs, idx, wffn, col, never):
    wp = _packed(wffn)
    _store_x_cols(col, lhs, idx)
    todo = [(j, u) for j in range(NFC - FFN_VPU, NFC) for u in range(2)]
    h = {}
    n = 0
    for j in range(NFC - FFN_VPU):
        for u in range(2):
            y = jnp.dot(lhs, _as_bf16(wp[u * NFC + j]), preferred_element_type=F32)
            h[j, u] = _select_row(y, idx)
            if n >= 4 and n % 2 == 0 and todo:
                jj, uu = todo.pop(0)
                part = _matvec_chunk(wffn, uu * NFC + jj, col, 0, never, y[0:8])
                h[jj, uu] = jnp.sum(part, axis=0, keepdims=True)
            n += 1
    assert not todo
    act = jnp.concatenate(
        [h[j, 0] * jax.nn.sigmoid(h[j, 0]) * h[j, 1] for j in range(NFC)], axis=1)
    act = jnp.broadcast_to(act, (16, FF)).astype(BF16)
    cols = []
    for j in range(NG):
        w = jnp.concatenate(
            [wp[_wd_idx(j, kb), 0:(min(FF, (kb + 1) * D) - kb * D) // 2, :]
             for kb in range(KB)], axis=0)
        cols.append(jnp.dot(act, _as_bf16(w), preferred_element_type=F32)[0:1])
    return jnp.concatenate(cols, axis=1)


def _bcast_cols(row):
    return jnp.broadcast_to(row, (128, 128)).T


def _matvec_chunk(wffn, w, col, c, never, after):
    wp = _packed(wffn)
    acc = None
    for g in range(D // 16):
        v = wp[w, 8 * g:8 * g + 8, :]
        if g == 0:
            v = jnp.where(never, pltpu.bitcast(after, U32), v)
        t = _as_bf16(v).astype(F32) * col[c, 16 * g:16 * g + 16, :]
        acc = t if acc is None else acc + t
    return acc[0:8] + acc[8:16]


def _fs_tables():
    mv, bc = [], []
    for k in range(FS_STEPS):
        for n in range(FS_N):
            if k < 3:
                j = FS_BC * k + n % FS_BC
                w = min(j, NFC - 1) + (NFC if n >= FS_BC else 0)
                mv.append((w, 0, w if j < NFC else NW))
            else:
                j, kb = (n % 16) // 2, 2 * (k - 3) + n % 2
                w = _wd_idx(j, kb)
                mv.append((w, 1 + kb, w if n < 16 else NW))
        for m in range(FS_BC):
            j = FS_BC * (k - 1) + m
            if 1 <= k <= 3 and j < NFC:
                bc.append((j, 1 + j // NG, j % NG))
            else:
                bc.append((m, COL_DUMMY, m % NG))
    return mv, bc


def _kernel(x_hbm, wqkv_hbm, wo_hbm, wr_ref, wg_hbm, wu_hbm, wd_hbm, out_hbm,
            xres, xn, qs, ks, vts, xs, ms, ps, ls, os_, wqkv, wo, wr, wffn, col, hp, gate,
            best_v, best_i, zero, order, sel, tab, sem_x, sem_q, sem_w, sem_o):
    zero[0] = 0

    x_cp = [pltpu.make_async_copy(x_hbm.at[0, pl.ds(t * TB, TB), :],
                                  xres.at[pl.ds(t * TB, TB), :], sem_x.at[t])
            for t in range(NTB)]
    def wqkv_group(k):
        cps = []
        for n in range(W_GROUP):
            j = _first_group_chunk(k, n)
            c0 = j * 128 if isinstance(j, int) else pl.multiple_of(j * 128, 128)
            cps.append(pltpu.make_async_copy(wqkv_hbm.at[:, pl.ds(c0, 128)],
                                             wqkv.at[j], sem_q.at[k]))
        return cps

    wo_cp = [pltpu.make_async_copy(wo_hbm.at[:, pl.ds(j * 128, 128)],
                                   wo.at[j], sem_w.at[0])
             for j in range(NG)]
    ffn_cp = [pltpu.make_async_copy(src.at[:, pl.ds(j * 128, 128)],
                                    wffn.at[off + j], sem_w.at[1])
              for src, off in ((wg_hbm, 0), (wu_hbm, NFC)) for j in range(NFC)]
    for j in range(NG):
        for kb in range(KB):
            rows = min(FF, (kb + 1) * D) - kb * D
            ffn_cp.append(pltpu.make_async_copy(
                wd_hbm.at[pl.ds(kb * D, rows), pl.ds(j * 128, 128)],
                wffn.at[_wd_idx(j, kb), pl.ds(0, rows), :], sem_w.at[1]))
    x_cp[0].start()

    with _scope('init'):
        vts[0:2] = jnp.zeros((2,) + vts.shape[1:], BF16)
        wr[...] = wr_ref[...].astype(F32).reshape(1, D)
        pad = KB * D - FF
        for j in range(NG):
            wffn[_wd_idx(j, KB - 1), D - pad:D, :] = jnp.zeros((pad, 128), BF16)
        col[KB, D - pad:D, :] = jnp.zeros((pad, 128), F32)
        hp[...] = jnp.zeros(hp.shape, F32)
        for t in range(NTB):
            order[t] = t
        mv_tab, bc_tab = _fs_tables()
        for i, v in enumerate(sum(mv_tab + bc_tab, ())):
            tab[i] = v
    for cp in wqkv_group(0):
        cp.start()
    with _scope('xwait'):
        x_cp[0].wait()
    for cp in wqkv_group(1) + x_cp[1:2]:
        cp.start()

    def out_copy(r0, n, slot):
        return pltpu.make_async_copy(xres.at[pl.ds(r0, n), :],
                                     out_hbm.at[0, pl.ds(r0, n), :], sem_o.at[slot])

    def layer(l, carry):
        hint = [None]

        def new_hint():
            hint[0] = jnp.full((8, 128), zero[0], I32) != 0


        @pl.when(l == 0)
        def _():
            with _scope('ln0'):
                _ln_stage(xres, xn, 0)

            wp = _packed(wqkv)

            def vq_group(k, c):
                for cp in wqkv_group(k):
                    cp.wait()
                for cp in wqkv_group(k + 2):
                    cp.start()
                lhs = _qkv_lhs(xn, 0)
                for n in range(W_GROUP):
                    j = _first_group_chunk(k, n)
                    y = jnp.dot(lhs, _as_bf16(wp[j]), preferred_element_type=F32)
                    if n < 2:
                        c0 = pl.multiple_of((j - 2 * NG) * 128, 128)
                        for t in range(TB // 128):
                            vts[2 + t, pl.ds(c0, 128), :] = (
                                y[t * 128:(t + 1) * 128, :].T.astype(BF16))
                    else:
                        qs[j, 0:TB, :] = (y * QSCALE).astype(BF16)
                return c

            def k_group(i, c):
                for cp in wqkv_group(4 + i):
                    cp.wait()

                @pl.when(i == 0)
                def _():
                    x_cp[1].wait()

                @pl.when(i == 1)
                def _():
                    for cp in x_cp[2:]:
                        cp.start()

                lhs = _qkv_lhs(xn, 0)
                for n in range(W_GROUP):
                    j = NG + W_GROUP * i + n
                    y = jnp.dot(lhs, _as_bf16(wp[j]), preferred_element_type=F32)
                    ks[j - NG, 0:TB, :] = y.astype(BF16)
                _ln_stage(xres, xn, TB // 128 + i, rows=128)
                return c

            with _scope('p1_first'):
                jax.lax.fori_loop(0, 4, vq_group, 0)
                jax.lax.fori_loop(0, 2, k_group, 0)

        def wait_x(t):
            @pl.when(l == 0)
            def _():
                pltpu.make_async_copy(
                    x_hbm.at[0, pl.ds(t * TB, TB), :],
                    xres.at[pl.ds(t * TB, TB), :], sem_x.at[t]).wait()

        def p1_step(k, c):
            wait_x(k + 1)

            @pl.when(jnp.logical_and(l == 0, k == 2))
            def _():
                for cp in wo_cp + ffn_cp[:2 * NFC]:
                    cp.start()

            @pl.when(jnp.logical_and(l == 0, k == 5))
            def _():
                for cp in ffn_cp[2 * NFC:]:
                    cp.start()

            _qkv_stage(xn, wqkv, qs, ks, vts, order[k])
            _ln_stage(xres, xn, order[k + 1])
            return c

        def fs_step(k, c):
            new_hint()
            b0 = 3 * (FS_STEPS * FS_N + k * FS_BC)
            for m in range(FS_BC):
                j, cs, rb = (tab[b0 + 3 * m + i] for i in range(3))
                hg = jnp.sum(hp[j], axis=0, keepdims=True)
                hu = jnp.sum(hp[NFC + j], axis=0, keepdims=True)
                a = (hg * jax.nn.sigmoid(hg) * hu).astype(BF16).astype(F32)
                col[cs, pl.ds(pl.multiple_of(rb * 128, 128), 128), :] = _bcast_cols(a)

            def matvec(n, y):
                n -= FS_LAG
                if 0 <= n < FS_N:
                    w, cs, slot = (tab[3 * (k * FS_N + n) + i] for i in range(3))
                    hp[slot] = _matvec_chunk(wffn, w, col, cs, hint[0], y)

            _qkv_stage(xn, wqkv, qs, ks, vts, order[k], after_chunk=matvec)
            _ln_stage(xres, xn, order[k + 1])
            return c

        @pl.when(l == 1)
        def _():
            with _scope('fs_loop'):
                jax.lax.fori_loop(0, FS_STEPS, fs_step, 0)
            with _scope('fs_fin'):
                y = jnp.concatenate(
                    [jnp.sum(sum(hp[_wd_idx(j, kb)] for kb in range(KB)),
                             axis=0, keepdims=True) for j in range(NG)], axis=1)
                _add_to_row(xres, sel[0], y * gate[...])

        with _scope('p1_loop'):
            jax.lax.fori_loop(jnp.where(l == 0, 1, FS_STEPS), NTB - 1, p1_step, 0)

        best_v[...] = jnp.full((8, 1), -jnp.inf, F32)
        best_i[...] = jnp.zeros((8, 1), I32)

        def pv_all(sb, groups=range(NG)):
            for g in groups:
                _unrotate_stage(_pv_stage(ps, ls, vts, sb, g), os_, g)

        def exp_groups(gs, after=None):
            for g in gs:
                _exp_stage(xs, ms, ps, ls, g, hint[0], after)

        def proj(exp_gs=None, **kw):
            if exp_gs is None:
                return _proj_matmul(os_, wo, hint[0], **kw)
            return _proj_matmul(os_, wo, hint[0],
                                overlap=lambda v: exp_groups(exp_gs, v),
                                fence=lambda: _packed(ps)[zero[0], 0, 0:8, :], **kw)

        def norm(acc, sb, lo=0, hi=SB, after=None):
            _norm_stage(acc, wr, xres, xn, best_v, best_i, sb, lo, hi, hint[0], after)

        def emit_out(sbs):
            @pl.when(l == N_LAYERS - 1)
            def _():
                for sb in sbs:
                    out_copy(sb * SB, SB, sb).start()

        one = zero[0] + 1

        def p1_last(_, c):
            new_hint()
            for g in range(NG):
                _score_stage(qs, ks, xs, ms, None, g, static_sb=0)
            exp_groups(range(NG))

            def mid(n):
                if n == P1_LAST_SCORES_AT:
                    for g in range(NG):
                        _score_stage(qs, ks, xs, ms, None, g, static_sb=1)

            _qkv_stage(xn, wqkv, qs, ks, vts, NTB - 1, mid)
            return c

        def steady(s, c):
            new_hint()
            g0 = NG - 1
            pv_all(s - 1, [g0] + list(range(g0)))
            exp_groups([g0])
            _score_stage(qs, ks, xs, ms, s + 1, g0)
            norm(proj(range(g0)), s - 1)
            for g in range(g0):
                _score_stage(qs, ks, xs, ms, s + 1, g)
            return c

        def post(_, c):
            new_hint()
            pv_all(NSB - 2)

            def mid(j):
                if j == POST_PV_AT:
                    pv_all(NSB - 1)

            exp_groups(range(POST_EARLY_EXP))
            norm(proj(range(POST_EARLY_EXP, NG), fence_at=POST_PV_AT - 1,
                      before_chunk=mid), NSB - 2)
            norm(proj(), NSB - 1)
            return c

        with _scope('p1_last'):
            jax.lax.fori_loop(0, one, p1_last, 0)

        @pl.when(l == 0)
        def _():
            with _scope('wowait'):
                for cp in wo_cp:
                    cp.wait()

        with _scope('steady'):
            jax.lax.fori_loop(1, NSB - 1, steady, 0)
        emit_out(range(NSB - 2))
        with _scope('post'):
            jax.lax.fori_loop(0, one, post, 0)
        emit_out(range(NSB - 2, NSB))

        rmax, idx = _router(best_v, best_i)
        lhs = _row_group(xn, idx)

        @pl.when(l == 0)
        def _():
            with _scope('route'):
                for cp in ffn_cp:
                    cp.wait()
                sel[0] = idx
                gate[...] = jax.nn.sigmoid(rmax)
                _store_x_cols(col, lhs, idx)
                t_idx = idx // TB
                for p in range(NTB - 2):
                    order[p] = p + (p >= t_idx).astype(I32)
                order[NTB - 2] = jnp.minimum(t_idx, NTB - 2)
                _ln_stage(xres, xn, (t_idx == 0).astype(I32))

        @pl.when(l == N_LAYERS - 1)
        def _():
            with _scope('ffn'):
                new_hint()
                y = _ffn_last(lhs, idx, wffn, col, hint[0]) * jax.nn.sigmoid(rmax)
                for sb in range(NSB):
                    out_copy(sb * SB, SB, sb).wait()
                g0 = _add_to_row(xres, idx, y)
            with _scope('ofinal'):
                cp = out_copy(g0, 16, NSB)
                cp.start()
                cp.wait()

        return carry

    jax.lax.fori_loop(0, N_LAYERS, layer, 0)


@jax.jit
def pallas_interleave_layers__sliding_block__moe_arch_mod__prompt_kernel(
    A_x: jax.Array,
    A_wqkv: jax.Array,
    A_wo: jax.Array,
    B_x: jax.Array,
    B_w_r: jax.Array,
    B_w_gate: jax.Array,
    B_w_up: jax.Array,
    B_w_down: jax.Array,
):
    del B_x
    any_spec = pl.BlockSpec(memory_space=pl.ANY)
    scratch = [
        pltpu.VMEM((S, D), BF16),
        pltpu.VMEM((NG, S, 128), BF16),
        pltpu.VMEM((NG, S, 128), BF16),
        pltpu.VMEM((NG, S, 128), BF16),
        pltpu.VMEM((NSB + 2, D, 128), BF16),
        pltpu.VMEM((NG, 4, XR, 128), F32),
        pltpu.VMEM((NG, 4, 8, 128), F32),
        pltpu.VMEM((NG, 4, XR, 128), BF16),
        pltpu.VMEM((NG, 4, 8, 128), F32),
        pltpu.VMEM((NG, SB, 128), BF16),
        pltpu.VMEM((3 * NG, D, 128), BF16),
        pltpu.VMEM((NG, D, 128), BF16),
        pltpu.VMEM((1, D), F32),
        pltpu.VMEM((NW, D, 128), BF16),
        pltpu.VMEM((COL_DUMMY + 1, D, 128), F32),
        pltpu.VMEM((NW + 1, 8, 128), F32),
        pltpu.VMEM((1, 1), F32),
        pltpu.VMEM((8, 1), F32),
        pltpu.VMEM((8, 1), I32),
        pltpu.SMEM((1,), I32),
        pltpu.SMEM((NTB,), I32),
        pltpu.SMEM((1,), I32),
        pltpu.SMEM((3 * FS_STEPS * (FS_N + FS_BC),), I32),
        pltpu.SemaphoreType.DMA((NTB,)),
        pltpu.SemaphoreType.DMA((3 * NG // W_GROUP,)),
        pltpu.SemaphoreType.DMA((2,)),
        pltpu.SemaphoreType.DMA((NSB + 1,)),
    ]
    return pl.pallas_call(
        _kernel,
        out_shape=jax.ShapeDtypeStruct((1, S, D), BF16),
        in_specs=[any_spec, any_spec, any_spec,
                  pl.BlockSpec(memory_space=pltpu.VMEM),
                  any_spec, any_spec, any_spec],
        out_specs=any_spec,
        scratch_shapes=scratch,
        compiler_params=pltpu.CompilerParams(vmem_limit_bytes=112 * 1024 * 1024),
        name="swa_moe",
    )(A_x, A_wqkv, A_wo, B_w_r, B_w_gate, B_w_up, B_w_down)
```
